```python
import jax
import jax.numpy as jnp

def _softmax(x, axis=-1):
    return jax.nn.softmax(x, axis=axis)

def _gelu(x):
    return jax.nn.gelu(x, approximate=True)

def _silu(x):
    return jax.nn.silu(x)

def _sigmoid(x):
    return jax.nn.sigmoid(x)

def _layernorm(x, axis=-1, eps=1e-05):
    m = jnp.mean(x, axis=axis, keepdims=True)
    v = jnp.var(x, axis=axis, keepdims=True)
    return (x - m) / jnp.sqrt(v + eps)

def _scatter_add(tgt, idx, src, axis=0):
    return tgt.at[idx].add(src)

def _segment_sum(src, seg, n):
    return jax.ops.segment_sum(src, seg, n)

class _Rng:

    def __init__(self, key):
        self._k = key

    def _next(self):
        self._k, sub = jax.random.split(self._k)
        return sub

    def normal(self, shape):
        return jax.random.normal(self._next(), shape, dtype=jnp.bfloat16)

    def randint(self, lo, hi, shape):
        return jax.random.randint(self._next(), shape, lo, hi, dtype=jnp.int32)

    def uniform(self, shape, lo=0.0, hi=1.0):
        return jax.random.uniform(self._next(), shape, jnp.bfloat16, lo, hi)

    def permutation(self, n):
        return jax.random.permutation(self._next(), n)
kernel_name = 'interleave_layers__memory_aug_recurrent_mem_tr__glu_gated_swiglu__prompt'

def setup_inputs():
    _rng = _Rng(jax.random.key(int.from_bytes(__import__("os").urandom(4), "little")))
    _w = lambda a: (lambda t: t.astype(jnp.bfloat16) if jnp.issubdtype(t.dtype, jnp.floating) else t)(jnp.asarray(a))

    def _A_setup():
        B, S, Dm = (1, 2048, 576)
        H, Dh = (32, 128)
        M, seg = (8, 32)
        seg = min(seg, S)
        S = S // seg * seg
        return {'x': _w((lambda *s: _rng.normal(s) * 0.05)(B, S, Dm)), 'mem0': _w((lambda *s: _rng.normal(s) * 0.05)(B, M, Dm)), 'Wq': _w((lambda *s: _rng.normal(s) * 0.05)(Dm, H, Dh) * Dm ** (-0.5)), 'Wk': _w((lambda *s: _rng.normal(s) * 0.05)(Dm, H, Dh) * Dm ** (-0.5)), 'Wv': _w((lambda *s: _rng.normal(s) * 0.05)(Dm, H, Dh) * Dm ** (-0.5)), 'Wo': _w((lambda *s: _rng.normal(s) * 0.05)(H, Dh, Dm) * (H * Dh) ** (-0.5)), 'seg_len': seg}
    _A_in = _A_setup()

    def _B_setup():
        B, S, D, F = (1, 2048, 576, 4608)
        return {'x': _w((lambda *s: _rng.normal(s) * 0.05)(B, S, D)), 'w1': _w((lambda *s: _rng.normal(s) * 0.05)(D, F) * (2.0 / D) ** 0.5), 'w3': _w((lambda *s: _rng.normal(s) * 0.05)(D, F) * (2.0 / D) ** 0.5), 'w2': _w((lambda *s: _rng.normal(s) * 0.05)(F, D) * (2.0 / F) ** 0.5)}
    _B_in = _B_setup()
    return {'A_x': _A_in['x'], 'A_mem0': _A_in['mem0'], 'A_Wq': _A_in['Wq'], 'A_Wk': _A_in['Wk'], 'A_Wv': _A_in['Wv'], 'A_Wo': _A_in['Wo'], 'A_seg_len': _A_in['seg_len'], 'B_x': _B_in['x'], 'B_w1': _B_in['w1'], 'B_w3': _B_in['w3'], 'B_w2': _B_in['w2']}

def reference(A_x, A_mem0, A_Wq, A_Wk, A_Wv, A_Wo, A_seg_len, B_x, B_w1, B_w3, B_w2):

    def _A_ref(x, mem0, Wq, Wk, Wv, Wo, seg_len):
        B, S, Dm = x.shape
        H, Dh = (Wq.shape[1], Wq.shape[2])
        M = mem0.shape[1]
        scale = Dh ** (-0.5)
        n_seg = S // seg_len
        L = M + seg_len
        idx = jnp.arange(L)
        mask = (idx[:, None] < M) | (idx[:, None] >= idx[None, :])
        mem = mem0
        outs = []
        for s in range(n_seg):
            xs = x[:, s * seg_len:(s + 1) * seg_len, :].copy()
            h = jnp.concatenate([mem, xs], axis=1)
            q = jnp.einsum('btd,dhe->bhte', h, Wq)
            k = jnp.einsum('btd,dhe->bhte', h, Wk)
            v = jnp.einsum('btd,dhe->bhte', h, Wv)
            scores = jnp.einsum('bhqe,bhke->bhqk', q, k) * scale
            scores = jnp.where(mask[None, None], scores, -1000000000.0)
            p = _softmax(scores, axis=-1)
            o = jnp.einsum('bhqk,bhke->bhqe', p, v)
            o = jnp.einsum('bhte,hed->btd', o, Wo)
            mem = o[:, :M, :].copy()
            outs.append(o[:, M:, :])
        return jnp.concatenate(outs, axis=1)

    def _B_ref(x, w1, w3, w2):
        gate = jnp.einsum('bsd,df->bsf', x, w1)
        up = jnp.einsum('bsd,df->bsf', x, w3)
        h = _silu(gate) * up
        out = jnp.einsum('bsf,fd->bsd', h, w2)
        return out
    x = A_x
    x = x + _A_ref(_layernorm(x, axis=-1), A_mem0, A_Wq, A_Wk, A_Wv, A_Wo, A_seg_len)
    x = x + _B_ref(_layernorm(x, axis=-1), B_w1, B_w3, B_w2)
    x = x + _A_ref(_layernorm(x, axis=-1), A_mem0, A_Wq, A_Wk, A_Wv, A_Wo, A_seg_len)
    x = x + _B_ref(_layernorm(x, axis=-1), B_w1, B_w3, B_w2)
    return x
```

```python
import functools

import jax
import jax.numpy as jnp
import numpy as np
from jax import lax
import jax.experimental.pallas as pl
import jax.experimental.pallas.tpu as pltpu

_BF16 = jnp.bfloat16
_F32 = jnp.float32
_NT = (((1,), (1,)), ((), ()))
_TOK = 128
_GROUP = 4
_FCHUNK = 512
_WCHUNK = 64
_INFLIGHT = 3
_MASKED = -1000000000.0


def _layernorm(x):
    m = jnp.mean(x, axis=-1, keepdims=True)
    c = x - m
    v = jnp.mean(c * c, axis=-1, keepdims=True)
    return c * lax.rsqrt(v + 1e-05)


def _dot(a, b):
    return jnp.dot(a, b, preferred_element_type=_F32)


def _dot_nt(a, b):
    return lax.dot_general(a, b, _NT, preferred_element_type=_F32)


def _masks(n_mem, seg, n_seq, first_layer):
    rows = 2 * n_mem + n_seq * seg

    def describe(axis):
        i = lax.broadcasted_iota(jnp.int32, (rows, rows), axis)
        is_mem = i < 2 * n_mem
        t = i - 2 * n_mem
        second = t >= seg
        layer = jnp.where(is_mem, jnp.where(i >= n_mem, 1, 0),
                          jnp.where(second, first_layer + 1, first_layer))
        pos = jnp.where(is_mem, -1, jnp.where(second, t - seg, t))
        return layer, pos

    lr, pr = describe(0)
    lc, pc = describe(1)
    same = lr == lc
    keep = same & ((pr < 0) | (pr >= pc))
    fill = jnp.where(same, _MASKED, -jnp.inf).astype(_F32)
    return keep, fill


def _attention(h, keep, fill, wq, wk, wv, wo_t, n_heads, dh):
    scale = dh ** -0.5
    width = _GROUP * dh
    n_groups = n_heads // _GROUP

    def project(g):
        cols = slice(g * width, (g + 1) * width)
        return tuple(_dot(h, w[:, cols]).astype(_BF16) for w in (wq, wk, wv))

    def attend(qkv):
        q, k, v = qkv
        outs = []
        for i in range(_GROUP):
            cols = slice(i * dh, (i + 1) * dh)
            s = jnp.where(keep, _dot_nt(q[:, cols], k[:, cols]) * scale, fill)
            e = jnp.exp(s - jnp.max(s, axis=-1, keepdims=True))
            inv = 1.0 / jnp.sum(e, axis=-1, keepdims=True)
            outs.append((_dot(e.astype(_BF16), v[:, cols]) * inv).astype(_BF16))
        return jnp.concatenate(outs, axis=1)

    qkv, o, acc = {}, {}, None
    for step in range(n_groups + 2):
        if step < n_groups:
            qkv[step] = project(step)
        if 0 <= step - 1 < n_groups:
            o[step - 1] = attend(qkv.pop(step - 1))
        if step - 2 >= 0:
            g = step - 2
            part = _dot_nt(o.pop(g), wo_t[:, g * width:(g + 1) * width])
            acc = part if acc is None else acc + part
    return acc


def _ffn_t(xn, w1, w3, w2_t):
    acc = None
    for c in range(w1.shape[1] // _FCHUNK):
        cols = slice(c * _FCHUNK, (c + 1) * _FCHUNK)
        gate = _dot(xn, w1[:, cols])
        up = _dot(xn, w3[:, cols])
        hid = (gate * jax.nn.sigmoid(gate) * up).astype(_BF16)
        part = _dot_nt(w2_t[:, cols], hid)
        acc = part if acc is None else acc + part
    return acc


def _load_weights(wq_hbm, wk_hbm, wv_hbm, wo_hbm, stage, wq, wk, wv, wo_t, wsem, osem):
    d_model, n_heads, dh = wq_hbm.shape
    per_weight = d_model // _WCHUNK
    jobs = [(src, dst, c) for src, dst in ((wq_hbm, wq), (wk_hbm, wk), (wv_hbm, wv))
            for c in range(per_weight)]
    slots = stage.shape[0]

    def copy(i):
        src, _, c = jobs[i]
        return pltpu.make_async_copy(src.at[pl.ds(c * _WCHUNK, _WCHUNK)],
                                     stage.at[i % slots], wsem.at[i % slots])

    def out_copy(head):
        return pltpu.make_async_copy(wo_hbm.at[head], wo_t.at[:, pl.ds(head * dh, dh)], osem)

    for i in range(_INFLIGHT):
        copy(i).start()
    for i, (_, dst, c) in enumerate(jobs):
        copy(i).wait()
        if i + _INFLIGHT < len(jobs):
            copy(i + _INFLIGHT).start()
        if i + _INFLIGHT == len(jobs):
            for head in range(n_heads):
                out_copy(head).start()

        def unpack(j, carry, i=i, dst=dst, c=c):
            r = pl.multiple_of(j * 16, 16)
            words = pltpu.bitcast(stage[i % slots, pl.ds(r, 16)], jnp.uint32)
            words = jnp.swapaxes(words, 0, 1)
            rows = pl.ds(pl.multiple_of(c * _WCHUNK + r, 16), 16)
            for p in range(n_heads // 2):
                even = pltpu.bitcast(words[p] << 16, _F32)
                odd = pltpu.bitcast(words[p] & jnp.uint32(0xFFFF0000), _F32)
                dst[rows, 2 * p * dh:(2 * p + 1) * dh] = even.astype(_BF16)
                dst[rows, (2 * p + 1) * dh:(2 * p + 2) * dh] = odd.astype(_BF16)
            return carry

        lax.fori_loop(0, _WCHUNK // 16, unpack, 0)
    for head in range(n_heads):
        out_copy(head).wait()


def _kernel(x_ref, mem0_ref, wq_hbm, wk_hbm, wv_hbm, wo_hbm, w1_hbm, w3_hbm, w2_hbm,
            out_ref,
            stage, wq, wk, wv, wo_t, w1, w3, w2_t, res, normed, mem, wsem, osem, fsem,
            *, seg):
    b = pl.program_id(0)
    n_blocks = pl.num_programs(0) - 1
    _, n_heads, dh = wq_hbm.shape
    n_mem = mem0_ref.shape[0]
    steps = _TOK // seg
    ffn_copies = [pltpu.make_async_copy(s, d, fsem.at[i])
                  for i, (s, d) in enumerate(((w1_hbm, w1), (w3_hbm, w3), (w2_hbm, w2_t)))]

    @pl.when(b == 0)
    def _():
        _load_weights(wq_hbm, wk_hbm, wv_hbm, wo_hbm, stage, wq, wk, wv, wo_t, wsem, osem)
        for c in ffn_copies:
            c.start()
        mem[0:n_mem] = mem0_ref[...].astype(_F32)

    @pl.when(b <= 1)
    def _():
        mem[n_mem:2 * n_mem] = mem0_ref[...].astype(_F32)

    @pl.when(b < n_blocks)
    def _():
        x = x_ref[...].astype(_F32).T
        res[0] = x
        normed[0] = _layernorm(x).astype(_BF16)

    def run_attention(first, n_seq):
        keep, fill = _masks(n_mem, seg, n_seq, first)

        def step(j, carry):
            rows = pl.ds(pl.multiple_of(j * seg, seg), seg)
            h = jnp.concatenate([mem[...].astype(_BF16)]
                                + [normed[first + i, rows] for i in range(n_seq)], axis=0)
            out = _attention(h, keep, fill, wq, wk, wv, wo_t, n_heads, dh)
            mem[...] = out[:2 * n_mem]
            for i in range(n_seq):
                lo = 2 * n_mem + i * seg
                res[first + i, rows] += out[lo:lo + seg]
            return carry

        lax.fori_loop(0, steps, step, 0)

    both = jnp.logical_and(b > 0, b < n_blocks)

    @pl.when(both)
    def _():
        run_attention(0, 2)

    @pl.when(jnp.logical_not(both))
    def _():
        run_attention(jnp.where(b == 0, 0, 1), 1)

    @pl.when(b == 0)
    def _():
        for c in ffn_copies:
            c.wait()

    def ffn(i, carry):
        slot = 1 - i
        x = res[slot]
        y = x + _ffn_t(_layernorm(x).astype(_BF16), w1, w3, w2_t).T

        @pl.when(slot == 1)
        def _():
            out_ref[...] = y.T.astype(out_ref.dtype)

        @pl.when(slot == 0)
        def _():
            res[1] = y
            normed[1] = _layernorm(y).astype(_BF16)

        return carry

    lax.fori_loop(jnp.where(b == 0, 1, 0), jnp.where(b == n_blocks, 1, 2), ffn, 0)


@functools.partial(jax.jit, static_argnames=("A_seg_len",))
def pallas_interleave_layers__memory_aug_recurrent_mem_tr__glu_gated_swiglu__prompt_kernel(
    A_x: jax.Array,
    A_mem0: jax.Array,
    A_Wq: jax.Array,
    A_Wk: jax.Array,
    A_Wv: jax.Array,
    A_Wo: jax.Array,
    A_seg_len: int,
    B_x: jax.Array,
    B_w1: jax.Array,
    B_w3: jax.Array,
    B_w2: jax.Array,
):
    del B_x
    batch, seq, d_model = A_x.shape
    n_mem = A_mem0.shape[1]
    _, n_heads, dh = A_Wq.shape
    d_ff = B_w1.shape[1]
    seg = int(A_seg_len)
    assert batch == 1 and seq % _TOK == 0 and _TOK % seg == 0 and seg % 16 == 0
    assert n_mem == 8 and n_heads % _GROUP == 0 and d_ff % _FCHUNK == 0
    assert d_model % _WCHUNK == 0
    n_blocks = seq // _TOK

    hbm = pl.BlockSpec(memory_space=pl.ANY)
    out_t = pl.pallas_call(
        functools.partial(_kernel, seg=seg),
        grid=(n_blocks + 1,),
        in_specs=[
            pl.BlockSpec((d_model, _TOK), lambda b: (0, jnp.minimum(b, n_blocks - 1))),
            pl.BlockSpec((n_mem, d_model), lambda b: (0, 0)),
            hbm, hbm, hbm, hbm, hbm, hbm, hbm,
        ],
        out_specs=pl.BlockSpec((d_model, _TOK), lambda b: (0, jnp.maximum(b - 1, 0))),
        out_shape=jax.ShapeDtypeStruct((d_model, seq), A_x.dtype),
        scratch_shapes=[
            pltpu.VMEM((_INFLIGHT + 1, _WCHUNK, n_heads, dh), _BF16),
            pltpu.VMEM((d_model, n_heads * dh), _BF16),
            pltpu.VMEM((d_model, n_heads * dh), _BF16),
            pltpu.VMEM((d_model, n_heads * dh), _BF16),
            pltpu.VMEM((d_model, n_heads * dh), _BF16),
            pltpu.VMEM((d_model, d_ff), _BF16),
            pltpu.VMEM((d_model, d_ff), _BF16),
            pltpu.VMEM((d_model, d_ff), _BF16),
            pltpu.VMEM((2, _TOK, d_model), _F32),
            pltpu.VMEM((2, _TOK, d_model), _BF16),
            pltpu.VMEM((2 * n_mem, d_model), _F32),
            pltpu.SemaphoreType.DMA((_INFLIGHT + 1,)),
            pltpu.SemaphoreType.DMA(()),
            pltpu.SemaphoreType.DMA((3,)),
        ],
        compiler_params=pltpu.CompilerParams(
            dimension_semantics=("arbitrary",),
            vmem_limit_bytes=100 * 1024 * 1024,
        ),
    )(A_x[0].T, A_mem0[0], A_Wq, A_Wk, A_Wv, jnp.transpose(A_Wo, (0, 2, 1)),
      B_w1, B_w3, B_w2.T)
    return out_t.T[None]
```

```python
import functools

import jax
import jax.numpy as jnp
import numpy as np
from jax import lax
import jax.experimental.pallas as pl
import jax.experimental.pallas.tpu as pltpu

_BF16 = jnp.bfloat16
_F32 = jnp.float32
_NT = (((1,), (1,)), ((), ()))
_TOK = 128
_GROUP = 4
_FCHUNK = 512
_WCHUNK = 64
_INFLIGHT = 3
_MASKED = -1000000000.0


def _layernorm(x):
    m = jnp.mean(x, axis=-1, keepdims=True)
    c = x - m
    v = jnp.mean(c * c, axis=-1, keepdims=True)
    return c * lax.rsqrt(v + 1e-05)


def _dot(a, b):
    return jnp.dot(a, b, preferred_element_type=_F32)


def _dot_nt(a, b):
    return lax.dot_general(a, b, _NT, preferred_element_type=_F32)


def _masks(n_mem, seg, n_seq, first_layer):
    rows = 2 * n_mem + n_seq * seg

    def describe(axis):
        i = lax.broadcasted_iota(jnp.int32, (rows, rows), axis)
        is_mem = i < 2 * n_mem
        t = i - 2 * n_mem
        second = t >= seg
        layer = jnp.where(is_mem, jnp.where(i >= n_mem, 1, 0),
                          jnp.where(second, first_layer + 1, first_layer))
        pos = jnp.where(is_mem, -1, jnp.where(second, t - seg, t))
        return layer, pos

    lr, pr = describe(0)
    lc, pc = describe(1)
    same = lr == lc
    keep = same & ((pr < 0) | (pr >= pc))
    fill = jnp.where(same, _MASKED, -jnp.inf).astype(_F32)
    return keep, fill


def _attention(h, keep, fill, wq, wk, wv, wo_t, n_heads, dh):
    scale = dh ** -0.5
    width = _GROUP * dh
    n_groups = n_heads // _GROUP
    heads = [slice(i * dh, (i + 1) * dh) for i in range(_GROUP)]

    def project(w, g):
        return _dot(h, w[:, g * width:(g + 1) * width]).astype(_BF16)

    def weights(q, k):
        out = []
        for cols in heads:
            s = jnp.where(keep, _dot_nt(q[:, cols], k[:, cols]) * scale, fill)
            e = jnp.exp(s - jnp.max(s, axis=-1, keepdims=True))
            out.append((e.astype(_BF16), 1.0 / jnp.sum(e, axis=-1, keepdims=True)))
        return out

    def mix(p, v):
        return jnp.concatenate(
            [(_dot(e, v[:, cols]) * inv).astype(_BF16) for (e, inv), cols in zip(p, heads)],
            axis=1)

    p, v, o, acc = {}, {}, {}, None
    for g in range(n_groups + 2):
        if g < n_groups:
            q = project(wq, g)
        if 0 <= g - 1 < n_groups:
            o[g - 1] = mix(p.pop(g - 1), v.pop(g - 1))
        if g < n_groups:
            k = project(wk, g)
            v[g] = project(wv, g)
            p[g] = weights(q, k)
        if g - 2 >= 0:
            part = _dot_nt(o.pop(g - 2), wo_t[:, (g - 2) * width:(g - 1) * width])
            acc = part if acc is None else acc + part
    return acc


def _ffn_t(xn, w1, w3, w2_t):
    n_chunks = w1.shape[1] // _FCHUNK
    hid, acc = {}, None
    for c in range(n_chunks + 1):
        if c < n_chunks:
            cols = slice(c * _FCHUNK, (c + 1) * _FCHUNK)
            gate = _dot(xn, w1[:, cols])
            up = _dot(xn, w3[:, cols])
            hid[c] = (gate * jax.nn.sigmoid(gate) * up).astype(_BF16)
        if c >= 1:
            part = _dot_nt(w2_t[:, (c - 1) * _FCHUNK:c * _FCHUNK], hid.pop(c - 1))
            acc = part if acc is None else acc + part
    return acc


def _load_weights(wq_hbm, wk_hbm, wv_hbm, wo_hbm, stage, wq, wk, wv, wo_t, wsem, osem):
    d_model, n_heads, dh = wq_hbm.shape
    per_weight = d_model // _WCHUNK
    jobs = [(src, dst, c) for src, dst in ((wq_hbm, wq), (wk_hbm, wk), (wv_hbm, wv))
            for c in range(per_weight)]
    slots = stage.shape[0]

    def copy(i):
        src, _, c = jobs[i]
        return pltpu.make_async_copy(src.at[pl.ds(c * _WCHUNK, _WCHUNK)],
                                     stage.at[i % slots], wsem.at[i % slots])

    def out_copy(head):
        return pltpu.make_async_copy(wo_hbm.at[head], wo_t.at[:, pl.ds(head * dh, dh)], osem)

    for i in range(_INFLIGHT):
        copy(i).start()
    for i, (_, dst, c) in enumerate(jobs):
        copy(i).wait()
        if i + _INFLIGHT < len(jobs):
            copy(i + _INFLIGHT).start()
        if i + _INFLIGHT == len(jobs):
            for head in range(n_heads):
                out_copy(head).start()

        def unpack(j, carry, i=i, dst=dst, c=c):
            r = pl.multiple_of(j * 16, 16)
            words = pltpu.bitcast(stage[i % slots, pl.ds(r, 16)], jnp.uint32)
            words = jnp.swapaxes(words, 0, 1)
            rows = pl.ds(pl.multiple_of(c * _WCHUNK + r, 16), 16)
            for p in range(n_heads // 2):
                even = pltpu.bitcast(words[p] << 16, _F32)
                odd = pltpu.bitcast(words[p] & jnp.uint32(0xFFFF0000), _F32)
                dst[rows, 2 * p * dh:(2 * p + 1) * dh] = even.astype(_BF16)
                dst[rows, (2 * p + 1) * dh:(2 * p + 2) * dh] = odd.astype(_BF16)
            return carry

        lax.fori_loop(0, _WCHUNK // 16, unpack, 0)
    for head in range(n_heads):
        out_copy(head).wait()


def _kernel(x_ref, mem0_ref, wq_hbm, wk_hbm, wv_hbm, wo_hbm, w1_hbm, w3_hbm, w2_hbm,
            out_ref,
            stage, wq, wk, wv, wo_t, w1, w3, w2_t, res, normed, mem, wsem, osem, fsem,
            *, seg):
    b = pl.program_id(0)
    n_blocks = pl.num_programs(0) - 1
    _, n_heads, dh = wq_hbm.shape
    n_mem = mem0_ref.shape[0]
    steps = _TOK // seg
    ffn_copies = [pltpu.make_async_copy(s, d, fsem.at[i])
                  for i, (s, d) in enumerate(((w1_hbm, w1), (w3_hbm, w3), (w2_hbm, w2_t)))]

    @pl.when(b == 0)
    def _():
        _load_weights(wq_hbm, wk_hbm, wv_hbm, wo_hbm, stage, wq, wk, wv, wo_t, wsem, osem)
        for c in ffn_copies:
            c.start()
        mem[0:n_mem] = mem0_ref[...].astype(_F32)

    @pl.when(b <= 1)
    def _():
        mem[n_mem:2 * n_mem] = mem0_ref[...].astype(_F32)

    @pl.when(b < n_blocks)
    def _():
        x = x_ref[...].astype(_F32).T
        res[0] = x
        normed[0] = _layernorm(x).astype(_BF16)

    def run_attention(first, n_seq):
        keep, fill = _masks(n_mem, seg, n_seq, first)

        def step(j, carry):
            rows = pl.ds(pl.multiple_of(j * seg, seg), seg)
            h = jnp.concatenate([mem[...].astype(_BF16)]
                                + [normed[first + i, rows] for i in range(n_seq)], axis=0)
            out = _attention(h, keep, fill, wq, wk, wv, wo_t, n_heads, dh)
            mem[...] = out[:2 * n_mem]
            for i in range(n_seq):
                lo = 2 * n_mem + i * seg
                res[first + i, rows] += out[lo:lo + seg]
            return carry

        lax.fori_loop(0, steps, step, 0)

    both = jnp.logical_and(b > 0, b < n_blocks)

    @pl.when(both)
    def _():
        run_attention(0, 2)

    @pl.when(jnp.logical_not(both))
    def _():
        run_attention(jnp.where(b == 0, 0, 1), 1)

    @pl.when(b == 0)
    def _():
        for c in ffn_copies:
            c.wait()

    def ffn(i, carry):
        slot = 1 - i
        x = res[slot]
        y = x + _ffn_t(_layernorm(x).astype(_BF16), w1, w3, w2_t).T

        @pl.when(slot == 1)
        def _():
            out_ref[...] = y.T.astype(out_ref.dtype)

        @pl.when(slot == 0)
        def _():
            res[1] = y
            normed[1] = _layernorm(y).astype(_BF16)

        return carry

    lax.fori_loop(jnp.where(b == 0, 1, 0), jnp.where(b == n_blocks, 1, 2), ffn, 0)


@functools.partial(jax.jit, static_argnames=("A_seg_len",))
def pallas_interleave_layers__memory_aug_recurrent_mem_tr__glu_gated_swiglu__prompt_kernel(
    A_x: jax.Array,
    A_mem0: jax.Array,
    A_Wq: jax.Array,
    A_Wk: jax.Array,
    A_Wv: jax.Array,
    A_Wo: jax.Array,
    A_seg_len: int,
    B_x: jax.Array,
    B_w1: jax.Array,
    B_w3: jax.Array,
    B_w2: jax.Array,
):
    del B_x
    batch, seq, d_model = A_x.shape
    n_mem = A_mem0.shape[1]
    _, n_heads, dh = A_Wq.shape
    d_ff = B_w1.shape[1]
    seg = int(A_seg_len)
    assert batch == 1 and seq % _TOK == 0 and _TOK % seg == 0 and seg % 16 == 0
    assert n_mem == 8 and n_heads % _GROUP == 0 and d_ff % _FCHUNK == 0
    assert d_model % _WCHUNK == 0
    n_blocks = seq // _TOK

    hbm = pl.BlockSpec(memory_space=pl.ANY)
    out_t = pl.pallas_call(
        functools.partial(_kernel, seg=seg),
        grid=(n_blocks + 1,),
        in_specs=[
            pl.BlockSpec((d_model, _TOK), lambda b: (0, jnp.minimum(b, n_blocks - 1))),
            pl.BlockSpec((n_mem, d_model), lambda b: (0, 0)),
            hbm, hbm, hbm, hbm, hbm, hbm, hbm,
        ],
        out_specs=pl.BlockSpec((d_model, _TOK), lambda b: (0, jnp.maximum(b - 1, 0))),
        out_shape=jax.ShapeDtypeStruct((d_model, seq), A_x.dtype),
        scratch_shapes=[
            pltpu.VMEM((_INFLIGHT + 1, _WCHUNK, n_heads, dh), _BF16),
            pltpu.VMEM((d_model, n_heads * dh), _BF16),
            pltpu.VMEM((d_model, n_heads * dh), _BF16),
            pltpu.VMEM((d_model, n_heads * dh), _BF16),
            pltpu.VMEM((d_model, n_heads * dh), _BF16),
            pltpu.VMEM((d_model, d_ff), _BF16),
            pltpu.VMEM((d_model, d_ff), _BF16),
            pltpu.VMEM((d_model, d_ff), _BF16),
            pltpu.VMEM((2, _TOK, d_model), _F32),
            pltpu.VMEM((2, _TOK, d_model), _BF16),
            pltpu.VMEM((2 * n_mem, d_model), _F32),
            pltpu.SemaphoreType.DMA((_INFLIGHT + 1,)),
            pltpu.SemaphoreType.DMA(()),
            pltpu.SemaphoreType.DMA((3,)),
        ],
        compiler_params=pltpu.CompilerParams(
            dimension_semantics=("arbitrary",),
            vmem_limit_bytes=100 * 1024 * 1024,
        ),
    )(A_x[0].T, A_mem0[0], A_Wq, A_Wk, A_Wv, jnp.transpose(A_Wo, (0, 2, 1)),
      B_w1, B_w3, B_w2.T)
    return out_t.T[None]
```

```python
import functools

import jax
import jax.numpy as jnp
import numpy as np
from jax import lax
import jax.experimental.pallas as pl
import jax.experimental.pallas.tpu as pltpu

_BF16 = jnp.bfloat16
_F32 = jnp.float32
_NT = (((1,), (1,)), ((), ()))
_TOK = 128
_GROUP = 4
_FCHUNK = 512
_WCHUNK = 64
_INFLIGHT = 3
_UNROLL = 1
_EDGE_CHUNKS = 3
_MASKED = -1000000000.0


def _layernorm(x):
    m = jnp.mean(x, axis=-1, keepdims=True)
    c = x - m
    v = jnp.mean(c * c, axis=-1, keepdims=True)
    return c * lax.rsqrt(v + 1e-05)


def _dot(a, b):
    return jnp.dot(a, b, preferred_element_type=_F32)


def _dot_nt(a, b):
    return lax.dot_general(a, b, _NT, preferred_element_type=_F32)


def _masks(n_mem, seg, n_seq, first_layer):
    rows = 2 * n_mem + n_seq * seg

    def describe(axis):
        i = lax.broadcasted_iota(jnp.int32, (rows, rows), axis)
        is_mem = i < 2 * n_mem
        t = i - 2 * n_mem
        second = t >= seg
        layer = jnp.where(is_mem, jnp.where(i >= n_mem, 1, 0),
                          jnp.where(second, first_layer + 1, first_layer))
        pos = jnp.where(is_mem, -1, jnp.where(second, t - seg, t))
        return layer, pos

    lr, pr = describe(0)
    lc, pc = describe(1)
    same = lr == lc
    keep = same & ((pr < 0) | (pr >= pc))
    fill = jnp.where(same, _MASKED, -jnp.inf).astype(_F32)
    return keep, fill


def _attention(h, keep, fill, wq, wk, wv, wo_t, n_heads, dh):
    scale = dh ** -0.5
    width = _GROUP * dh
    n_groups = n_heads // _GROUP
    heads = [slice(i * dh, (i + 1) * dh) for i in range(_GROUP)]

    def project(w, g):
        return _dot(h, w[:, g * width:(g + 1) * width]).astype(_BF16)

    def weights(q, k):
        out = []
        for cols in heads:
            s = jnp.where(keep, _dot_nt(q[:, cols], k[:, cols]) * scale, fill)
            e = jnp.exp(s - jnp.max(s, axis=-1, keepdims=True))
            out.append((e.astype(_BF16), 1.0 / jnp.sum(e, axis=-1, keepdims=True)))
        return out

    def mix(p, v):
        return jnp.concatenate(
            [(_dot(e, v[:, cols]) * inv).astype(_BF16) for (e, inv), cols in zip(p, heads)],
            axis=1)

    p, v, o, acc = {}, {}, {}, None
    for g in range(n_groups + 2):
        if g < n_groups:
            q = project(wq, g)
        if 0 <= g - 1 < n_groups:
            o[g - 1] = mix(p.pop(g - 1), v.pop(g - 1))
        if g < n_groups:
            k = project(wk, g)
            v[g] = project(wv, g)
            p[g] = weights(q, k)
        if g - 2 >= 0:
            part = _dot_nt(o.pop(g - 2), wo_t[:, (g - 2) * width:(g - 1) * width])
            acc = part if acc is None else acc + part
    return acc


def _hidden(xn, w1, w3, cols):
    gate = _dot(xn, w1[:, cols])
    up = _dot(xn, w3[:, cols])
    return (gate * jax.nn.sigmoid(gate) * up).astype(_BF16)


def _swiglu_t(inputs, w1, w3, w2_t, chunks):
    jobs = [(i, cols) for i in range(len(inputs)) for cols in chunks]
    acc = [None] * len(inputs)
    hid = None
    for n in range(len(jobs) + 1):
        prev = hid
        if n < len(jobs):
            i, cols = jobs[n]
            hid = _hidden(inputs[i], w1, w3, cols)
        if n >= 1:
            i, cols = jobs[n - 1]
            part = _dot_nt(w2_t[:, cols], prev)
            acc[i] = part if acc[i] is None else acc[i] + part
    return acc


def _load_weights(wq_hbm, wk_hbm, wv_hbm, wo_hbm, stage, wq, wk, wv, wo_t, wsem, osem):
    d_model, n_heads, dh = wq_hbm.shape
    per_weight = d_model // _WCHUNK
    jobs = [(src, dst, c) for src, dst in ((wq_hbm, wq), (wk_hbm, wk), (wv_hbm, wv))
            for c in range(per_weight)]
    slots = stage.shape[0]

    def copy(i):
        src, _, c = jobs[i]
        return pltpu.make_async_copy(src.at[pl.ds(c * _WCHUNK, _WCHUNK)],
                                     stage.at[i % slots], wsem.at[i % slots])

    def out_copy(head):
        return pltpu.make_async_copy(wo_hbm.at[head], wo_t.at[:, pl.ds(head * dh, dh)], osem)

    for i in range(_INFLIGHT):
        copy(i).start()
    for i, (_, dst, c) in enumerate(jobs):
        copy(i).wait()
        if i + _INFLIGHT < len(jobs):
            copy(i + _INFLIGHT).start()
        if i + _INFLIGHT == len(jobs):
            for head in range(n_heads):
                out_copy(head).start()

        def unpack(j, carry, i=i, dst=dst, c=c):
            r = pl.multiple_of(j * 16, 16)
            words = pltpu.bitcast(stage[i % slots, pl.ds(r, 16)], jnp.uint32)
            words = jnp.swapaxes(words, 0, 1)
            rows = pl.ds(pl.multiple_of(c * _WCHUNK + r, 16), 16)
            for p in range(n_heads // 2):
                even = pltpu.bitcast(words[p] << 16, _F32)
                odd = pltpu.bitcast(words[p] & jnp.uint32(0xFFFF0000), _F32)
                dst[rows, 2 * p * dh:(2 * p + 1) * dh] = even.astype(_BF16)
                dst[rows, (2 * p + 1) * dh:(2 * p + 2) * dh] = odd.astype(_BF16)
            return carry

        lax.fori_loop(0, _WCHUNK // 16, unpack, 0)
    for head in range(n_heads):
        out_copy(head).wait()


def _kernel(x0_ref, x_next_ref, mem0_ref, wq_hbm, wk_hbm, wv_hbm, wo_hbm, w1_hbm, w3_hbm,
            w2_hbm, out_ref,
            stage, wq, wk, wv, wo_t, w1, w3, w2_t, res, normed, mem, acc_t, wsem, osem, fsem,
            *, seg):
    b = pl.program_id(0)
    n_blocks = pl.num_programs(0) - 1
    _, n_heads, dh = wq_hbm.shape
    n_mem = mem0_ref.shape[0]
    n_chunks = w1.shape[1] // _FCHUNK
    steps = _TOK // seg
    ffn_copies = [pltpu.make_async_copy(s, d, fsem.at[i])
                  for i, (s, d) in enumerate(((w1_hbm, w1), (w3_hbm, w3), (w2_hbm, w2_t)))]

    def start_layer(slot, x):
        res[slot] = x
        normed[slot] = _layernorm(x).astype(_BF16)

    @pl.when(b == 0)
    def _():
        _load_weights(wq_hbm, wk_hbm, wv_hbm, wo_hbm, stage, wq, wk, wv, wo_t, wsem, osem)
        for c in ffn_copies:
            c.start()
        mem[0:n_mem] = mem0_ref[...].astype(_F32)
        start_layer(0, x0_ref[...].astype(_F32).T)

    @pl.when(b <= 1)
    def _():
        mem[n_mem:2 * n_mem] = mem0_ref[...].astype(_F32)

    def run_attention(first, n_seq, unroll):
        keep, fill = _masks(n_mem, seg, n_seq, first)

        def segment(j):
            rows = pl.ds(pl.multiple_of(j * seg, seg), seg)
            h = jnp.concatenate([mem[...].astype(_BF16)]
                                + [normed[first + i, rows] for i in range(n_seq)], axis=0)
            out = _attention(h, keep, fill, wq, wk, wv, wo_t, n_heads, dh)
            mem[...] = out[:2 * n_mem]
            for i in range(n_seq):
                lo = 2 * n_mem + i * seg
                res[first + i, rows] += out[lo:lo + seg]

        def step(j, carry):
            for u in range(unroll):
                segment(j * unroll + u)
            return carry

        lax.fori_loop(0, steps // unroll, step, 0)

    both = jnp.logical_and(b > 0, b < n_blocks)

    @pl.when(both)
    def _():
        run_attention(0, 2, _UNROLL)
        x1, x3 = res[0], res[1]
        chunks = [slice(c * _FCHUNK, (c + 1) * _FCHUNK) for c in range(n_chunks)]
        f2, f4 = _swiglu_t([_layernorm(x1).astype(_BF16), _layernorm(x3).astype(_BF16)],
                           w1, w3, w2_t, chunks)
        start_layer(1, x1 + f2.T)
        start_layer(0, x_next_ref[...].astype(_F32).T)
        out_ref[...] = (x3.T + f4).astype(out_ref.dtype)

    @pl.when(jnp.logical_not(both))
    def _():
        slot = jnp.where(b == 0, 0, 1)
        run_attention(slot, 1, 1)

        @pl.when(b == 0)
        def _():
            for c in ffn_copies:
                c.wait()

        x = res[slot]
        xn = _layernorm(x).astype(_BF16)
        acc_t[...] = x.T

        def part(i, carry):
            chunks = [pl.ds(pl.multiple_of((i * _EDGE_CHUNKS + c) * _FCHUNK, _FCHUNK), _FCHUNK)
                      for c in range(_EDGE_CHUNKS)]
            acc_t[...] += _swiglu_t([xn], w1, w3, w2_t, chunks)[0]
            return carry

        lax.fori_loop(0, n_chunks // _EDGE_CHUNKS, part, 0)

        @pl.when(b == 0)
        def _():
            start_layer(1, acc_t[...].T)
            start_layer(0, x_next_ref[...].astype(_F32).T)

        @pl.when(b > 0)
        def _():
            out_ref[...] = acc_t[...].astype(out_ref.dtype)


@functools.partial(jax.jit, static_argnames=("A_seg_len",))
def pallas_interleave_layers__memory_aug_recurrent_mem_tr__glu_gated_swiglu__prompt_kernel(
    A_x: jax.Array,
    A_mem0: jax.Array,
    A_Wq: jax.Array,
    A_Wk: jax.Array,
    A_Wv: jax.Array,
    A_Wo: jax.Array,
    A_seg_len: int,
    B_x: jax.Array,
    B_w1: jax.Array,
    B_w3: jax.Array,
    B_w2: jax.Array,
):
    del B_x
    batch, seq, d_model = A_x.shape
    n_mem = A_mem0.shape[1]
    _, n_heads, dh = A_Wq.shape
    d_ff = B_w1.shape[1]
    seg = int(A_seg_len)
    assert batch == 1 and seq % _TOK == 0 and _TOK % seg == 0 and seg % 16 == 0
    assert n_mem == 8 and n_heads % _GROUP == 0 and d_ff % (_FCHUNK * _EDGE_CHUNKS) == 0
    assert d_model % _WCHUNK == 0
    n_blocks = seq // _TOK

    x_t = A_x[0].T
    hbm = pl.BlockSpec(memory_space=pl.ANY)
    out_t = pl.pallas_call(
        functools.partial(_kernel, seg=seg),
        grid=(n_blocks + 1,),
        in_specs=[
            pl.BlockSpec((d_model, _TOK), lambda b: (0, 0)),
            pl.BlockSpec((d_model, _TOK), lambda b: (0, jnp.minimum(b + 1, n_blocks - 1))),
            pl.BlockSpec((n_mem, d_model), lambda b: (0, 0)),
            hbm, hbm, hbm, hbm, hbm, hbm, hbm,
        ],
        out_specs=pl.BlockSpec((d_model, _TOK), lambda b: (0, jnp.maximum(b - 1, 0))),
        out_shape=jax.ShapeDtypeStruct((d_model, seq), A_x.dtype),
        scratch_shapes=[
            pltpu.VMEM((_INFLIGHT + 1, _WCHUNK, n_heads, dh), _BF16),
            pltpu.VMEM((d_model, n_heads * dh), _BF16),
            pltpu.VMEM((d_model, n_heads * dh), _BF16),
            pltpu.VMEM((d_model, n_heads * dh), _BF16),
            pltpu.VMEM((d_model, n_heads * dh), _BF16),
            pltpu.VMEM((d_model, d_ff), _BF16),
            pltpu.VMEM((d_model, d_ff), _BF16),
            pltpu.VMEM((d_model, d_ff), _BF16),
            pltpu.VMEM((2, _TOK, d_model), _F32),
            pltpu.VMEM((2, _TOK, d_model), _BF16),
            pltpu.VMEM((2 * n_mem, d_model), _F32),
            pltpu.VMEM((d_model, _TOK), _F32),
            pltpu.SemaphoreType.DMA((_INFLIGHT + 1,)),
            pltpu.SemaphoreType.DMA(()),
            pltpu.SemaphoreType.DMA((3,)),
        ],
        compiler_params=pltpu.CompilerParams(
            dimension_semantics=("arbitrary",),
            vmem_limit_bytes=100 * 1024 * 1024,
        ),
    )(x_t, x_t, A_mem0[0], A_Wq, A_Wk, A_Wv, jnp.transpose(A_Wo, (0, 2, 1)),
      B_w1, B_w3, B_w2.T)
    return out_t.T[None]
```

```python
import functools

import jax
import jax.numpy as jnp
import numpy as np
from jax import lax
import jax.experimental.pallas as pl
import jax.experimental.pallas.tpu as pltpu

_BF16 = jnp.bfloat16
_F32 = jnp.float32
_NT = (((1,), (1,)), ((), ()))
_TOK = 128
_GROUP = 4
_FCHUNK = 512
_WCHUNK = 64
_INFLIGHT = 3
_UNROLL = 1
_EDGE_CHUNKS = 3
_HALF = 256
_WO_FROM = 6
_MASKED = -1000000000.0


def _layernorm(x):
    m = jnp.mean(x, axis=-1, keepdims=True)
    c = x - m
    v = jnp.mean(c * c, axis=-1, keepdims=True)
    return c * lax.rsqrt(v + 1e-05)


def _dot(a, b):
    return lax.dot_general(a, b, (((1,), (0,)), ((), ())), preferred_element_type=_F32)


def _dot_nt(a, b):
    return lax.dot_general(a, b, _NT, preferred_element_type=_F32)


def _pack(x):
    return pltpu.bitcast(x.astype(_BF16), jnp.uint32)


def _unpack(words):
    return pltpu.bitcast(words, _BF16)


def _left_terms(a11, a12, a21, a22):
    if a21 is None:
        return [a11, None, a11, None, a11 + a12, None, a12]
    return [a11 + a22, a21 + a22, a11, a22, a11 + a12, a21 - a11, a12 - a22]


def _right_terms(b11, b12, b21, b22):
    return [b11 + b22, b11, b12 - b22, b21 - b11, b22, b11 + b12, b21 + b22]


def _combine(m):
    top = (m[0] - m[4] + m[6], m[2] + m[4])
    if m[1] is None:
        return [top]
    return [(top[0] + m[3], top[1]), (m[1] + m[3], m[0] - m[1] + m[2] + m[5])]


def _masks(n_mem, length, n_seq):
    rows = n_seq * length

    def describe(axis):
        i = lax.broadcasted_iota(jnp.int32, (rows, rows), axis)
        second = i >= length
        return jnp.where(second, 1, 0), jnp.where(second, i - length, i)

    (seq_r, idx_r), (seq_c, idx_c) = describe(0), describe(1)
    same = seq_r == seq_c
    keep = same & ((idx_r < n_mem) | (idx_r >= idx_c))
    fill = jnp.where(same, _MASKED, -jnp.inf).astype(_F32)
    return keep, fill


def _attention(hs, keep, fill, wq, wk, wv, wo, n_heads, dh):
    scale = dh ** -0.5
    width = _GROUP * dh
    half = width // 2
    n_groups = n_heads // _GROUP
    length = hs[0].shape[0]
    heads = [slice(i * dh, (i + 1) * dh) for i in range(_GROUP)]
    lhs_dtype = _BF16 if (len(hs) * length) % 16 == 0 else _F32

    def blocks(rows, size):
        out = [r[:, i * size:(i + 1) * size] for r in rows for i in range(2)]
        return out + [None] * (4 - len(out))

    h_terms = _left_terms(*blocks(hs, _HALF))
    h_rest = jnp.concatenate([h[:, 2 * _HALF:] for h in hs], axis=0).astype(lhs_dtype)

    def project(w, g):
        main, rest = w
        m = [None if t is None else _dot(t, _unpack(main[i, :, g * half:(g + 1) * half]))
             for i, t in enumerate(h_terms)]
        full = jnp.concatenate([jnp.concatenate(c, axis=1) for c in _combine(m)], axis=0)
        return full + _dot(h_rest, _unpack(rest[:, g * width:(g + 1) * width]))

    def weights(q, k):
        out = []
        for cols in heads:
            s = jnp.where(keep, _dot_nt(q[:, cols], k[:, cols]) * scale, fill)
            e = jnp.exp(s - jnp.max(s, axis=-1, keepdims=True))
            out.append((e.astype(lhs_dtype), 1.0 / jnp.sum(e, axis=-1, keepdims=True)))
        return out

    def mix(p, v):
        return jnp.concatenate(
            [_dot(e, v[:, cols]) * inv for (e, inv), cols in zip(p, heads)], axis=1)

    def output(o, g):
        main, rest = wo
        rows = [o[i * length:(i + 1) * length] for i in range(len(hs))]
        m = [None if t is None
             else _dot(t, _unpack(main[i, g * half // 2:(g + 1) * half // 2, :]))
             for i, t in enumerate(_left_terms(*blocks(rows, half)))]
        return m + [_dot(o.astype(lhs_dtype), _unpack(rest[g * half:(g + 1) * half, :]))]

    p, v, o, acc = {}, {}, {}, None
    for g in range(n_groups + 2):
        if g < n_groups:
            q = project(wq, g).astype(lhs_dtype)
        if 0 <= g - 1 < n_groups:
            o[g - 1] = mix(p.pop(g - 1), v.pop(g - 1))
        if g < n_groups:
            k = project(wk, g).astype(_BF16)
            v[g] = project(wv, g).astype(_BF16)
            p[g] = weights(q, k)
        if g - 2 >= 0:
            part = output(o.pop(g - 2), g - 2)
            acc = part if acc is None else [
                None if x is None else x + y for x, y in zip(acc, part)]
    return [jnp.concatenate([*c, acc[7][i * length:(i + 1) * length]], axis=1)
            for i, c in enumerate(_combine(acc))]


def _hidden(xn, w1, w3, cols):
    gate = _dot(xn, w1[:, cols])
    up = _dot(xn, w3[:, cols])
    return (gate * jax.nn.sigmoid(gate) * up).astype(_BF16)


def _swiglu_t(inputs, w1, w3, w2_t, chunks):
    jobs = [(i, cols) for i in range(len(inputs)) for cols in chunks]
    acc = [None] * len(inputs)
    hid = None
    for n in range(len(jobs) + 1):
        prev = hid
        if n < len(jobs):
            i, cols = jobs[n]
            hid = _hidden(inputs[i], w1, w3, cols)
        if n >= 1:
            i, cols = jobs[n - 1]
            part = _dot_nt(w2_t[:, cols], prev)
            acc[i] = part if acc[i] is None else acc[i] + part
    return acc


def _load_weights(sources, targets, wo_hbm, wo, stage, wo_stage, wsem, osem):
    _, n_heads, dh = sources[0].shape
    pairs = _GROUP // 2
    main_chunks = _HALF // _WCHUNK
    jobs = [(src, dst, c) for src, dst in zip(sources, targets) for c in range(main_chunks + 1)]
    slots = stage.shape[0]

    def copies(i):
        src, _, c = jobs[i]
        starts = [c * _WCHUNK, _HALF + c * _WCHUNK] if c < main_chunks else [2 * _HALF]
        return [pltpu.make_async_copy(src.at[pl.ds(r, _WCHUNK)], stage.at[i % slots, n],
                                      wsem.at[2 * (i % slots) + n])
                for n, r in enumerate(starts)]

    def head_pairs(slot, n, r):
        words = jnp.swapaxes(pltpu.bitcast(stage[slot, n, pl.ds(r, 16)], jnp.uint32), 0, 1)
        return [(pltpu.bitcast(words[p] << 16, _F32),
                 pltpu.bitcast(words[p] & jnp.uint32(0xFFFF0000), _F32))
                for p in range(n_heads // 2)]

    def output_pair(p, carry):
        even, odd = (wo_stage[2 * p + i, :2 * _HALF].T.astype(_F32) for i in range(2))
        terms = _right_terms(even[:, :_HALF], even[:, _HALF:], odd[:, :_HALF], odd[:, _HALF:])
        for i, t in enumerate(terms):
            wo[0][i, pl.ds(pl.multiple_of(p * (dh // 2), dh // 2), dh // 2), :] = _pack(t)
        for i in range(2):
            at = (p // pairs) * _GROUP + i * pairs + p % pairs
            wo[1][pl.ds(pl.multiple_of(at * (dh // 2), dh // 2), dh // 2), :] = _pack(
                wo_stage[2 * p + i, 2 * _HALF:].astype(_F32).T)
        return carry

    wo_copy = pltpu.make_async_copy(wo_hbm, wo_stage, osem)
    for i in range(_INFLIGHT):
        for c in copies(i):
            c.start()
    wo_copy.start()
    done = 0
    for i, (_, (main, rest), c) in enumerate(jobs):
        for copy in copies(i):
            copy.wait()
        if i + _INFLIGHT < len(jobs):
            for copy in copies(i + _INFLIGHT):
                copy.start()

        def main_rows(j, carry, slot=i % slots, main=main, c=c):
            r = pl.multiple_of(j * 16, 16)
            rows = pl.ds(pl.multiple_of(c * (_WCHUNK // 2) + j * 8, 8), 8)
            for p, (lo, hi) in enumerate(zip(head_pairs(slot, 0, r), head_pairs(slot, 1, r))):
                for n, t in enumerate(_right_terms(*lo, *hi)):
                    main[n, rows, p * dh:(p + 1) * dh] = _pack(t)
            return carry

        def rest_rows(j, carry, slot=i % slots, rest=rest):
            rows = pl.ds(pl.multiple_of(j * 8, 8), 8)
            for p, pair in enumerate(head_pairs(slot, 0, pl.multiple_of(j * 16, 16))):
                for n, t in enumerate(pair):
                    at = (p // pairs) * _GROUP + n * pairs + p % pairs
                    rest[rows, at * dh:(at + 1) * dh] = _pack(t)
            return carry

        lax.fori_loop(0, _WCHUNK // 16, main_rows if c < main_chunks else rest_rows, 0)
        if i == _WO_FROM:
            wo_copy.wait()
        if i >= _WO_FROM:
            upto = (n_heads // 2) * (i + 1 - _WO_FROM) // (len(jobs) - _WO_FROM)
            lax.fori_loop(done, upto, output_pair, 0)
            done = upto


def _kernel(x0_ref, x_next_ref, mem0_ref, wq_hbm, wk_hbm, wv_hbm, wo_hbm, w1_hbm, w3_hbm,
            w2_hbm, out_ref,
            stage, wo_stage, wq, wq_rest, wk, wk_rest, wv, wv_rest, wo, wo_rest,
            w1, w3, w2_t, res, normed, mem, acc_t, wsem, osem, fsem, *, seg):
    b = pl.program_id(0)
    n_blocks = pl.num_programs(0) - 1
    _, n_heads, dh = wq_hbm.shape
    n_mem = mem0_ref.shape[0]
    n_chunks = w1.shape[1] // _FCHUNK
    steps = _TOK // seg
    ffn_copies = [pltpu.make_async_copy(s, d, fsem.at[i])
                  for i, (s, d) in enumerate(((w1_hbm, w1), (w3_hbm, w3), (w2_hbm, w2_t)))]

    attn_weights = ((wq, wq_rest), (wk, wk_rest), (wv, wv_rest), (wo, wo_rest))

    def start_layer(slot, x):
        res[slot] = x
        normed[slot] = _layernorm(x)

    @pl.when(b == 0)
    def _():
        _load_weights((wq_hbm, wk_hbm, wv_hbm), attn_weights[:3], wo_hbm, attn_weights[3],
                      stage, wo_stage, wsem, osem)
        for c in ffn_copies:
            c.start()
        mem[0] = mem0_ref[...].astype(_F32)
        mem[1] = mem0_ref[...].astype(_F32)
        start_layer(0, x0_ref[...].astype(_F32).T)

    def run_attention(first, n_seq, unroll):
        keep, fill = _masks(n_mem, n_mem + seg, n_seq)

        def segment(j):
            rows = pl.ds(pl.multiple_of(j * seg, seg), seg)
            hs = [jnp.concatenate([mem[first + i], normed[first + i, rows]], axis=0)
                  for i in range(n_seq)]
            for i, out in enumerate(_attention(hs, keep, fill, *attn_weights, n_heads, dh)):
                mem[first + i] = out[:n_mem]
                res[first + i, rows] += out[n_mem:]

        def step(j, carry):
            for u in range(unroll):
                segment(j * unroll + u)
            return carry

        lax.fori_loop(0, steps // unroll, step, 0)

    both = jnp.logical_and(b > 0, b < n_blocks)

    @pl.when(both)
    def _():
        run_attention(0, 2, _UNROLL)
        x1, x3 = res[0], res[1]
        chunks = [slice(c * _FCHUNK, (c + 1) * _FCHUNK) for c in range(n_chunks)]
        f2, f4 = _swiglu_t([_layernorm(x1).astype(_BF16), _layernorm(x3).astype(_BF16)],
                           w1, w3, w2_t, chunks)
        start_layer(1, x1 + f2.T)
        start_layer(0, x_next_ref[...].astype(_F32).T)
        out_ref[...] = (x3.T + f4).astype(out_ref.dtype)

    @pl.when(jnp.logical_not(both))
    def _():
        slot = jnp.where(b == 0, 0, 1)
        run_attention(slot, 1, 1)

        @pl.when(b == 0)
        def _():
            for c in ffn_copies:
                c.wait()

        x = res[slot]
        xn = _layernorm(x).astype(_BF16)
        acc_t[...] = x.T

        def part(i, carry):
            chunks = [pl.ds(pl.multiple_of((i * _EDGE_CHUNKS + c) * _FCHUNK, _FCHUNK), _FCHUNK)
                      for c in range(_EDGE_CHUNKS)]
            acc_t[...] += _swiglu_t([xn], w1, w3, w2_t, chunks)[0]
            return carry

        lax.fori_loop(0, n_chunks // _EDGE_CHUNKS, part, 0)

        @pl.when(b == 0)
        def _():
            start_layer(1, acc_t[...].T)
            start_layer(0, x_next_ref[...].astype(_F32).T)

        @pl.when(b > 0)
        def _():
            out_ref[...] = acc_t[...].astype(out_ref.dtype)


@functools.partial(jax.jit, static_argnames=("A_seg_len",))
def pallas_interleave_layers__memory_aug_recurrent_mem_tr__glu_gated_swiglu__prompt_kernel(
    A_x: jax.Array,
    A_mem0: jax.Array,
    A_Wq: jax.Array,
    A_Wk: jax.Array,
    A_Wv: jax.Array,
    A_Wo: jax.Array,
    A_seg_len: int,
    B_x: jax.Array,
    B_w1: jax.Array,
    B_w3: jax.Array,
    B_w2: jax.Array,
):
    del B_x
    batch, seq, d_model = A_x.shape
    n_mem = A_mem0.shape[1]
    _, n_heads, dh = A_Wq.shape
    d_ff = B_w1.shape[1]
    seg = int(A_seg_len)
    assert batch == 1 and seq % _TOK == 0 and _TOK % seg == 0 and seg % 16 == 0
    assert n_mem == 8 and n_heads % _GROUP == 0 and d_ff % (_FCHUNK * _EDGE_CHUNKS) == 0
    d_rest = d_model - 2 * _HALF
    assert d_rest == _WCHUNK and _HALF % _WCHUNK == 0
    n_blocks = seq // _TOK

    x_t = A_x[0].T
    hbm = pl.BlockSpec(memory_space=pl.ANY)
    out_t = pl.pallas_call(
        functools.partial(_kernel, seg=seg),
        grid=(n_blocks + 1,),
        in_specs=[
            pl.BlockSpec((d_model, _TOK), lambda b: (0, 0)),
            pl.BlockSpec((d_model, _TOK), lambda b: (0, jnp.minimum(b + 1, n_blocks - 1))),
            pl.BlockSpec((n_mem, d_model), lambda b: (0, 0)),
            hbm, hbm, hbm, hbm, hbm, hbm, hbm,
        ],
        out_specs=pl.BlockSpec((d_model, _TOK), lambda b: (0, jnp.maximum(b - 1, 0))),
        out_shape=jax.ShapeDtypeStruct((d_model, seq), A_x.dtype),
        scratch_shapes=[
            pltpu.VMEM((_INFLIGHT + 1, 2, _WCHUNK, n_heads, dh), _BF16),
            pltpu.VMEM((n_heads, d_model, dh), _BF16),
            *3 * [pltpu.VMEM((7, _HALF // 2, n_heads * dh // 2), jnp.uint32),
                  pltpu.VMEM((d_rest // 2, n_heads * dh), jnp.uint32)],
            pltpu.VMEM((7, n_heads * dh // 4, _HALF), jnp.uint32),
            pltpu.VMEM((n_heads * dh // 2, d_rest), jnp.uint32),
            pltpu.VMEM((d_model, d_ff), _BF16),
            pltpu.VMEM((d_model, d_ff), _BF16),
            pltpu.VMEM((d_model, d_ff), _BF16),
            pltpu.VMEM((2, _TOK, d_model), _F32),
            pltpu.VMEM((2, _TOK, d_model), _F32),
            pltpu.VMEM((2, n_mem, d_model), _F32),
            pltpu.VMEM((d_model, _TOK), _F32),
            pltpu.SemaphoreType.DMA((2 * (_INFLIGHT + 1),)),
            pltpu.SemaphoreType.DMA(()),
            pltpu.SemaphoreType.DMA((3,)),
        ],
        compiler_params=pltpu.CompilerParams(
            dimension_semantics=("arbitrary",),
            vmem_limit_bytes=100 * 1024 * 1024,
        ),
    )(x_t, x_t, A_mem0[0], A_Wq, A_Wk, A_Wv, jnp.transpose(A_Wo, (0, 2, 1)),
      B_w1, B_w3, B_w2.T)
    return out_t.T[None]
```

```python
import functools

import jax
import jax.numpy as jnp
import numpy as np
from jax import lax
import jax.experimental.pallas as pl
import jax.experimental.pallas.tpu as pltpu

_BF16 = jnp.bfloat16
_F32 = jnp.float32
_NT = (((1,), (1,)), ((), ()))
_TOK = 128
_GROUP = 4
_FCHUNK = 512
_WCHUNK = 64
_INFLIGHT = 3
_UNROLL = 1
_EDGE_CHUNKS = 3
_HALF = 256
_WO_FROM = 6
_PAIR_CHUNKS = (768,) * 3
_FIRST_BLOCK_ORDER = (0, 1, 3, 4, 6, 2, 5)
_MASKED = -1000000000.0


def _layernorm(x):
    m = jnp.mean(x, axis=-1, keepdims=True)
    c = x - m
    v = jnp.mean(c * c, axis=-1, keepdims=True)
    return c * lax.rsqrt(v + 1e-05)


def _dot(a, b):
    return lax.dot_general(a, b, (((1,), (0,)), ((), ())), preferred_element_type=_F32)


def _dot_nt(a, b):
    return lax.dot_general(a, b, _NT, preferred_element_type=_F32)


def _pack(x):
    return pltpu.bitcast(x.astype(_BF16), jnp.uint32)


def _unpack(words):
    return pltpu.bitcast(words, _BF16)


def _left_terms(a11, a12, a21, a22):
    if a21 is None:
        return [a11, None, a11, None, a11 + a12, None, a12]
    return [a11 + a22, a21 + a22, a11, a22, a11 + a12, a21 - a11, a12 - a22]


def _right_terms(b11, b12, b21, b22):
    return [b11 + b22, b11, b12 - b22, b21 - b11, b22, b11 + b12, b21 + b22]


def _combine(m):
    top = (m[0] - m[4] + m[6], m[2] + m[4])
    if m[1] is None:
        return [top]
    return [(top[0] + m[3], top[1]), (m[1] + m[3], m[0] - m[1] + m[2] + m[5])]


def _masks(n_mem, length, n_seq):
    rows = n_seq * length

    def describe(axis):
        i = lax.broadcasted_iota(jnp.int32, (rows, rows), axis)
        second = i >= length
        return jnp.where(second, 1, 0), jnp.where(second, i - length, i)

    (seq_r, idx_r), (seq_c, idx_c) = describe(0), describe(1)
    same = seq_r == seq_c
    keep = same & ((idx_r < n_mem) | (idx_r >= idx_c))
    fill = jnp.where(same, _MASKED, -jnp.inf).astype(_F32)
    return keep, fill


def _attention(hs, keep, fill, qkv, qkv_rest, wo, wo_rest, n_heads, dh):
    scale = dh ** -0.5
    width = _GROUP * dh
    half = width // 2
    n_groups = n_heads // _GROUP
    length = hs[0].shape[0]
    heads = [slice(i * dh, (i + 1) * dh) for i in range(_GROUP)]
    lhs_dtype = _BF16 if (len(hs) * length) % 16 == 0 else _F32

    def blocks(rows, size):
        out = [r[:, i * size:(i + 1) * size] for r in rows for i in range(2)]
        return out + [None] * (4 - len(out))

    h_terms = _left_terms(*blocks(hs, _HALF))
    h_rest = jnp.concatenate([h[:, 2 * _HALF:] for h in hs], axis=0).astype(lhs_dtype)

    def project(w, g):
        m = [None if t is None else _dot(t, _unpack(qkv[w, i, :, g * half:(g + 1) * half]))
             for i, t in enumerate(h_terms)]
        full = jnp.concatenate([jnp.concatenate(c, axis=1) for c in _combine(m)], axis=0)
        return full + _dot(h_rest, _unpack(qkv_rest[w, :, g * width:(g + 1) * width]))

    def weights(q, k):
        out = []
        for cols in heads:
            s = jnp.where(keep, _dot_nt(q[:, cols], k[:, cols]) * scale, fill)
            e = jnp.exp(s - jnp.max(s, axis=-1, keepdims=True))
            out.append((e.astype(lhs_dtype), 1.0 / jnp.sum(e, axis=-1, keepdims=True)))
        return out

    def mix(p, v):
        return jnp.concatenate(
            [_dot(e, v[:, cols]) * inv for (e, inv), cols in zip(p, heads)], axis=1)

    def output(o, g):
        rows = [o[i * length:(i + 1) * length] for i in range(len(hs))]
        m = [None if t is None
             else _dot(t, _unpack(wo[i, g * half // 2:(g + 1) * half // 2, :]))
             for i, t in enumerate(_left_terms(*blocks(rows, half)))]
        return m + [_dot(o.astype(lhs_dtype), _unpack(wo_rest[g * half:(g + 1) * half, :]))]

    p, v, o, acc = {}, {}, {}, None
    for g in range(n_groups + 2):
        if g < n_groups:
            q = project(0, g).astype(lhs_dtype)
        if 0 <= g - 1 < n_groups:
            o[g - 1] = mix(p.pop(g - 1), v.pop(g - 1))
        if g < n_groups:
            k = project(1, g).astype(_BF16)
            v[g] = project(2, g).astype(_BF16)
            p[g] = weights(q, k)
        if g - 2 >= 0:
            part = output(o.pop(g - 2), g - 2)
            acc = part if acc is None else [
                None if x is None else x + y for x, y in zip(acc, part)]
    return [jnp.concatenate([*c, acc[7][i * length:(i + 1) * length]], axis=1)
            for i, c in enumerate(_combine(acc))]


def _silu(x):
    half = 0.5 * x
    return half + half * jnp.tanh(half)


def _swiglu_one(xn, w1, w3, w2_t, chunks):
    acc = hid = None
    for n in range(len(chunks) + 1):
        prev = hid
        if n < len(chunks):
            gate = _silu(_dot(xn, w1[:, chunks[n]]))
            hid = (gate * _dot(xn, w3[:, chunks[n]])).astype(_BF16)
        if n >= 1:
            part = _dot_nt(w2_t[:, chunks[n - 1]], prev)
            acc = part if acc is None else acc + part
    return acc


def _swiglu_pair(xa, xb, w1, w3, w1_terms, w3_terms, w2_terms, side_work):
    half = w1.shape[1] // 2
    tok = xa.shape[0]
    x_terms = [t.astype(_BF16) for t in _left_terms(
        xa[:, :_HALF], xa[:, _HALF:2 * _HALF], xb[:, :_HALF], xb[:, _HALF:2 * _HALF])]
    x_rest = jnp.concatenate([xa[:, 2 * _HALF:], xb[:, 2 * _HALF:]], axis=0).astype(_BF16)
    edges = np.cumsum((0,) + _PAIR_CHUNKS)
    chunks = [slice(int(lo), int(hi)) for lo, hi in zip(edges[:-1], edges[1:])]

    def project(w, terms, cols):
        (c11, c12), (c21, c22) = _combine(
            [_dot(t, _unpack(terms[i, :, cols])) for i, t in enumerate(x_terms)])
        lo = _dot(x_rest, w[2 * _HALF:, cols])
        hi = _dot(x_rest, w[2 * _HALF:, half + cols.start:half + cols.stop])
        return c11 + lo[:tok], c21 + lo[tok:], c12 + hi[:tok], c22 + hi[tok:]

    acc, hid = [None] * 7, None
    for n in range(len(chunks) + 1):
        prev = hid
        if n < len(chunks):
            gates = [_silu(g) for g in project(w1, w1_terms, chunks[n])]
            ups = project(w3, w3_terms, chunks[n])
            hid = [t.astype(_BF16) for t in _right_terms(*[g * u for g, u in zip(gates, ups)])]
        if n >= 1:
            for i in _FIRST_BLOCK_ORDER:
                part = _dot_nt(_unpack(w2_terms[i, :, chunks[n - 1]]), prev[i])
                acc[i] = part if acc[i] is None else acc[i] + part
        side_work(n)
    (c11, c12), (c21, c22) = _combine(acc)
    return jnp.concatenate([c11, c21], axis=0), jnp.concatenate([c12, c22], axis=0)


def _store_terms(w, terms, form):
    half_rows, half_cols = 2 * terms.shape[1], terms.shape[2]

    def tile(j, carry):
        near = pl.ds(pl.multiple_of(j * 16, 16), 16)
        far = pl.ds(pl.multiple_of(half_rows + j * 16, 16), 16)
        for c in range(0, half_cols, _HALF):
            blocks = [w[rows, lo:lo + _HALF].astype(_F32)
                      for rows in (near, far) for lo in (c, half_cols + c)]
            for i, t in enumerate(form(*blocks)):
                terms[i, pl.ds(pl.multiple_of(j * 8, 8), 8), c:c + _HALF] = _pack(t)
        return carry

    lax.fori_loop(0, half_rows // 16, tile, 0)


def _load_weights(sources, main, rest, wo_hbm, wo, wo_rest, stage, wo_stage, wsem, osem):
    _, n_heads, dh = sources[0].shape
    pairs = _GROUP // 2
    main_chunks = _HALF // _WCHUNK
    per_weight = main_chunks + 1
    n_jobs = len(sources) * per_weight
    slots = stage.shape[0]

    def copy(src, job, row, n):
        slot = job % slots
        return pltpu.make_async_copy(src.at[pl.ds(row, _WCHUNK)], stage.at[slot, n],
                                     wsem.at[2 * slot + n])

    def for_copies(src, job, action):
        c = job % per_weight
        action(copy(src, job, jnp.where(c < main_chunks, c * _WCHUNK, 2 * _HALF), 0))

        @pl.when(c < main_chunks)
        def _():
            action(copy(src, job, _HALF + c * _WCHUNK, 1))

    def start(job):
        for i, src in enumerate(sources):
            pl.when(job // per_weight == i)(
                functools.partial(for_copies, src, job, lambda c: c.start()))

    def wait(job):
        for i, src in enumerate(sources):
            pl.when(job // per_weight == i)(
                functools.partial(for_copies, src, job, lambda c: c.wait()))

    def head_pairs(slot, n, j):
        rows = pl.ds(pl.multiple_of(j * 16, 16), 16)
        words = jnp.swapaxes(pltpu.bitcast(stage[slot, n, rows], jnp.uint32), 0, 1)
        return [(pltpu.bitcast(words[p] << 16, _F32),
                 pltpu.bitcast(words[p] & jnp.uint32(0xFFFF0000), _F32))
                for p in range(n_heads // 2)]

    def output_pair(p, carry):
        def rows(i):
            return pl.ds(pl.multiple_of(i * (dh // 2), dh // 2), dh // 2)

        even, odd = (wo_stage[2 * p + i, :2 * _HALF].T.astype(_F32) for i in range(2))
        terms = _right_terms(even[:, :_HALF], even[:, _HALF:], odd[:, :_HALF], odd[:, _HALF:])
        for i, t in enumerate(terms):
            wo[i, rows(p), :] = _pack(t)
        for i in range(2):
            at = (p // pairs) * _GROUP + i * pairs + p % pairs
            wo_rest[rows(at), :] = _pack(wo_stage[2 * p + i, 2 * _HALF:].astype(_F32).T)
        return carry

    wo_copy = pltpu.make_async_copy(wo_hbm, wo_stage, osem)
    lax.fori_loop(0, _INFLIGHT, lambda job, carry: start(job), None)
    wo_copy.start()

    def pairs_done(job):
        return (n_heads // 2) * jnp.maximum(job - _WO_FROM, 0) // (n_jobs - _WO_FROM)

    def run(job, carry):
        which, c, slot = job // per_weight, job % per_weight, job % slots
        wait(job)
        start(job + _INFLIGHT)

        def main_rows(j, carry):
            rows = pl.ds(pl.multiple_of(c * (_WCHUNK // 2) + j * 8, 8), 8)
            for p, (lo, hi) in enumerate(zip(head_pairs(slot, 0, j), head_pairs(slot, 1, j))):
                for n, t in enumerate(_right_terms(*lo, *hi)):
                    main[which, n, rows, p * dh:(p + 1) * dh] = _pack(t)
            return carry

        def rest_rows(j, carry):
            rows = pl.ds(pl.multiple_of(j * 8, 8), 8)
            for p, pair in enumerate(head_pairs(slot, 0, j)):
                for n, t in enumerate(pair):
                    at = (p // pairs) * _GROUP + n * pairs + p % pairs
                    rest[which, rows, at * dh:(at + 1) * dh] = _pack(t)
            return carry

        tiles = _WCHUNK // 16
        lax.fori_loop(0, jnp.where(c < main_chunks, tiles, 0), main_rows, 0)
        lax.fori_loop(0, jnp.where(c < main_chunks, 0, tiles), rest_rows, 0)
        pl.when(job == _WO_FROM)(wo_copy.wait)
        lax.fori_loop(pairs_done(job), pairs_done(job + 1), output_pair, 0)
        return carry

    lax.fori_loop(0, n_jobs, run, 0)


def _kernel(x0_ref, x_next_ref, mem0_ref, wq_hbm, wk_hbm, wv_hbm, wo_hbm, w1_hbm, w3_hbm,
            w2_hbm, out_ref,
            stage, wo_stage, qkv, qkv_rest, wo, wo_rest,
            w1, w3, w2_t, w1_terms, w3_terms, w2_terms, res, normed, mem, acc_t, wsem, osem, fsem, *, seg):
    b = pl.program_id(0)
    n_blocks = pl.num_programs(0) - 1
    _, n_heads, dh = wq_hbm.shape
    n_mem = mem0_ref.shape[0]
    n_chunks = w1.shape[1] // _FCHUNK
    steps = _TOK // seg
    ffn_copies = [pltpu.make_async_copy(s, d, fsem.at[i])
                  for i, (s, d) in enumerate(((w1_hbm, w1), (w3_hbm, w3), (w2_hbm, w2_t)))]

    def start_layer(slot, x):
        res[slot] = x
        normed[slot] = _layernorm(x)

    @pl.when(b == 0)
    def _():
        _load_weights((wq_hbm, wk_hbm, wv_hbm), qkv, qkv_rest, wo_hbm, wo, wo_rest,
                      stage, wo_stage, wsem, osem)
        for c in ffn_copies:
            c.start()
        mem[0] = mem0_ref[...].astype(_F32)
        mem[1] = mem0_ref[...].astype(_F32)
        start_layer(0, x0_ref[...].astype(_F32).T)

    def run_attention(first, n_seq, unroll):
        keep, fill = _masks(n_mem, n_mem + seg, n_seq)

        def segment(j):
            rows = pl.ds(pl.multiple_of(j * seg, seg), seg)
            hs = [jnp.concatenate([mem[first + i], normed[first + i, rows]], axis=0)
                  for i in range(n_seq)]
            for i, out in enumerate(_attention(hs, keep, fill, qkv, qkv_rest, wo, wo_rest,
                                               n_heads, dh)):
                mem[first + i] = out[:n_mem]
                res[first + i, rows] += out[n_mem:]

        def step(j, carry):
            for u in range(unroll):
                segment(j * unroll + u)
            return carry

        lax.fori_loop(0, steps // unroll, step, 0)

    both = jnp.logical_and(b > 0, b < n_blocks)

    @pl.when(both)
    def _():
        run_attention(0, 2, _UNROLL)
        x1, x3 = res[0], res[1]

        def side_work(n):
            if n == 0:
                acc_t[...] = x3.T
                res[1] = x1
            if n == 1:
                start_layer(0, x_next_ref[...].astype(_F32).T)

        f2, f4 = _swiglu_pair(_layernorm(x1), _layernorm(x3), w1, w3,
                              w1_terms, w3_terms, w2_terms, side_work)
        start_layer(1, res[1] + f2.T)
        out_ref[...] = (acc_t[...] + f4).astype(out_ref.dtype)

    @pl.when(jnp.logical_not(both))
    def _():
        slot = jnp.where(b == 0, 0, 1)
        run_attention(slot, 1, 1)

        @pl.when(b == 0)
        def _():
            for c, w, terms, form in zip(ffn_copies, (w1, w3, w2_t),
                                         (w1_terms, w3_terms, w2_terms),
                                         (_right_terms, _right_terms, _left_terms)):
                c.wait()
                _store_terms(w, terms, form)

        x = res[slot]
        xn = _layernorm(x).astype(_BF16)
        acc_t[...] = x.T

        def part(i, carry):
            chunks = [pl.ds(pl.multiple_of((i * _EDGE_CHUNKS + c) * _FCHUNK, _FCHUNK), _FCHUNK)
                      for c in range(_EDGE_CHUNKS)]
            acc_t[...] += _swiglu_one(xn, w1, w3, w2_t, chunks)
            return carry

        lax.fori_loop(0, n_chunks // _EDGE_CHUNKS, part, 0)

        @pl.when(b == 0)
        def _():
            start_layer(1, acc_t[...].T)
            start_layer(0, x_next_ref[...].astype(_F32).T)

        @pl.when(b > 0)
        def _():
            out_ref[...] = acc_t[...].astype(out_ref.dtype)


@functools.partial(jax.jit, static_argnames=("A_seg_len",))
def pallas_interleave_layers__memory_aug_recurrent_mem_tr__glu_gated_swiglu__prompt_kernel(
    A_x: jax.Array,
    A_mem0: jax.Array,
    A_Wq: jax.Array,
    A_Wk: jax.Array,
    A_Wv: jax.Array,
    A_Wo: jax.Array,
    A_seg_len: int,
    B_x: jax.Array,
    B_w1: jax.Array,
    B_w3: jax.Array,
    B_w2: jax.Array,
):
    del B_x
    batch, seq, d_model = A_x.shape
    n_mem = A_mem0.shape[1]
    _, n_heads, dh = A_Wq.shape
    d_ff = B_w1.shape[1]
    seg = int(A_seg_len)
    assert batch == 1 and seq % _TOK == 0 and _TOK % seg == 0 and seg % 16 == 0
    assert n_mem == 8 and n_heads % _GROUP == 0 and d_ff % (_FCHUNK * _EDGE_CHUNKS) == 0
    d_rest = d_model - 2 * _HALF
    assert d_rest == _WCHUNK and _HALF % _WCHUNK == 0
    assert sum(_PAIR_CHUNKS) == d_ff // 2 and (d_ff // 2) % _HALF == 0
    n_blocks = seq // _TOK

    x_t = A_x[0].T
    hbm = pl.BlockSpec(memory_space=pl.ANY)
    out_t = pl.pallas_call(
        functools.partial(_kernel, seg=seg),
        grid=(n_blocks + 1,),
        in_specs=[
            pl.BlockSpec((d_model, _TOK), lambda b: (0, 0)),
            pl.BlockSpec((d_model, _TOK), lambda b: (0, jnp.minimum(b + 1, n_blocks - 1))),
            pl.BlockSpec((n_mem, d_model), lambda b: (0, 0)),
            hbm, hbm, hbm, hbm, hbm, hbm, hbm,
        ],
        out_specs=pl.BlockSpec((d_model, _TOK), lambda b: (0, jnp.maximum(b - 1, 0))),
        out_shape=jax.ShapeDtypeStruct((d_model, seq), A_x.dtype),
        scratch_shapes=[
            pltpu.VMEM((_INFLIGHT + 1, 2, _WCHUNK, n_heads, dh), _BF16),
            pltpu.VMEM((n_heads, d_model, dh), _BF16),
            pltpu.VMEM((3, 7, _HALF // 2, n_heads * dh // 2), jnp.uint32),
            pltpu.VMEM((3, d_rest // 2, n_heads * dh), jnp.uint32),
            pltpu.VMEM((7, n_heads * dh // 4, _HALF), jnp.uint32),
            pltpu.VMEM((n_heads * dh // 2, d_rest), jnp.uint32),
            pltpu.VMEM((d_model, d_ff), _BF16),
            pltpu.VMEM((d_model, d_ff), _BF16),
            pltpu.VMEM((d_model, d_ff), _BF16),
            *2 * [pltpu.VMEM((7, _HALF // 2, d_ff // 2), jnp.uint32)],
            pltpu.VMEM((7, d_model // 4, d_ff // 2), jnp.uint32),
            pltpu.VMEM((2, _TOK, d_model), _F32),
            pltpu.VMEM((2, _TOK, d_model), _F32),
            pltpu.VMEM((2, n_mem, d_model), _F32),
            pltpu.VMEM((d_model, _TOK), _F32),
            pltpu.SemaphoreType.DMA((2 * (_INFLIGHT + 1),)),
            pltpu.SemaphoreType.DMA(()),
            pltpu.SemaphoreType.DMA((3,)),
        ],
        compiler_params=pltpu.CompilerParams(
            dimension_semantics=("arbitrary",),
            vmem_limit_bytes=112 * 1024 * 1024,
        ),
    )(x_t, x_t, A_mem0[0], A_Wq, A_Wk, A_Wv, jnp.transpose(A_Wo, (0, 2, 1)),
      B_w1, B_w3, B_w2.T)
    return out_t.T[None]
```

```python
import functools

import jax
import jax.numpy as jnp
import numpy as np
from jax import lax
import jax.experimental.pallas as pl
import jax.experimental.pallas.tpu as pltpu

_BF16 = jnp.bfloat16
_F32 = jnp.float32
_NT = (((1,), (1,)), ((), ()))
_TOK = 128
_GROUP = 4
_FCHUNK = 512
_WCHUNK = 32
_INFLIGHT = 3
_UNROLL = 1
_EDGE_CHUNKS = 3
_QUARTER = 128
_WO_FROM = 6
_PAIR_CHUNK = 384
_MASKED = -1000000000.0


def _layernorm(x):
    m = jnp.mean(x, axis=-1, keepdims=True)
    c = x - m
    v = jnp.mean(c * c, axis=-1, keepdims=True)
    return c * lax.rsqrt(v + 1e-05)


def _dot(a, b):
    return lax.dot_general(a, b, (((1,), (0,)), ((), ())), preferred_element_type=_F32)


def _dot_nt(a, b):
    return lax.dot_general(a, b, _NT, preferred_element_type=_F32)


def _pack(x):
    return pltpu.bitcast(x.astype(_BF16), jnp.uint32)


def _unpack(words):
    return pltpu.bitcast(words, _BF16)


_SCHEME = (
    "...+.... +.......++..--.. .-......",
    "..+++..+ +.........-..... ..-.+...",
    ".+++.... ....+++......... +..-....",
    ".+.+.+.. ...+.......+...- ...-.-.+",
    "++-..... ......+......... -.+++.--",
    "+...+..+ .+-.......-...+. ..-..++.",
    "+.-..... +.....+......... +.-.....",
    "..++..+. +....-..++..-... -+..+...",
    "+....... .+.............. .++..--.",
    ".+...+.. ....++++...+...- ...+....",
    "++-..+.. ...+..-......... ...++.--",
    "..++.-.. ...++++....+.... ...+-...",
    "+..++..+ +.........-...+. ..+.....",
    ".+.+..-. .....+.......... -+...-.+",
    "..++.... +...---.++...... +...-...",
    "..+...+. +....-..+...-... +-......",
    "......+. .....+...-...... -+..+-..",
    ".....+.. ...+..+-...+.... ...+...-",
    "++-.++-. ...+............ ....-.++",
    "....+..+ .+-.......-..... ..+...-.",
    ".+.+.+.+ ...+.+.....+...- .....+.-",
    "....+.-. ...+......+..... ....+.-.",
    ".....+++ ...+.+.....+.... ....-..+",
    "+...+... ..+.......+...-. .....++.",
    ".......+ .+-+.+....-+.-+- .....-..",
    "..++..++ +..-.-....---... ....-...",
)


def _sum_program(rows):
    n_in = len(rows[0])
    rows = [{i: c for i, c in enumerate(row) if c} for row in rows]
    steps, ready = [], list(range(n_in))

    def emit(a, b, sign):
        steps.append((a, b, sign))
        ready.append(max(ready[a], ready[b]))
        return len(ready) - 1

    while True:
        count = {}
        for row in rows:
            items = sorted(row.items())
            for n, (a, x) in enumerate(items):
                for b, y in items[n + 1:]:
                    count[a, b, x * y] = count.get((a, b, x * y), 0) + 1
        best = max(sorted(count), key=count.get, default=None)
        if best is None or count[best] < 2:
            break
        a, b, sign = best
        new = emit(a, b, sign)
        for row in rows:
            if a in row and b in row and row[a] * row[b] == sign:
                row[new] = row.pop(a)
                del row[b]
    outs = []
    for row in rows:
        items = sorted(row.items(), key=lambda item: (ready[item[0]], item[0]))
        at, sign = items[0]
        for b, y in items[1:]:
            if sign < 0 < y:
                at, sign = emit(b, at, -1), 1
            else:
                at = emit(at, b, sign * y)
        outs.append((at, sign))
    return n_in, steps, ready, outs


def _evaluate(program, make):
    n_in, steps, ready, outs = program
    vals = {}
    for i in range(n_in):
        vals[i] = make(i)
        for n, (a, b, sign) in enumerate(steps):
            if ready[n_in + n] == i:
                vals[n_in + n] = vals[a] + vals[b] if sign > 0 else vals[a] - vals[b]
    return [vals[i] if sign > 0 else -vals[i] for i, sign in outs]


def _programs():
    u, v, w = (np.array([[{"+": 1, ".": 0, "-": -1}[c] for c in line.split()[f]]
                         for line in _SCHEME]) for f in range(3))
    want = np.zeros((8, 16, 8), np.int64)
    for i in range(2):
        for k in range(4):
            for j in range(4):
                want[4 * i + k, 4 * k + j, 4 * i + j] = 1
    assert np.array_equal(np.einsum("ra,rb,rc->abc", u, v, w), want)
    assert np.array_equal(np.einsum("ra,rb,rc->abc", u[:16, :4], v[:16], w[:16, :4]),
                          want[:4, :, :4])
    left = {1: _sum_program(u[:16, :4].tolist()), 2: _sum_program(u.tolist())}
    out = {1: _sum_program(w[:16, :4].T.tolist()), 2: _sum_program(w.T.tolist())}
    return left, _sum_program(v.tolist()), out


_LEFT, _RIGHT, _OUT = _programs()
_PRODUCTS = len(_SCHEME)


def _left_terms(rows):
    blocks = [blk for row in rows for blk in row]
    return _evaluate(_LEFT[len(rows)], blocks.__getitem__)


def _right_terms(blocks):
    return _evaluate(_RIGHT, blocks.__getitem__)


def _combine(n_rows, product):
    c = _evaluate(_OUT[n_rows], product)
    return [c[4 * i:4 * i + 4] for i in range(n_rows)]


def _quarters(x):
    return [x[:, i * _QUARTER:(i + 1) * _QUARTER] for i in range(4)]


def _masks(n_mem, length, n_seq):
    rows = n_seq * length

    def describe(axis):
        i = lax.broadcasted_iota(jnp.int32, (rows, rows), axis)
        second = i >= length
        return jnp.where(second, 1, 0), jnp.where(second, i - length, i)

    (seq_r, idx_r), (seq_c, idx_c) = describe(0), describe(1)
    same = seq_r == seq_c
    keep = same & ((idx_r < n_mem) | (idx_r >= idx_c))
    fill = jnp.where(same, _MASKED, -jnp.inf).astype(_F32)
    return keep, fill


def _attention(hs, keep, fill, qkv, qkv_rest, wo, wo_rest, n_heads, dh):
    scale = dh ** -0.5
    width = _GROUP * dh
    n_groups = n_heads // _GROUP
    n_seq, length = len(hs), hs[0].shape[0]
    heads = [slice(i * dh, (i + 1) * dh) for i in range(_GROUP)]
    lhs_dtype = _BF16 if (n_seq * length) % 16 == 0 else _F32

    h_terms = _left_terms([_quarters(h) for h in hs])
    h_rest = jnp.concatenate([h[:, 4 * _QUARTER:] for h in hs], axis=0).astype(lhs_dtype)

    def project(w, g):
        c = _combine(n_seq, lambda i: _dot(
            h_terms[i], _unpack(qkv[w, i, :, g * dh:(g + 1) * dh])))
        full = jnp.concatenate([jnp.concatenate(row, axis=1) for row in c], axis=0)
        return full + _dot(h_rest, _unpack(qkv_rest[w, :, g * width:(g + 1) * width]))

    def weights(q, k):
        out = []
        for cols in heads:
            s = jnp.where(keep, _dot_nt(q[:, cols], k[:, cols]) * scale, fill)
            e = jnp.exp(s - jnp.max(s, axis=-1, keepdims=True))
            out.append((e.astype(lhs_dtype), 1.0 / jnp.sum(e, axis=-1, keepdims=True)))
        return out

    def mix(p, v):
        return jnp.concatenate(
            [_dot(e, v[:, cols]) * inv for (e, inv), cols in zip(p, heads)], axis=1)

    def output(o, g):
        terms = _left_terms([_quarters(o[i * length:(i + 1) * length]) for i in range(n_seq)])
        m = [_dot(t, _unpack(wo[i, g * dh // 2:(g + 1) * dh // 2, :]))
             for i, t in enumerate(terms)]
        rest = _unpack(wo_rest[g * width // 2:(g + 1) * width // 2, :])
        return m + [_dot(o.astype(lhs_dtype), rest)]

    p, v, o, acc = {}, {}, {}, None
    for g in range(n_groups + 2):
        if g < n_groups:
            q = project(0, g).astype(lhs_dtype)
        if 0 <= g - 1 < n_groups:
            o[g - 1] = mix(p.pop(g - 1), v.pop(g - 1))
        if g < n_groups:
            k = project(1, g).astype(_BF16)
            v[g] = project(2, g).astype(_BF16)
            p[g] = weights(q, k)
        if g - 2 >= 0:
            part = output(o.pop(g - 2), g - 2)
            acc = part if acc is None else [x + y for x, y in zip(acc, part)]
    return [jnp.concatenate([*row, acc[-1][i * length:(i + 1) * length]], axis=1)
            for i, row in enumerate(_combine(n_seq, acc.__getitem__))]


def _silu(x):
    half = 0.5 * x
    return half + half * jnp.tanh(half)


def _swiglu_one(xn, w1, w3, w2_t, chunks):
    acc = hid = None
    for n in range(len(chunks) + 1):
        prev = hid
        if n < len(chunks):
            gate = _silu(_dot(xn, w1[:, chunks[n]]))
            hid = (gate * _dot(xn, w3[:, chunks[n]])).astype(_BF16)
        if n >= 1:
            part = _dot_nt(w2_t[:, chunks[n - 1]], prev)
            acc = part if acc is None else acc + part
    return acc


def _swiglu_pair(xa, xb, w1, w3, w1_terms, w3_terms, w2_terms, side_work):
    quarter = w1.shape[1] // 4
    tok = xa.shape[0]
    x_terms = [t.astype(_BF16) for t in _left_terms([_quarters(xa), _quarters(xb)])]
    x_rest = jnp.concatenate([xa[:, 4 * _QUARTER:], xb[:, 4 * _QUARTER:]], axis=0).astype(_BF16)

    def project(w, terms, lo):
        c = _combine(2, lambda i: _dot(x_terms[i], _unpack(terms[i, :, lo:lo + _QUARTER])))
        rest = [_dot(x_rest, w[4 * _QUARTER:, j * quarter + lo:j * quarter + lo + _QUARTER])
                for j in range(4)]
        return [c[i][j] + rest[j][i * tok:(i + 1) * tok] for i in range(2) for j in range(4)]

    def hidden(lo):
        gates = [_silu(g) for g in project(w1, w1_terms, lo)]
        hid = [g * u for g, u in zip(gates, project(w3, w3_terms, lo))]
        return [t.astype(_BF16) for t in _left_terms([hid[:4], hid[4:]])]

    chunks = list(range(0, quarter, _PAIR_CHUNK))
    acc, hid = [None] * _PRODUCTS, None
    for n in range(len(chunks) + 1):
        prev = hid
        if n < len(chunks):
            tiles = [hidden(lo) for lo in range(chunks[n], chunks[n] + _PAIR_CHUNK, _QUARTER)]
            hid = [jnp.concatenate(t, axis=1) for t in zip(*tiles)]
        if n >= 1:
            cols = slice(chunks[n - 1], chunks[n - 1] + _PAIR_CHUNK)
            for i in range(_PRODUCTS):
                part = _dot_nt(_unpack(w2_terms[i, :, cols]), prev[i])
                acc[i] = part if acc[i] is None else acc[i] + part
        side_work(n)
    return [jnp.concatenate(row, axis=0) for row in _combine(2, acc.__getitem__)]


def _store_terms(w, terms, transposed):
    block_rows, block_cols = 2 * terms.shape[1], terms.shape[2]

    def tile(j, carry):
        def block(r, c, lo):
            rows = pl.ds(pl.multiple_of(r * block_rows + j * 16, 16), 16)
            return w[rows, c * block_cols + lo:c * block_cols + lo + _QUARTER].astype(_F32)

        for lo in range(0, block_cols, _QUARTER):
            blocks = [block(n, k, lo) if transposed else block(k, n, lo)
                      for k in range(4) for n in range(4)]
            for i, t in enumerate(_right_terms(blocks)):
                terms[i, pl.ds(pl.multiple_of(j * 8, 8), 8), lo:lo + _QUARTER] = _pack(t)
        return carry

    lax.fori_loop(0, block_rows // 16, tile, 0)


def _load_weights(sources, main, rest, wo_hbm, wo, wo_rest, stage, wo_stage, wsem, osem):
    _, n_heads, dh = sources[0].shape
    n_groups = n_heads // _GROUP
    main_chunks = _QUARTER // _WCHUNK
    per_weight = main_chunks + 1
    n_jobs = len(sources) * per_weight
    slots = stage.shape[0]
    rest_parts = 2 * rest.shape[1] // _WCHUNK

    def for_copies(src, job, action):
        c, slot = job % per_weight, job % slots

        def copy(row, n):
            action(pltpu.make_async_copy(src.at[pl.ds(row, _WCHUNK)], stage.at[slot, n],
                                         wsem.at[4 * slot + n]))

        @pl.when(c < main_chunks)
        def _():
            for n in range(4):
                copy(n * _QUARTER + c * _WCHUNK, n)

        @pl.when(c == main_chunks)
        def _():
            for n in range(rest_parts):
                copy(4 * _QUARTER + n * _WCHUNK, n)

    def start(job):
        for i, src in enumerate(sources):
            pl.when(job // per_weight == i)(
                functools.partial(for_copies, src, job, lambda c: c.start()))

    def wait(job):
        for i, src in enumerate(sources):
            pl.when(job // per_weight == i)(
                functools.partial(for_copies, src, job, lambda c: c.wait()))

    def split_heads(slot, n, j):
        rows = pl.ds(pl.multiple_of(j * 16, 16), 16)
        words = jnp.swapaxes(pltpu.bitcast(stage[slot, n, rows], jnp.uint32), 0, 1)
        return [pltpu.bitcast(half, _F32) for p in range(n_heads // 2)
                for half in (words[p] << 16, words[p] & jnp.uint32(0xFFFF0000))]

    def output_group(g, carry):
        heads = [wo_stage[_GROUP * g + i, :4 * _QUARTER].T for i in range(_GROUP)]
        for r in range(0, dh, 16):
            blocks = [blk for h in heads for blk in _quarters(h[r:r + 16].astype(_F32))]
            rows = pl.ds(pl.multiple_of(g * (dh // 2) + r // 2, 8), 8)
            for i, t in enumerate(_right_terms(blocks)):
                wo[i, rows, :] = _pack(t)
        for i in range(_GROUP):
            head = _GROUP * g + i
            wo_rest[pl.ds(pl.multiple_of(head * (dh // 2), dh // 2), dh // 2), :] = _pack(
                wo_stage[head, 4 * _QUARTER:].astype(_F32).T)
        return carry

    wo_copy = pltpu.make_async_copy(wo_hbm, wo_stage, osem)
    lax.fori_loop(0, _INFLIGHT, lambda job, carry: start(job), None)
    wo_copy.start()

    def groups_done(job):
        return n_groups * jnp.maximum(job - _WO_FROM, 0) // (n_jobs - _WO_FROM)

    def run(job, carry):
        which, c, slot = job // per_weight, job % per_weight, job % slots
        wait(job)
        start(job + _INFLIGHT)

        def main_rows(j, carry):
            rows = pl.ds(pl.multiple_of(c * (_WCHUNK // 2) + j * 8, 8), 8)
            parts = [split_heads(slot, n, j) for n in range(4)]
            for g in range(n_groups):
                blocks = [h for part in parts for h in part[_GROUP * g:_GROUP * (g + 1)]]
                for n, t in enumerate(_right_terms(blocks)):
                    main[which, n, rows, g * dh:(g + 1) * dh] = _pack(t)
            return carry

        def rest_rows(j, carry):
            rows = pl.ds(pl.multiple_of(j * 8, 8), 8)
            for h, t in enumerate(split_heads(slot, j // tiles, j % tiles)):
                rest[which, rows, h * dh:(h + 1) * dh] = _pack(t)
            return carry

        tiles = _WCHUNK // 16
        lax.fori_loop(0, jnp.where(c < main_chunks, tiles, 0), main_rows, 0)
        lax.fori_loop(0, jnp.where(c < main_chunks, 0, rest_parts * tiles), rest_rows, 0)
        pl.when(job == _WO_FROM)(wo_copy.wait)
        lax.fori_loop(groups_done(job), groups_done(job + 1), output_group, 0)
        return carry

    lax.fori_loop(0, n_jobs, run, 0)


def _kernel(x0_ref, x_next_ref, mem0_ref, wq_hbm, wk_hbm, wv_hbm, wo_hbm, w1_hbm, w3_hbm,
            w2_hbm, out_ref,
            stage, wo_stage, qkv, qkv_rest, wo, wo_rest,
            w1, w3, w2_t, w1_terms, w3_terms, w2_terms, res, normed, mem, acc_t, wsem, osem, fsem, *, seg):
    b = pl.program_id(0)
    n_blocks = pl.num_programs(0) - 1
    _, n_heads, dh = wq_hbm.shape
    n_mem = mem0_ref.shape[0]
    n_chunks = w1.shape[1] // _FCHUNK
    steps = _TOK // seg
    ffn_copies = [pltpu.make_async_copy(s, d, fsem.at[i])
                  for i, (s, d) in enumerate(((w1_hbm, w1), (w3_hbm, w3), (w2_hbm, w2_t)))]

    def start_layer(slot, x):
        res[slot] = x
        normed[slot] = _layernorm(x)

    @pl.when(b == 0)
    def _():
        _load_weights((wq_hbm, wk_hbm, wv_hbm), qkv, qkv_rest, wo_hbm, wo, wo_rest,
                      stage, wo_stage, wsem, osem)
        for c in ffn_copies:
            c.start()
        mem[0] = mem0_ref[...].astype(_F32)
        mem[1] = mem0_ref[...].astype(_F32)
        start_layer(0, x0_ref[...].astype(_F32).T)

    def run_attention(first, n_seq, unroll):
        keep, fill = _masks(n_mem, n_mem + seg, n_seq)

        def segment(j):
            rows = pl.ds(pl.multiple_of(j * seg, seg), seg)
            hs = [jnp.concatenate([mem[first + i], normed[first + i, rows]], axis=0)
                  for i in range(n_seq)]
            for i, out in enumerate(_attention(hs, keep, fill, qkv, qkv_rest, wo, wo_rest,
                                               n_heads, dh)):
                mem[first + i] = out[:n_mem]
                res[first + i, rows] += out[n_mem:]

        def step(j, carry):
            for u in range(unroll):
                segment(j * unroll + u)
            return carry

        lax.fori_loop(0, steps // unroll, step, 0)

    both = jnp.logical_and(b > 0, b < n_blocks)

    @pl.when(both)
    def _():
        run_attention(0, 2, _UNROLL)
        x1, x3 = res[0], res[1]

        def side_work(n):
            if n == 0:
                acc_t[...] = x3.T
                res[1] = x1
            if n == 1:
                start_layer(0, x_next_ref[...].astype(_F32).T)

        f2, f4 = _swiglu_pair(_layernorm(x1), _layernorm(x3), w1, w3,
                              w1_terms, w3_terms, w2_terms, side_work)
        start_layer(1, res[1] + f2.T)
        out_ref[...] = (acc_t[...] + f4).astype(out_ref.dtype)

    @pl.when(jnp.logical_not(both))
    def _():
        slot = jnp.where(b == 0, 0, 1)
        run_attention(slot, 1, 1)

        @pl.when(b == 0)
        def _():
            for c, w, terms in zip(ffn_copies, (w1, w3, w2_t), (w1_terms, w3_terms, w2_terms)):
                c.wait()
                _store_terms(w, terms, w is w2_t)

        x = res[slot]
        xn = _layernorm(x).astype(_BF16)
        acc_t[...] = x.T

        def part(i, carry):
            chunks = [pl.ds(pl.multiple_of((i * _EDGE_CHUNKS + c) * _FCHUNK, _FCHUNK), _FCHUNK)
                      for c in range(_EDGE_CHUNKS)]
            acc_t[...] += _swiglu_one(xn, w1, w3, w2_t, chunks)
            return carry

        lax.fori_loop(0, n_chunks // _EDGE_CHUNKS, part, 0)

        @pl.when(b == 0)
        def _():
            start_layer(1, acc_t[...].T)
            start_layer(0, x_next_ref[...].astype(_F32).T)

        @pl.when(b > 0)
        def _():
            out_ref[...] = acc_t[...].astype(out_ref.dtype)


@functools.partial(jax.jit, static_argnames=("A_seg_len",))
def pallas_interleave_layers__memory_aug_recurrent_mem_tr__glu_gated_swiglu__prompt_kernel(
    A_x: jax.Array,
    A_mem0: jax.Array,
    A_Wq: jax.Array,
    A_Wk: jax.Array,
    A_Wv: jax.Array,
    A_Wo: jax.Array,
    A_seg_len: int,
    B_x: jax.Array,
    B_w1: jax.Array,
    B_w3: jax.Array,
    B_w2: jax.Array,
):
    del B_x
    batch, seq, d_model = A_x.shape
    n_mem = A_mem0.shape[1]
    _, n_heads, dh = A_Wq.shape
    d_ff = B_w1.shape[1]
    seg = int(A_seg_len)
    assert batch == 1 and seq % _TOK == 0 and _TOK % seg == 0 and seg % 16 == 0
    assert n_mem == 8 and n_heads % _GROUP == 0 and d_ff % (_FCHUNK * _EDGE_CHUNKS) == 0
    d_rest = d_model - 4 * _QUARTER
    assert 0 < d_rest <= 4 * _WCHUNK and d_rest % _WCHUNK == 0 and d_model % 64 == 0
    assert dh == _QUARTER and d_ff % (4 * _PAIR_CHUNK) == 0
    n_blocks = seq // _TOK

    x_t = A_x[0].T
    hbm = pl.BlockSpec(memory_space=pl.ANY)
    out_t = pl.pallas_call(
        functools.partial(_kernel, seg=seg),
        grid=(n_blocks + 1,),
        in_specs=[
            pl.BlockSpec((d_model, _TOK), lambda b: (0, 0)),
            pl.BlockSpec((d_model, _TOK), lambda b: (0, jnp.minimum(b + 1, n_blocks - 1))),
            pl.BlockSpec((n_mem, d_model), lambda b: (0, 0)),
            hbm, hbm, hbm, hbm, hbm, hbm, hbm,
        ],
        out_specs=pl.BlockSpec((d_model, _TOK), lambda b: (0, jnp.maximum(b - 1, 0))),
        out_shape=jax.ShapeDtypeStruct((d_model, seq), A_x.dtype),
        scratch_shapes=[
            pltpu.VMEM((_INFLIGHT + 1, 4, _WCHUNK, n_heads, dh), _BF16),
            pltpu.VMEM((n_heads, d_model, dh), _BF16),
            pltpu.VMEM((3, _PRODUCTS, _QUARTER // 2, n_heads * dh // 4), jnp.uint32),
            pltpu.VMEM((3, d_rest // 2, n_heads * dh), jnp.uint32),
            pltpu.VMEM((_PRODUCTS, n_heads * dh // 8, _QUARTER), jnp.uint32),
            pltpu.VMEM((n_heads * dh // 2, d_rest), jnp.uint32),
            pltpu.VMEM((d_model, d_ff), _BF16),
            pltpu.VMEM((d_model, d_ff), _BF16),
            pltpu.VMEM((d_model, d_ff), _BF16),
            *2 * [pltpu.VMEM((_PRODUCTS, _QUARTER // 2, d_ff // 4), jnp.uint32)],
            pltpu.VMEM((_PRODUCTS, d_model // 8, d_ff // 4), jnp.uint32),
            pltpu.VMEM((2, _TOK, d_model), _F32),
            pltpu.VMEM((2, _TOK, d_model), _F32),
            pltpu.VMEM((2, n_mem, d_model), _F32),
            pltpu.VMEM((d_model, _TOK), _F32),
            pltpu.SemaphoreType.DMA((4 * (_INFLIGHT + 1),)),
            pltpu.SemaphoreType.DMA(()),
            pltpu.SemaphoreType.DMA((3,)),
        ],
        compiler_params=pltpu.CompilerParams(
            dimension_semantics=("arbitrary",),
            vmem_limit_bytes=112 * 1024 * 1024,
        ),
    )(x_t, x_t, A_mem0[0], A_Wq, A_Wk, A_Wv, jnp.transpose(A_Wo, (0, 2, 1)),
      B_w1, B_w3, B_w2.T)
    return out_t.T[None]
```

```python
import functools

import jax
import jax.numpy as jnp
import numpy as np
from jax import lax
import jax.experimental.pallas as pl
import jax.experimental.pallas.tpu as pltpu

_BF16 = jnp.bfloat16
_F32 = jnp.float32
_NT = (((1,), (1,)), ((), ()))
_TOK = 128
_GROUP = 4
_FCHUNK = 512
_WCHUNK = 32
_INFLIGHT = 3
_UNROLL = 1
_EDGE_CHUNKS = 3
_QUARTER = 128
_WO_FROM = 6
_PAIR_CHUNK = 384
_LATER_FROM = 1
_MASKED = -1000000000.0


def _layernorm(x):
    m = jnp.mean(x, axis=-1, keepdims=True)
    c = x - m
    v = jnp.mean(c * c, axis=-1, keepdims=True)
    return c * lax.rsqrt(v + 1e-05)


def _dot(a, b):
    return lax.dot_general(a, b, (((1,), (0,)), ((), ())), preferred_element_type=_F32)


def _dot_nt(a, b):
    return lax.dot_general(a, b, _NT, preferred_element_type=_F32)


def _pack(x):
    return pltpu.bitcast(x.astype(_BF16), jnp.uint32)


def _split_words(words):
    return (pltpu.bitcast(words << 16, _F32),
            pltpu.bitcast(words & jnp.uint32(0xFFFF0000), _F32))


def _unpack(words):
    return pltpu.bitcast(words, _BF16)


_SCHEME = (
    "...+.... +.......++..--.. .-......",
    "..+++..+ +.........-..... ..-.+...",
    ".+++.... ....+++......... +..-....",
    ".+.+.+.. ...+.......+...- ...-.-.+",
    "++-..... ......+......... -.+++.--",
    "+...+..+ .+-.......-...+. ..-..++.",
    "+.-..... +.....+......... +.-.....",
    "..++..+. +....-..++..-... -+..+...",
    "+....... .+.............. .++..--.",
    ".+...+.. ....++++...+...- ...+....",
    "++-..+.. ...+..-......... ...++.--",
    "..++.-.. ...++++....+.... ...+-...",
    "+..++..+ +.........-...+. ..+.....",
    ".+.+..-. .....+.......... -+...-.+",
    "..++.... +...---.++...... +...-...",
    "..+...+. +....-..+...-... +-......",
    "......+. .....+...-...... -+..+-..",
    ".....+.. ...+..+-...+.... ...+...-",
    "++-.++-. ...+............ ....-.++",
    "....+..+ .+-.......-..... ..+...-.",
    ".+.+.+.+ ...+.+.....+...- .....+.-",
    "....+.-. ...+......+..... ....+.-.",
    ".....+++ ...+.+.....+.... ....-..+",
    "+...+... ..+.......+...-. .....++.",
    ".......+ .+-+.+....-+.-+- .....-..",
    "..++..++ +..-.-....---... ....-...",
)


def _sum_program(rows):
    n_in = len(rows[0])
    rows = [{i: c for i, c in enumerate(row) if c} for row in rows]
    steps, ready = [], list(range(n_in))

    def emit(a, b, sign):
        steps.append((a, b, sign))
        ready.append(max(ready[a], ready[b]))
        return len(ready) - 1

    while True:
        count = {}
        for row in rows:
            items = sorted(row.items())
            for n, (a, x) in enumerate(items):
                for b, y in items[n + 1:]:
                    count[a, b, x * y] = count.get((a, b, x * y), 0) + 1
        best = max(sorted(count), key=count.get, default=None)
        if best is None or count[best] < 2:
            break
        a, b, sign = best
        new = emit(a, b, sign)
        for row in rows:
            if a in row and b in row and row[a] * row[b] == sign:
                row[new] = row.pop(a)
                del row[b]
    outs = []
    for row in rows:
        items = sorted(row.items(), key=lambda item: (ready[item[0]], item[0]))
        at, sign = items[0]
        for b, y in items[1:]:
            if sign < 0 < y:
                at, sign = emit(b, at, -1), 1
            else:
                at = emit(at, b, sign * y)
        outs.append((at, sign))
    return n_in, steps, ready, outs


def _evaluate(program, make):
    n_in, steps, ready, outs = program
    vals = {}
    for i in range(n_in):
        vals[i] = make(i)
        for n, (a, b, sign) in enumerate(steps):
            if ready[n_in + n] == i:
                vals[n_in + n] = vals[a] + vals[b] if sign > 0 else vals[a] - vals[b]
    return [vals[i] if sign > 0 else -vals[i] for i, sign in outs]


def _programs():
    u, v, w = (np.array([[{"+": 1, ".": 0, "-": -1}[c] for c in line.split()[f]]
                         for line in _SCHEME]) for f in range(3))
    want = np.zeros((8, 16, 8), np.int64)
    for i in range(2):
        for k in range(4):
            for j in range(4):
                want[4 * i + k, 4 * k + j, 4 * i + j] = 1
    assert np.array_equal(np.einsum("ra,rb,rc->abc", u, v, w), want)
    assert np.array_equal(np.einsum("ra,rb,rc->abc", u[:16, :4], v[:16], w[:16, :4]),
                          want[:4, :, :4])
    left = {1: _sum_program(u[:16, :4].tolist()), 2: _sum_program(u.tolist())}
    out = {1: _sum_program(w[:16, :4].T.tolist()), 2: _sum_program(w.T.tolist())}
    return left, _sum_program(v.tolist()), out


_LEFT, _RIGHT, _OUT = _programs()
_PRODUCTS = len(_SCHEME)


def _left_terms(rows):
    blocks = [blk for row in rows for blk in row]
    return _evaluate(_LEFT[len(rows)], blocks.__getitem__)


def _right_terms(blocks):
    return _evaluate(_RIGHT, blocks.__getitem__)


def _combine(n_rows, product):
    c = _evaluate(_OUT[n_rows], product)
    return [c[4 * i:4 * i + 4] for i in range(n_rows)]


def _quarters(x):
    return [x[:, i * _QUARTER:(i + 1) * _QUARTER] for i in range(4)]


def _masks(n_mem, length, n_seq):
    rows = n_seq * length

    def describe(axis):
        i = lax.broadcasted_iota(jnp.int32, (rows, rows), axis)
        second = i >= length
        return jnp.where(second, 1, 0), jnp.where(second, i - length, i)

    (seq_r, idx_r), (seq_c, idx_c) = describe(0), describe(1)
    same = seq_r == seq_c
    keep = same & ((idx_r < n_mem) | (idx_r >= idx_c))
    fill = jnp.where(same, _MASKED, -jnp.inf).astype(_F32)
    return keep, fill


def _attention(hs, keep, fill, qkv, qkv_rest, wo, wo_rest, n_heads, dh):
    scale = dh ** -0.5
    width = _GROUP * dh
    n_groups = n_heads // _GROUP
    n_seq, length = len(hs), hs[0].shape[0]
    heads = [slice(i * dh, (i + 1) * dh) for i in range(_GROUP)]
    lhs_dtype = _BF16 if (n_seq * length) % 16 == 0 else _F32

    h_terms = _left_terms([_quarters(h) for h in hs])
    h_rest = jnp.concatenate([h[:, 4 * _QUARTER:] for h in hs], axis=0).astype(lhs_dtype)

    def project(w, g):
        c = _combine(n_seq, lambda i: _dot(
            h_terms[i], _unpack(qkv[w, i, :, g * dh:(g + 1) * dh])))
        full = jnp.concatenate([jnp.concatenate(row, axis=1) for row in c], axis=0)
        return full + _dot(h_rest, _unpack(qkv_rest[w, :, g * width:(g + 1) * width]))

    def weights(q, k):
        out = []
        for cols in heads:
            s = jnp.where(keep, _dot_nt(q[:, cols], k[:, cols]) * scale, fill)
            e = jnp.exp(s - jnp.max(s, axis=-1, keepdims=True))
            out.append((e.astype(lhs_dtype), 1.0 / jnp.sum(e, axis=-1, keepdims=True)))
        return out

    def mix(p, v):
        return jnp.concatenate(
            [_dot(e, v[:, cols]) * inv for (e, inv), cols in zip(p, heads)], axis=1)

    def output(o, g):
        terms = _left_terms([_quarters(o[i * length:(i + 1) * length]) for i in range(n_seq)])
        m = [_dot(t, _unpack(wo[i, g * dh // 2:(g + 1) * dh // 2, :]))
             for i, t in enumerate(terms)]
        rest = _unpack(wo_rest[g * width // 2:(g + 1) * width // 2, :])
        return m + [_dot(o.astype(lhs_dtype), rest)]

    p, v, o, acc = {}, {}, {}, None
    for g in range(n_groups + 2):
        if g < n_groups:
            q = project(0, g).astype(lhs_dtype)
        if 0 <= g - 1 < n_groups:
            o[g - 1] = mix(p.pop(g - 1), v.pop(g - 1))
        if g < n_groups:
            k = project(1, g).astype(_BF16)
            v[g] = project(2, g).astype(_BF16)
            p[g] = weights(q, k)
        if g - 2 >= 0:
            part = output(o.pop(g - 2), g - 2)
            acc = part if acc is None else [x + y for x, y in zip(acc, part)]
    return [jnp.concatenate([*row, acc[-1][i * length:(i + 1) * length]], axis=1)
            for i, row in enumerate(_combine(n_seq, acc.__getitem__))]


def _silu(x):
    half = 0.5 * x
    return half + half * jnp.tanh(half)


def _swiglu_one(xn, w1, w3, w2_t, chunks):
    acc = hid = None
    for n in range(len(chunks) + 1):
        prev = hid
        if n < len(chunks):
            gate = _silu(_dot(xn, w1[:, chunks[n]]))
            hid = (gate * _dot(xn, w3[:, chunks[n]])).astype(_BF16)
        if n >= 1:
            part = _dot_nt(w2_t[:, chunks[n - 1]], prev)
            acc = part if acc is None else acc + part
    return acc


def _swiglu_pair(xa, xb, w1, w3, w1_terms, w3_terms, w2_terms, side_work):
    quarter = w1.shape[1] // 4
    tok = xa.shape[0]
    x_terms = [t.astype(_BF16) for t in _left_terms([_quarters(xa), _quarters(xb)])]
    x_rest = jnp.concatenate([xa[:, 4 * _QUARTER:], xb[:, 4 * _QUARTER:]], axis=0).astype(_BF16)

    def project(w, terms, lo):
        c = _combine(2, lambda i: _dot(x_terms[i], _unpack(terms[i, :, lo:lo + _QUARTER])))
        rest = [_dot(x_rest, w[4 * _QUARTER:, j * quarter + lo:j * quarter + lo + _QUARTER])
                for j in range(4)]
        return [c[i][j] + rest[j][i * tok:(i + 1) * tok] for i in range(2) for j in range(4)]

    def hidden(lo):
        gates = [_silu(g) for g in project(w1, w1_terms, lo)]
        hid = [g * u for g, u in zip(gates, project(w3, w3_terms, lo))]
        return [t.astype(_BF16) for t in _left_terms([hid[:4], hid[4:]])]

    chunks = list(range(0, quarter, _PAIR_CHUNK))
    acc, hid = [None] * _PRODUCTS, None
    for n in range(len(chunks) + 1):
        prev = hid
        if n < len(chunks):
            tiles = [hidden(lo) for lo in range(chunks[n], chunks[n] + _PAIR_CHUNK, _QUARTER)]
            hid = [jnp.concatenate(t, axis=1) for t in zip(*tiles)]
        if n >= 1:
            cols = slice(chunks[n - 1], chunks[n - 1] + _PAIR_CHUNK)
            for i in range(_PRODUCTS):
                part = _dot_nt(_unpack(w2_terms[i, :, cols]), prev[i])
                acc[i] = part if acc[i] is None else acc[i] + part
        side_work(n)
    return [jnp.concatenate(row, axis=0) for row in _combine(2, acc.__getitem__)]


def _store_terms(w, terms, transposed):
    block_rows, block_cols = 2 * terms.shape[1], terms.shape[2]

    def tile(j, carry):
        def block(r, c, lo):
            rows = pl.ds(pl.multiple_of(r * block_rows + j * 16, 16), 16)
            return pltpu.bitcast(
                w[rows, c * block_cols + lo:c * block_cols + lo + _QUARTER], jnp.uint32)

        for lo in range(0, block_cols, _QUARTER):
            words = [block(n, k, lo) if transposed else block(k, n, lo)
                     for k in range(4) for n in range(4)]
            even, odd = (_right_terms(rows) for rows in zip(*map(_split_words, words)))
            for i, pair in enumerate(zip(even, odd)):
                terms[i, pl.ds(pl.multiple_of(j * 8, 8), 8), lo:lo + _QUARTER] = (
                    pltpu.pack_elementwise(pair, packed_dtype=_BF16))
        return carry

    lax.fori_loop(0, block_rows // 16, tile, 0)


def _load_weights(sources, main, rest, wo_hbm, wo, wo_rest, stage, wo_stage, wsem, osem,
                  later_copies):
    _, n_heads, dh = sources[0].shape
    n_groups = n_heads // _GROUP
    main_chunks = _QUARTER // _WCHUNK
    per_weight = main_chunks + 1
    n_jobs = len(sources) * per_weight
    slots = stage.shape[0]
    rest_parts = 2 * rest.shape[1] // _WCHUNK

    def for_copies(src, job, action):
        c, slot = job % per_weight, job % slots

        def copy(row, n):
            action(pltpu.make_async_copy(src.at[pl.ds(row, _WCHUNK)], stage.at[slot, n],
                                         wsem.at[4 * slot + n]))

        @pl.when(c < main_chunks)
        def _():
            for n in range(4):
                copy(n * _QUARTER + c * _WCHUNK, n)

        @pl.when(c == main_chunks)
        def _():
            for n in range(rest_parts):
                copy(4 * _QUARTER + n * _WCHUNK, n)

    def start(job):
        for i, src in enumerate(sources):
            pl.when(job // per_weight == i)(
                functools.partial(for_copies, src, job, lambda c: c.start()))

    def wait(job):
        for i, src in enumerate(sources):
            pl.when(job // per_weight == i)(
                functools.partial(for_copies, src, job, lambda c: c.wait()))

    def split_heads(slot, n, j):
        rows = pl.ds(pl.multiple_of(j * 16, 16), 16)
        words = jnp.swapaxes(pltpu.bitcast(stage[slot, n, rows], jnp.uint32), 0, 1)
        return [half for p in range(n_heads // 2) for half in _split_words(words[p])]

    def output_group(g, carry):
        heads = [wo_stage[_GROUP * g + i, :4 * _QUARTER].T for i in range(_GROUP)]
        for r in range(0, dh, 16):
            blocks = [blk for h in heads for blk in _quarters(h[r:r + 16].astype(_F32))]
            rows = pl.ds(pl.multiple_of(g * (dh // 2) + r // 2, 8), 8)
            for i, t in enumerate(_right_terms(blocks)):
                wo[i, rows, :] = _pack(t)
        for i in range(_GROUP):
            head = _GROUP * g + i
            wo_rest[pl.ds(pl.multiple_of(head * (dh // 2), dh // 2), dh // 2), :] = _pack(
                wo_stage[head, 4 * _QUARTER:].astype(_F32).T)
        return carry

    wo_copy = pltpu.make_async_copy(wo_hbm, wo_stage, osem)
    lax.fori_loop(0, _INFLIGHT, lambda job, carry: start(job), None)
    wo_copy.start()

    def groups_done(job):
        return n_groups * jnp.maximum(job - _WO_FROM, 0) // (n_jobs - _WO_FROM)

    def run(job, carry):
        which, c, slot = job // per_weight, job % per_weight, job % slots
        wait(job)
        start(job + _INFLIGHT)

        @pl.when(job == n_jobs - _LATER_FROM)
        def _():
            for copy in later_copies:
                copy.start()


        def main_rows(j, carry):
            rows = pl.ds(pl.multiple_of(c * (_WCHUNK // 2) + j * 8, 8), 8)
            parts = [split_heads(slot, n, j) for n in range(4)]
            for g in range(n_groups):
                blocks = [h for part in parts for h in part[_GROUP * g:_GROUP * (g + 1)]]
                for n, t in enumerate(_right_terms(blocks)):
                    main[which, n, rows, g * dh:(g + 1) * dh] = _pack(t)
            return carry

        def rest_rows(j, carry):
            rows = pl.ds(pl.multiple_of(j * 8, 8), 8)
            for h, t in enumerate(split_heads(slot, j // tiles, j % tiles)):
                rest[which, rows, h * dh:(h + 1) * dh] = _pack(t)
            return carry

        tiles = _WCHUNK // 16
        lax.fori_loop(0, jnp.where(c < main_chunks, tiles, 0), main_rows, 0)
        lax.fori_loop(0, jnp.where(c < main_chunks, 0, rest_parts * tiles), rest_rows, 0)
        pl.when(job == _WO_FROM)(wo_copy.wait)
        lax.fori_loop(groups_done(job), groups_done(job + 1), output_group, 0)
        return carry

    lax.fori_loop(0, n_jobs, run, 0)


def _kernel(x0_ref, x_next_ref, mem0_ref, wq_hbm, wk_hbm, wv_hbm, wo_hbm, w1_hbm, w3_hbm,
            w2_hbm, out_ref,
            stage, wo_stage, qkv, qkv_rest, wo, wo_rest,
            w1, w3, w2_t, w1_terms, w3_terms, w2_terms, res, normed, mem, acc_t, wsem, osem, fsem, *, seg):
    b = pl.program_id(0)
    n_blocks = pl.num_programs(0) - 1
    _, n_heads, dh = wq_hbm.shape
    n_mem = mem0_ref.shape[0]
    n_chunks = w1.shape[1] // _FCHUNK
    steps = _TOK // seg
    ffn_copies = [pltpu.make_async_copy(s, d, fsem.at[i])
                  for i, (s, d) in enumerate(((w1_hbm, w1), (w3_hbm, w3), (w2_hbm, w2_t)))]

    def start_layer(slot, x):
        res[slot] = x
        normed[slot] = _layernorm(x)

    @pl.when(b == 0)
    def _():
        _load_weights((wq_hbm, wk_hbm, wv_hbm), qkv, qkv_rest, wo_hbm, wo, wo_rest,
                      stage, wo_stage, wsem, osem, ffn_copies)
        mem[0] = mem0_ref[...].astype(_F32)
        mem[1] = mem0_ref[...].astype(_F32)
        start_layer(0, x0_ref[...].astype(_F32).T)

    def run_attention(first, n_seq, unroll):
        keep, fill = _masks(n_mem, n_mem + seg, n_seq)

        def segment(j):
            rows = pl.ds(pl.multiple_of(j * seg, seg), seg)
            hs = [jnp.concatenate([mem[first + i], normed[first + i, rows]], axis=0)
                  for i in range(n_seq)]
            for i, out in enumerate(_attention(hs, keep, fill, qkv, qkv_rest, wo, wo_rest,
                                               n_heads, dh)):
                mem[first + i] = out[:n_mem]
                res[first + i, rows] += out[n_mem:]

        def step(j, carry):
            for u in range(unroll):
                segment(j * unroll + u)
            return carry

        lax.fori_loop(0, steps // unroll, step, 0)

    both = jnp.logical_and(b > 0, b < n_blocks)

    @pl.when(both)
    def _():
        run_attention(0, 2, _UNROLL)
        x1, x3 = res[0], res[1]

        def side_work(n):
            if n == 0:
                acc_t[...] = x3.T
                res[1] = x1
            if n == 1:
                start_layer(0, x_next_ref[...].astype(_F32).T)

        f2, f4 = _swiglu_pair(_layernorm(x1), _layernorm(x3), w1, w3,
                              w1_terms, w3_terms, w2_terms, side_work)
        start_layer(1, res[1] + f2.T)
        out_ref[...] = (acc_t[...] + f4).astype(out_ref.dtype)

    @pl.when(jnp.logical_not(both))
    def _():
        slot = jnp.where(b == 0, 0, 1)
        run_attention(slot, 1, 1)

        @pl.when(b == 0)
        def _():
            for c, w, terms in zip(ffn_copies, (w1, w3, w2_t), (w1_terms, w3_terms, w2_terms)):
                c.wait()
                _store_terms(w, terms, w is w2_t)

        x = res[slot]
        xn = _layernorm(x).astype(_BF16)
        acc_t[...] = x.T

        def part(i, carry):
            chunks = [pl.ds(pl.multiple_of((i * _EDGE_CHUNKS + c) * _FCHUNK, _FCHUNK), _FCHUNK)
                      for c in range(_EDGE_CHUNKS)]
            acc_t[...] += _swiglu_one(xn, w1, w3, w2_t, chunks)
            return carry

        lax.fori_loop(0, n_chunks // _EDGE_CHUNKS, part, 0)

        @pl.when(b == 0)
        def _():
            start_layer(1, acc_t[...].T)
            start_layer(0, x_next_ref[...].astype(_F32).T)

        @pl.when(b > 0)
        def _():
            out_ref[...] = acc_t[...].astype(out_ref.dtype)


@functools.partial(jax.jit, static_argnames=("A_seg_len",))
def pallas_interleave_layers__memory_aug_recurrent_mem_tr__glu_gated_swiglu__prompt_kernel(
    A_x: jax.Array,
    A_mem0: jax.Array,
    A_Wq: jax.Array,
    A_Wk: jax.Array,
    A_Wv: jax.Array,
    A_Wo: jax.Array,
    A_seg_len: int,
    B_x: jax.Array,
    B_w1: jax.Array,
    B_w3: jax.Array,
    B_w2: jax.Array,
):
    del B_x
    batch, seq, d_model = A_x.shape
    n_mem = A_mem0.shape[1]
    _, n_heads, dh = A_Wq.shape
    d_ff = B_w1.shape[1]
    seg = int(A_seg_len)
    assert batch == 1 and seq % _TOK == 0 and _TOK % seg == 0 and seg % 16 == 0
    assert n_mem == 8 and n_heads % _GROUP == 0 and d_ff % (_FCHUNK * _EDGE_CHUNKS) == 0
    d_rest = d_model - 4 * _QUARTER
    assert 0 < d_rest <= 4 * _WCHUNK and d_rest % _WCHUNK == 0 and d_model % 64 == 0
    assert dh == _QUARTER and d_ff % (4 * _PAIR_CHUNK) == 0
    n_blocks = seq // _TOK

    x_t = A_x[0].T
    hbm = pl.BlockSpec(memory_space=pl.ANY)
    out_t = pl.pallas_call(
        functools.partial(_kernel, seg=seg),
        grid=(n_blocks + 1,),
        in_specs=[
            pl.BlockSpec((d_model, _TOK), lambda b: (0, 0)),
            pl.BlockSpec((d_model, _TOK), lambda b: (0, jnp.minimum(b + 1, n_blocks - 1))),
            pl.BlockSpec((n_mem, d_model), lambda b: (0, 0)),
            hbm, hbm, hbm, hbm, hbm, hbm, hbm,
        ],
        out_specs=pl.BlockSpec((d_model, _TOK), lambda b: (0, jnp.maximum(b - 1, 0))),
        out_shape=jax.ShapeDtypeStruct((d_model, seq), A_x.dtype),
        scratch_shapes=[
            pltpu.VMEM((_INFLIGHT + 1, 4, _WCHUNK, n_heads, dh), _BF16),
            pltpu.VMEM((n_heads, d_model, dh), _BF16),
            pltpu.VMEM((3, _PRODUCTS, _QUARTER // 2, n_heads * dh // 4), jnp.uint32),
            pltpu.VMEM((3, d_rest // 2, n_heads * dh), jnp.uint32),
            pltpu.VMEM((_PRODUCTS, n_heads * dh // 8, _QUARTER), jnp.uint32),
            pltpu.VMEM((n_heads * dh // 2, d_rest), jnp.uint32),
            pltpu.VMEM((d_model, d_ff), _BF16),
            pltpu.VMEM((d_model, d_ff), _BF16),
            pltpu.VMEM((d_model, d_ff), _BF16),
            *2 * [pltpu.VMEM((_PRODUCTS, _QUARTER // 2, d_ff // 4), jnp.uint32)],
            pltpu.VMEM((_PRODUCTS, d_model // 8, d_ff // 4), jnp.uint32),
            pltpu.VMEM((2, _TOK, d_model), _F32),
            pltpu.VMEM((2, _TOK, d_model), _F32),
            pltpu.VMEM((2, n_mem, d_model), _F32),
            pltpu.VMEM((d_model, _TOK), _F32),
            pltpu.SemaphoreType.DMA((4 * (_INFLIGHT + 1),)),
            pltpu.SemaphoreType.DMA(()),
            pltpu.SemaphoreType.DMA((3,)),
        ],
        compiler_params=pltpu.CompilerParams(
            dimension_semantics=("arbitrary",),
            vmem_limit_bytes=112 * 1024 * 1024,
        ),
    )(x_t, x_t, A_mem0[0], A_Wq, A_Wk, A_Wv, jnp.transpose(A_Wo, (0, 2, 1)),
      B_w1, B_w3, B_w2.T)
    return out_t.T[None]
```

```python
import functools

import jax
import jax.numpy as jnp
import numpy as np
from jax import lax
import jax.experimental.pallas as pl
import jax.experimental.pallas.tpu as pltpu

_BF16 = jnp.bfloat16
_F32 = jnp.float32
_NT = (((1,), (1,)), ((), ()))
_TOK = 128
_GROUP = 4
_FCHUNK = 512
_WCHUNK = 32
_INFLIGHT = 3
_UNROLL = 1
_EDGE_CHUNKS = 3
_QUARTER = 128
_WO_FROM = 6
_PAIR_CHUNK = 384
_LATER_FROM = 1
_STAGE_ORDER = (((0, 1), 0), ("mix", 1), ((2,), 0), ("scores", 0), ("output", 2))
_MASKED = -1000000000.0


def _layernorm(x):
    m = jnp.mean(x, axis=-1, keepdims=True)
    c = x - m
    v = jnp.mean(c * c, axis=-1, keepdims=True)
    return c * lax.rsqrt(v + 1e-05)


def _dot(a, b):
    return lax.dot_general(a, b, (((1,), (0,)), ((), ())), preferred_element_type=_F32)


def _dot_nt(a, b):
    return lax.dot_general(a, b, _NT, preferred_element_type=_F32)


def _pack(x):
    return pltpu.bitcast(x.astype(_BF16), jnp.uint32)


def _split_words(words):
    return (pltpu.bitcast(words << 16, _F32),
            pltpu.bitcast(words & jnp.uint32(0xFFFF0000), _F32))


def _unpack(words):
    return pltpu.bitcast(words, _BF16)


_SCHEME = (
    "...+.... +.......++..--.. .-......",
    "..+++..+ +.........-..... ..-.+...",
    ".+++.... ....+++......... +..-....",
    ".+.+.+.. ...+.......+...- ...-.-.+",
    "++-..... ......+......... -.+++.--",
    "+...+..+ .+-.......-...+. ..-..++.",
    "+.-..... +.....+......... +.-.....",
    "..++..+. +....-..++..-... -+..+...",
    "+....... .+.............. .++..--.",
    ".+...+.. ....++++...+...- ...+....",
    "++-..+.. ...+..-......... ...++.--",
    "..++.-.. ...++++....+.... ...+-...",
    "+..++..+ +.........-...+. ..+.....",
    ".+.+..-. .....+.......... -+...-.+",
    "..++.... +...---.++...... +...-...",
    "..+...+. +....-..+...-... +-......",
    "......+. .....+...-...... -+..+-..",
    ".....+.. ...+..+-...+.... ...+...-",
    "++-.++-. ...+............ ....-.++",
    "....+..+ .+-.......-..... ..+...-.",
    ".+.+.+.+ ...+.+.....+...- .....+.-",
    "....+.-. ...+......+..... ....+.-.",
    ".....+++ ...+.+.....+.... ....-..+",
    "+...+... ..+.......+...-. .....++.",
    ".......+ .+-+.+....-+.-+- .....-..",
    "..++..++ +..-.-....---... ....-...",
)


def _sum_program(rows):
    n_in = len(rows[0])
    rows = [{i: c for i, c in enumerate(row) if c} for row in rows]
    steps, ready = [], list(range(n_in))

    def emit(a, b, sign):
        steps.append((a, b, sign))
        ready.append(max(ready[a], ready[b]))
        return len(ready) - 1

    while True:
        count = {}
        for row in rows:
            items = sorted(row.items())
            for n, (a, x) in enumerate(items):
                for b, y in items[n + 1:]:
                    count[a, b, x * y] = count.get((a, b, x * y), 0) + 1
        best = max(sorted(count), key=count.get, default=None)
        if best is None or count[best] < 2:
            break
        a, b, sign = best
        new = emit(a, b, sign)
        for row in rows:
            if a in row and b in row and row[a] * row[b] == sign:
                row[new] = row.pop(a)
                del row[b]
    outs = []
    for row in rows:
        items = sorted(row.items(), key=lambda item: (ready[item[0]], item[0]))
        at, sign = items[0]
        for b, y in items[1:]:
            if sign < 0 < y:
                at, sign = emit(b, at, -1), 1
            else:
                at = emit(at, b, sign * y)
        outs.append((at, sign))
    return n_in, steps, ready, outs


def _evaluate(program, make):
    n_in, steps, ready, outs = program
    vals = {}
    for i in range(n_in):
        vals[i] = make(i)
        for n, (a, b, sign) in enumerate(steps):
            if ready[n_in + n] == i:
                vals[n_in + n] = vals[a] + vals[b] if sign > 0 else vals[a] - vals[b]
    return [vals[i] if sign > 0 else -vals[i] for i, sign in outs]


def _programs():
    u, v, w = (np.array([[{"+": 1, ".": 0, "-": -1}[c] for c in line.split()[f]]
                         for line in _SCHEME]) for f in range(3))
    want = np.zeros((8, 16, 8), np.int64)
    for i in range(2):
        for k in range(4):
            for j in range(4):
                want[4 * i + k, 4 * k + j, 4 * i + j] = 1
    assert np.array_equal(np.einsum("ra,rb,rc->abc", u, v, w), want)
    assert np.array_equal(np.einsum("ra,rb,rc->abc", u[:16, :4], v[:16], w[:16, :4]),
                          want[:4, :, :4])
    left = {1: _sum_program(u[:16, :4].tolist()), 2: _sum_program(u.tolist())}
    out = {1: _sum_program(w[:16, :4].T.tolist()), 2: _sum_program(w.T.tolist())}
    return left, _sum_program(v.tolist()), out


_LEFT, _RIGHT, _OUT = _programs()
_PRODUCTS = len(_SCHEME)


def _left_terms(rows):
    blocks = [blk for row in rows for blk in row]
    return _evaluate(_LEFT[len(rows)], blocks.__getitem__)


def _right_terms(blocks):
    return _evaluate(_RIGHT, blocks.__getitem__)


def _combine(n_rows, product):
    c = _evaluate(_OUT[n_rows], product)
    return [c[4 * i:4 * i + 4] for i in range(n_rows)]


def _quarters(x):
    return [x[:, i * _QUARTER:(i + 1) * _QUARTER] for i in range(4)]


def _masks(n_mem, length, n_seq):
    rows = n_seq * length

    def describe(axis):
        i = lax.broadcasted_iota(jnp.int32, (rows, rows), axis)
        second = i >= length
        return jnp.where(second, 1, 0), jnp.where(second, i - length, i)

    (seq_r, idx_r), (seq_c, idx_c) = describe(0), describe(1)
    same = seq_r == seq_c
    keep = same & ((idx_r < n_mem) | (idx_r >= idx_c))
    fill = jnp.where(same, _MASKED, -jnp.inf).astype(_F32)
    return keep, fill


def _attention(hs, keep, fill, qkv, qkv_rest, wo, wo_rest, n_heads, dh):
    scale = dh ** -0.5
    width = _GROUP * dh
    n_groups = n_heads // _GROUP
    n_seq, length = len(hs), hs[0].shape[0]
    heads = [slice(i * dh, (i + 1) * dh) for i in range(_GROUP)]
    lhs_dtype = _BF16 if (n_seq * length) % 16 == 0 else _F32

    h_terms = _left_terms([_quarters(h) for h in hs])
    h_rest = jnp.concatenate([h[:, 4 * _QUARTER:] for h in hs], axis=0).astype(lhs_dtype)

    def project(ws, g):
        c = _combine(n_seq, lambda i: _dot(h_terms[i], jnp.concatenate(
            [_unpack(qkv[w, i, :, g * dh:(g + 1) * dh]) for w in ws], axis=1)))
        return [jnp.concatenate(
            [jnp.concatenate([blk[:, n * dh:(n + 1) * dh] for blk in row], axis=1) for row in c],
            axis=0) + _dot(h_rest, _unpack(qkv_rest[w, :, g * width:(g + 1) * width]))
            for n, w in enumerate(ws)]

    def weights(q, k):
        out = []
        for cols in heads:
            s = jnp.where(keep, _dot_nt(q[:, cols], k[:, cols]) * scale, fill)
            e = jnp.exp(s - jnp.max(s, axis=-1, keepdims=True))
            out.append((e.astype(lhs_dtype), 1.0 / jnp.sum(e, axis=-1, keepdims=True)))
        return out

    def mix(p, v):
        return jnp.concatenate(
            [_dot(e, v[:, cols]) * inv for (e, inv), cols in zip(p, heads)], axis=1)

    def output(o, g):
        terms = _left_terms([_quarters(o[i * length:(i + 1) * length]) for i in range(n_seq)])
        m = [_dot(t, _unpack(wo[i, g * dh // 2:(g + 1) * dh // 2, :]))
             for i, t in enumerate(terms)]
        rest = _unpack(wo_rest[g * width // 2:(g + 1) * width // 2, :])
        return m + [_dot(o.astype(lhs_dtype), rest)]

    proj, p, o, acc = {}, {}, {}, None
    for stage in range(n_groups + max(lag for _, lag in _STAGE_ORDER)):
        for task, lag in _STAGE_ORDER:
            g = stage - lag
            if not 0 <= g < n_groups:
                continue
            if task == "scores":
                p[g] = weights(proj.pop((0, g)), proj.pop((1, g)))
            elif task == "mix":
                o[g] = mix(p.pop(g), proj.pop((2, g)))
            elif task == "output":
                part = output(o.pop(g), g)
                acc = part if acc is None else [x + y for x, y in zip(acc, part)]
            else:
                for w, x in zip(task, project(task, g)):
                    proj[w, g] = x.astype(lhs_dtype if w == 0 else _BF16)
    return [jnp.concatenate([*row, acc[-1][i * length:(i + 1) * length]], axis=1)
            for i, row in enumerate(_combine(n_seq, acc.__getitem__))]


def _silu(x):
    half = 0.5 * x
    return half + half * jnp.tanh(half)


def _swiglu_one(xn, w1, w3, w2_t, chunks):
    acc = hid = None
    for n in range(len(chunks) + 1):
        prev = hid
        if n < len(chunks):
            gate = _silu(_dot(xn, w1[:, chunks[n]]))
            hid = (gate * _dot(xn, w3[:, chunks[n]])).astype(_BF16)
        if n >= 1:
            part = _dot_nt(w2_t[:, chunks[n - 1]], prev)
            acc = part if acc is None else acc + part
    return acc


def _swiglu_pair(xa, xb, w1, w3, w1_terms, w3_terms, w2_terms, side_work):
    quarter = w1.shape[1] // 4
    tok = xa.shape[0]
    x_terms = [t.astype(_BF16) for t in _left_terms([_quarters(xa), _quarters(xb)])]
    x_rest = jnp.concatenate([xa[:, 4 * _QUARTER:], xb[:, 4 * _QUARTER:]], axis=0).astype(_BF16)

    def project(w, terms, lo):
        c = _combine(2, lambda i: _dot(x_terms[i], _unpack(terms[i, :, lo:lo + _QUARTER])))
        rest = [_dot(x_rest, w[4 * _QUARTER:, j * quarter + lo:j * quarter + lo + _QUARTER])
                for j in range(4)]
        return [c[i][j] + rest[j][i * tok:(i + 1) * tok] for i in range(2) for j in range(4)]

    def hidden(lo):
        gates = [_silu(g) for g in project(w1, w1_terms, lo)]
        hid = [g * u for g, u in zip(gates, project(w3, w3_terms, lo))]
        return [t.astype(_BF16) for t in _left_terms([hid[:4], hid[4:]])]

    chunks = list(range(0, quarter, _PAIR_CHUNK))
    acc, hid = [None] * _PRODUCTS, None
    for n in range(len(chunks) + 1):
        prev = hid
        if n < len(chunks):
            tiles = [hidden(lo) for lo in range(chunks[n], chunks[n] + _PAIR_CHUNK, _QUARTER)]
            hid = [jnp.concatenate(t, axis=1) for t in zip(*tiles)]
        if n >= 1:
            cols = slice(chunks[n - 1], chunks[n - 1] + _PAIR_CHUNK)
            for i in range(_PRODUCTS):
                part = _dot_nt(_unpack(w2_terms[i, :, cols]), prev[i])
                acc[i] = part if acc[i] is None else acc[i] + part
        side_work(n)
    return [jnp.concatenate(row, axis=0) for row in _combine(2, acc.__getitem__)]


def _store_terms(w, terms, transposed):
    block_rows, block_cols = 2 * terms.shape[1], terms.shape[2]

    def tile(j, carry):
        def block(r, c, lo):
            rows = pl.ds(pl.multiple_of(r * block_rows + j * 16, 16), 16)
            return pltpu.bitcast(
                w[rows, c * block_cols + lo:c * block_cols + lo + _QUARTER], jnp.uint32)

        for lo in range(0, block_cols, _QUARTER):
            words = [block(n, k, lo) if transposed else block(k, n, lo)
                     for k in range(4) for n in range(4)]
            even, odd = (_right_terms(rows) for rows in zip(*map(_split_words, words)))
            for i, pair in enumerate(zip(even, odd)):
                terms[i, pl.ds(pl.multiple_of(j * 8, 8), 8), lo:lo + _QUARTER] = (
                    pltpu.pack_elementwise(pair, packed_dtype=_BF16))
        return carry

    lax.fori_loop(0, block_rows // 16, tile, 0)


def _load_weights(sources, main, rest, wo_hbm, wo, wo_rest, stage, wo_stage, wsem, osem,
                  later_copies):
    _, n_heads, dh = sources[0].shape
    n_groups = n_heads // _GROUP
    main_chunks = _QUARTER // _WCHUNK
    per_weight = main_chunks + 1
    n_jobs = len(sources) * per_weight
    slots = stage.shape[0]
    rest_parts = 2 * rest.shape[1] // _WCHUNK

    def for_copies(src, job, action):
        c, slot = job % per_weight, job % slots

        def copy(row, n):
            action(pltpu.make_async_copy(src.at[pl.ds(row, _WCHUNK)], stage.at[slot, n],
                                         wsem.at[4 * slot + n]))

        @pl.when(c < main_chunks)
        def _():
            for n in range(4):
                copy(n * _QUARTER + c * _WCHUNK, n)

        @pl.when(c == main_chunks)
        def _():
            for n in range(rest_parts):
                copy(4 * _QUARTER + n * _WCHUNK, n)

    def start(job):
        for i, src in enumerate(sources):
            pl.when(job // per_weight == i)(
                functools.partial(for_copies, src, job, lambda c: c.start()))

    def wait(job):
        for i, src in enumerate(sources):
            pl.when(job // per_weight == i)(
                functools.partial(for_copies, src, job, lambda c: c.wait()))

    def split_heads(slot, n, j):
        rows = pl.ds(pl.multiple_of(j * 16, 16), 16)
        words = jnp.swapaxes(pltpu.bitcast(stage[slot, n, rows], jnp.uint32), 0, 1)
        return [half for p in range(n_heads // 2) for half in _split_words(words[p])]

    def output_group(g, carry):
        heads = [wo_stage[_GROUP * g + i, :4 * _QUARTER].T for i in range(_GROUP)]
        for r in range(0, dh, 16):
            blocks = [blk for h in heads for blk in _quarters(h[r:r + 16].astype(_F32))]
            rows = pl.ds(pl.multiple_of(g * (dh // 2) + r // 2, 8), 8)
            for i, t in enumerate(_right_terms(blocks)):
                wo[i, rows, :] = _pack(t)
        for i in range(_GROUP):
            head = _GROUP * g + i
            wo_rest[pl.ds(pl.multiple_of(head * (dh // 2), dh // 2), dh // 2), :] = _pack(
                wo_stage[head, 4 * _QUARTER:].astype(_F32).T)
        return carry

    wo_copy = pltpu.make_async_copy(wo_hbm, wo_stage, osem)
    lax.fori_loop(0, _INFLIGHT, lambda job, carry: start(job), None)
    wo_copy.start()

    def groups_done(job):
        return n_groups * jnp.maximum(job - _WO_FROM, 0) // (n_jobs - _WO_FROM)

    def run(job, carry):
        which, c, slot = job // per_weight, job % per_weight, job % slots
        wait(job)
        start(job + _INFLIGHT)

        @pl.when(job == n_jobs - _LATER_FROM)
        def _():
            for copy in later_copies:
                copy.start()


        def main_rows(j, carry):
            rows = pl.ds(pl.multiple_of(c * (_WCHUNK // 2) + j * 8, 8), 8)
            parts = [split_heads(slot, n, j) for n in range(4)]
            for g in range(n_groups):
                blocks = [h for part in parts for h in part[_GROUP * g:_GROUP * (g + 1)]]
                for n, t in enumerate(_right_terms(blocks)):
                    main[which, n, rows, g * dh:(g + 1) * dh] = _pack(t)
            return carry

        def rest_rows(j, carry):
            rows = pl.ds(pl.multiple_of(j * 8, 8), 8)
            for h, t in enumerate(split_heads(slot, j // tiles, j % tiles)):
                rest[which, rows, h * dh:(h + 1) * dh] = _pack(t)
            return carry

        tiles = _WCHUNK // 16
        lax.fori_loop(0, jnp.where(c < main_chunks, tiles, 0), main_rows, 0)
        lax.fori_loop(0, jnp.where(c < main_chunks, 0, rest_parts * tiles), rest_rows, 0)
        pl.when(job == _WO_FROM)(wo_copy.wait)
        lax.fori_loop(groups_done(job), groups_done(job + 1), output_group, 0)
        return carry

    lax.fori_loop(0, n_jobs, run, 0)


def _kernel(x0_ref, x_next_ref, mem0_ref, wq_hbm, wk_hbm, wv_hbm, wo_hbm, w1_hbm, w3_hbm,
            w2_hbm, out_ref,
            stage, wo_stage, qkv, qkv_rest, wo, wo_rest,
            w1, w3, w2_t, w1_terms, w3_terms, w2_terms, res, normed, mem, acc_t, wsem, osem, fsem, *, seg):
    b = pl.program_id(0)
    n_blocks = pl.num_programs(0) - 1
    _, n_heads, dh = wq_hbm.shape
    n_mem = mem0_ref.shape[0]
    n_chunks = w1.shape[1] // _FCHUNK
    steps = _TOK // seg
    ffn_copies = [pltpu.make_async_copy(s, d, fsem.at[i])
                  for i, (s, d) in enumerate(((w1_hbm, w1), (w3_hbm, w3), (w2_hbm, w2_t)))]

    def start_layer(slot, x):
        res[slot] = x
        normed[slot] = _layernorm(x)

    @pl.when(b == 0)
    def _():
        _load_weights((wq_hbm, wk_hbm, wv_hbm), qkv, qkv_rest, wo_hbm, wo, wo_rest,
                      stage, wo_stage, wsem, osem, ffn_copies)
        mem[0] = mem0_ref[...].astype(_F32)
        mem[1] = mem0_ref[...].astype(_F32)
        start_layer(0, x0_ref[...].astype(_F32).T)

    def run_attention(first, n_seq, unroll):
        keep, fill = _masks(n_mem, n_mem + seg, n_seq)

        def segment(j):
            rows = pl.ds(pl.multiple_of(j * seg, seg), seg)
            hs = [jnp.concatenate([mem[first + i], normed[first + i, rows]], axis=0)
                  for i in range(n_seq)]
            for i, out in enumerate(_attention(hs, keep, fill, qkv, qkv_rest, wo, wo_rest,
                                               n_heads, dh)):
                mem[first + i] = out[:n_mem]
                res[first + i, rows] += out[n_mem:]

        def step(j, carry):
            for u in range(unroll):
                segment(j * unroll + u)
            return carry

        lax.fori_loop(0, steps // unroll, step, 0)

    both = jnp.logical_and(b > 0, b < n_blocks)

    @pl.when(both)
    def _():
        run_attention(0, 2, _UNROLL)
        x1, x3 = res[0], res[1]

        def side_work(n):
            if n == 0:
                acc_t[...] = x3.T
                res[1] = x1
            if n == 1:
                start_layer(0, x_next_ref[...].astype(_F32).T)

        f2, f4 = _swiglu_pair(_layernorm(x1), _layernorm(x3), w1, w3,
                              w1_terms, w3_terms, w2_terms, side_work)
        start_layer(1, res[1] + f2.T)
        out_ref[...] = (acc_t[...] + f4).astype(out_ref.dtype)

    @pl.when(jnp.logical_not(both))
    def _():
        slot = jnp.where(b == 0, 0, 1)
        run_attention(slot, 1, 1)

        @pl.when(b == 0)
        def _():
            for c, w, terms in zip(ffn_copies, (w1, w3, w2_t), (w1_terms, w3_terms, w2_terms)):
                c.wait()
                _store_terms(w, terms, w is w2_t)

        x = res[slot]
        xn = _layernorm(x).astype(_BF16)
        acc_t[...] = x.T

        def part(i, carry):
            chunks = [pl.ds(pl.multiple_of((i * _EDGE_CHUNKS + c) * _FCHUNK, _FCHUNK), _FCHUNK)
                      for c in range(_EDGE_CHUNKS)]
            acc_t[...] += _swiglu_one(xn, w1, w3, w2_t, chunks)
            return carry

        lax.fori_loop(0, n_chunks // _EDGE_CHUNKS, part, 0)

        @pl.when(b == 0)
        def _():
            start_layer(1, acc_t[...].T)
            start_layer(0, x_next_ref[...].astype(_F32).T)

        @pl.when(b > 0)
        def _():
            out_ref[...] = acc_t[...].astype(out_ref.dtype)


@functools.partial(jax.jit, static_argnames=("A_seg_len",))
def pallas_interleave_layers__memory_aug_recurrent_mem_tr__glu_gated_swiglu__prompt_kernel(
    A_x: jax.Array,
    A_mem0: jax.Array,
    A_Wq: jax.Array,
    A_Wk: jax.Array,
    A_Wv: jax.Array,
    A_Wo: jax.Array,
    A_seg_len: int,
    B_x: jax.Array,
    B_w1: jax.Array,
    B_w3: jax.Array,
    B_w2: jax.Array,
):
    del B_x
    batch, seq, d_model = A_x.shape
    n_mem = A_mem0.shape[1]
    _, n_heads, dh = A_Wq.shape
    d_ff = B_w1.shape[1]
    seg = int(A_seg_len)
    assert batch == 1 and seq % _TOK == 0 and _TOK % seg == 0 and seg % 16 == 0
    assert n_mem == 8 and n_heads % _GROUP == 0 and d_ff % (_FCHUNK * _EDGE_CHUNKS) == 0
    d_rest = d_model - 4 * _QUARTER
    assert 0 < d_rest <= 4 * _WCHUNK and d_rest % _WCHUNK == 0 and d_model % 64 == 0
    assert dh == _QUARTER and d_ff % (4 * _PAIR_CHUNK) == 0
    n_blocks = seq // _TOK

    x_t = A_x[0].T
    hbm = pl.BlockSpec(memory_space=pl.ANY)
    out_t = pl.pallas_call(
        functools.partial(_kernel, seg=seg),
        grid=(n_blocks + 1,),
        in_specs=[
            pl.BlockSpec((d_model, _TOK), lambda b: (0, 0)),
            pl.BlockSpec((d_model, _TOK), lambda b: (0, jnp.minimum(b + 1, n_blocks - 1))),
            pl.BlockSpec((n_mem, d_model), lambda b: (0, 0)),
            hbm, hbm, hbm, hbm, hbm, hbm, hbm,
        ],
        out_specs=pl.BlockSpec((d_model, _TOK), lambda b: (0, jnp.maximum(b - 1, 0))),
        out_shape=jax.ShapeDtypeStruct((d_model, seq), A_x.dtype),
        scratch_shapes=[
            pltpu.VMEM((_INFLIGHT + 1, 4, _WCHUNK, n_heads, dh), _BF16),
            pltpu.VMEM((n_heads, d_model, dh), _BF16),
            pltpu.VMEM((3, _PRODUCTS, _QUARTER // 2, n_heads * dh // 4), jnp.uint32),
            pltpu.VMEM((3, d_rest // 2, n_heads * dh), jnp.uint32),
            pltpu.VMEM((_PRODUCTS, n_heads * dh // 8, _QUARTER), jnp.uint32),
            pltpu.VMEM((n_heads * dh // 2, d_rest), jnp.uint32),
            pltpu.VMEM((d_model, d_ff), _BF16),
            pltpu.VMEM((d_model, d_ff), _BF16),
            pltpu.VMEM((d_model, d_ff), _BF16),
            *2 * [pltpu.VMEM((_PRODUCTS, _QUARTER // 2, d_ff // 4), jnp.uint32)],
            pltpu.VMEM((_PRODUCTS, d_model // 8, d_ff // 4), jnp.uint32),
            pltpu.VMEM((2, _TOK, d_model), _F32),
            pltpu.VMEM((2, _TOK, d_model), _F32),
            pltpu.VMEM((2, n_mem, d_model), _F32),
            pltpu.VMEM((d_model, _TOK), _F32),
            pltpu.SemaphoreType.DMA((4 * (_INFLIGHT + 1),)),
            pltpu.SemaphoreType.DMA(()),
            pltpu.SemaphoreType.DMA((3,)),
        ],
        compiler_params=pltpu.CompilerParams(
            dimension_semantics=("arbitrary",),
            vmem_limit_bytes=112 * 1024 * 1024,
        ),
    )(x_t, x_t, A_mem0[0], A_Wq, A_Wk, A_Wv, jnp.transpose(A_Wo, (0, 2, 1)),
      B_w1, B_w3, B_w2.T)
    return out_t.T[None]
```

```python
import functools

import jax
import jax.numpy as jnp
import numpy as np
from jax import lax
import jax.experimental.pallas as pl
import jax.experimental.pallas.tpu as pltpu

_BF16 = jnp.bfloat16
_F32 = jnp.float32
_NT = (((1,), (1,)), ((), ()))
_TOK = 128
_GROUP = 4
_FCHUNK = 512
_WCHUNK = 32
_INFLIGHT = 3
_UNROLL = 1
_EDGE_CHUNKS = 3
_QUARTER = 128
_WO_FROM = 6
_PAIR_CHUNK = 384
_LATER_FROM = 1
_STAGE_ORDER = (((0, 1), 0), ("mix", 1), ((2,), 0), ("scores", 0), ("output", 2))
_MASKED = -1000000000.0


def _layernorm(x):
    m = jnp.mean(x, axis=-1, keepdims=True)
    c = x - m
    v = jnp.mean(c * c, axis=-1, keepdims=True)
    return c * lax.rsqrt(v + 1e-05)


def _dot(a, b):
    return lax.dot_general(a, b, (((1,), (0,)), ((), ())), preferred_element_type=_F32)


def _dot_nt(a, b):
    return lax.dot_general(a, b, _NT, preferred_element_type=_F32)


def _pack(x):
    return pltpu.bitcast(x.astype(_BF16), jnp.uint32)


def _split_words(words):
    return (pltpu.bitcast(words << 16, _F32),
            pltpu.bitcast(words & jnp.uint32(0xFFFF0000), _F32))


def _unpack(words):
    return pltpu.bitcast(words, _BF16)


_SCHEME = (
    "...+.... +.......++..--.. .-......",
    "..+++..+ +.........-..... ..-.+...",
    ".+++.... ....+++......... +..-....",
    ".+.+.+.. ...+.......+...- ...-.-.+",
    "++-..... ......+......... -.+++.--",
    "+...+..+ .+-.......-...+. ..-..++.",
    "+.-..... +.....+......... +.-.....",
    "..++..+. +....-..++..-... -+..+...",
    "+....... .+.............. .++..--.",
    ".+...+.. ....++++...+...- ...+....",
    "++-..+.. ...+..-......... ...++.--",
    "..++.-.. ...++++....+.... ...+-...",
    "+..++..+ +.........-...+. ..+.....",
    ".+.+..-. .....+.......... -+...-.+",
    "..++.... +...---.++...... +...-...",
    "..+...+. +....-..+...-... +-......",
    "......+. .....+...-...... -+..+-..",
    ".....+.. ...+..+-...+.... ...+...-",
    "++-.++-. ...+............ ....-.++",
    "....+..+ .+-.......-..... ..+...-.",
    ".+.+.+.+ ...+.+.....+...- .....+.-",
    "....+.-. ...+......+..... ....+.-.",
    ".....+++ ...+.+.....+.... ....-..+",
    "+...+... ..+.......+...-. .....++.",
    ".......+ .+-+.+....-+.-+- .....-..",
    "..++..++ +..-.-....---... ....-...",
)


def _sum_program(rows):
    n_in = len(rows[0])
    rows = [{i: c for i, c in enumerate(row) if c} for row in rows]
    steps, ready = [], list(range(n_in))

    def emit(a, b, sign):
        steps.append((a, b, sign))
        ready.append(max(ready[a], ready[b]))
        return len(ready) - 1

    while True:
        count = {}
        for row in rows:
            items = sorted(row.items())
            for n, (a, x) in enumerate(items):
                for b, y in items[n + 1:]:
                    count[a, b, x * y] = count.get((a, b, x * y), 0) + 1
        best = max(sorted(count), key=count.get, default=None)
        if best is None or count[best] < 2:
            break
        a, b, sign = best
        new = emit(a, b, sign)
        for row in rows:
            if a in row and b in row and row[a] * row[b] == sign:
                row[new] = row.pop(a)
                del row[b]
    outs = []
    for row in rows:
        items = sorted(row.items(), key=lambda item: (ready[item[0]], item[0]))
        at, sign = items[0]
        for b, y in items[1:]:
            if sign < 0 < y:
                at, sign = emit(b, at, -1), 1
            else:
                at = emit(at, b, sign * y)
        outs.append((at, sign))
    return n_in, steps, ready, outs


def _evaluate(program, make):
    n_in, steps, ready, outs = program
    vals = {}
    for i in range(n_in):
        vals[i] = make(i)
        for n, (a, b, sign) in enumerate(steps):
            if ready[n_in + n] == i:
                vals[n_in + n] = vals[a] + vals[b] if sign > 0 else vals[a] - vals[b]
    return [vals[i] if sign > 0 else -vals[i] for i, sign in outs]


def _programs():
    u, v, w = (np.array([[{"+": 1, ".": 0, "-": -1}[c] for c in line.split()[f]]
                         for line in _SCHEME]) for f in range(3))
    want = np.zeros((8, 16, 8), np.int64)
    for i in range(2):
        for k in range(4):
            for j in range(4):
                want[4 * i + k, 4 * k + j, 4 * i + j] = 1
    assert np.array_equal(np.einsum("ra,rb,rc->abc", u, v, w), want)
    assert np.array_equal(np.einsum("ra,rb,rc->abc", u[:16, :4], v[:16], w[:16, :4]),
                          want[:4, :, :4])
    left = {1: _sum_program(u[:16, :4].tolist()), 2: _sum_program(u.tolist())}
    out = {1: _sum_program(w[:16, :4].T.tolist()), 2: _sum_program(w.T.tolist())}
    return left, _sum_program(v.tolist()), out


_LEFT, _RIGHT, _OUT = _programs()
_PRODUCTS = len(_SCHEME)


def _left_terms(rows):
    blocks = [blk for row in rows for blk in row]
    return _evaluate(_LEFT[len(rows)], blocks.__getitem__)


def _right_terms(blocks):
    return _evaluate(_RIGHT, blocks.__getitem__)


def _combine(n_rows, product):
    c = _evaluate(_OUT[n_rows], product)
    return [c[4 * i:4 * i + 4] for i in range(n_rows)]


def _quarters(x):
    return [x[:, i * _QUARTER:(i + 1) * _QUARTER] for i in range(4)]


def _masks(n_mem, length, n_seq):
    rows = n_seq * length

    def describe(axis):
        i = lax.broadcasted_iota(jnp.int32, (rows, rows), axis)
        second = i >= length
        return jnp.where(second, 1, 0), jnp.where(second, i - length, i)

    (seq_r, idx_r), (seq_c, idx_c) = describe(0), describe(1)
    same = seq_r == seq_c
    keep = same & ((idx_r < n_mem) | (idx_r >= idx_c))
    fill = jnp.where(same, _MASKED, -jnp.inf).astype(_F32)
    return keep, fill


def _attention(hs, keep, fill, qkv, qkv_rest, wo, wo_rest, n_heads, dh):
    scale = dh ** -0.5
    width = _GROUP * dh
    n_groups = n_heads // _GROUP
    n_seq, length = len(hs), hs[0].shape[0]
    heads = [slice(i * dh, (i + 1) * dh) for i in range(_GROUP)]
    lhs_dtype = _BF16 if (n_seq * length) % 16 == 0 else _F32

    h_terms = _left_terms([_quarters(h) for h in hs])
    h_rest = jnp.concatenate([h[:, 4 * _QUARTER:] for h in hs], axis=0).astype(lhs_dtype)

    def project(ws, g):
        c = _combine(n_seq, lambda i: _dot(h_terms[i], jnp.concatenate(
            [_unpack(qkv[w, g, i]) for w in ws], axis=1)))
        return [jnp.concatenate(
            [jnp.concatenate([blk[:, n * dh:(n + 1) * dh] for blk in row], axis=1) for row in c],
            axis=0) + _dot(h_rest, jnp.concatenate(
                [_unpack(qkv_rest[w, g * _GROUP + i]) for i in range(_GROUP)], axis=1))
            for n, w in enumerate(ws)]

    def weights(q, k):
        out = []
        for cols in heads:
            s = jnp.where(keep, _dot_nt(q[:, cols], k[:, cols]) * scale, fill)
            e = jnp.exp(s - jnp.max(s, axis=-1, keepdims=True))
            out.append((e.astype(lhs_dtype), 1.0 / jnp.sum(e, axis=-1, keepdims=True)))
        return out

    def mix(p, v):
        return jnp.concatenate(
            [_dot(e, v[:, cols]) * inv for (e, inv), cols in zip(p, heads)], axis=1)

    def output(o, g):
        terms = _left_terms([_quarters(o[i * length:(i + 1) * length]) for i in range(n_seq)])
        m = [_dot(t, _unpack(wo[i, g * dh // 2:(g + 1) * dh // 2, :]))
             for i, t in enumerate(terms)]
        rest = _unpack(wo_rest[g * width // 2:(g + 1) * width // 2, :])
        return m + [_dot(o.astype(lhs_dtype), rest)]

    proj, p, o, acc = {}, {}, {}, None
    for stage in range(n_groups + max(lag for _, lag in _STAGE_ORDER)):
        for task, lag in _STAGE_ORDER:
            g = stage - lag
            if not 0 <= g < n_groups:
                continue
            if task == "scores":
                p[g] = weights(proj.pop((0, g)), proj.pop((1, g)))
            elif task == "mix":
                o[g] = mix(p.pop(g), proj.pop((2, g)))
            elif task == "output":
                part = output(o.pop(g), g)
                acc = part if acc is None else [x + y for x, y in zip(acc, part)]
            else:
                for w, x in zip(task, project(task, g)):
                    proj[w, g] = x.astype(lhs_dtype if w == 0 else _BF16)
    return [jnp.concatenate([*row, acc[-1][i * length:(i + 1) * length]], axis=1)
            for i, row in enumerate(_combine(n_seq, acc.__getitem__))]


def _silu(x):
    half = 0.5 * x
    return half + half * jnp.tanh(half)


def _swiglu_one(xn, w1, w3, w2_t, chunks):
    acc = hid = None
    for n in range(len(chunks) + 1):
        prev = hid
        if n < len(chunks):
            gate = _silu(_dot(xn, w1[:, chunks[n]]))
            hid = (gate * _dot(xn, w3[:, chunks[n]])).astype(_BF16)
        if n >= 1:
            part = _dot_nt(w2_t[:, chunks[n - 1]], prev)
            acc = part if acc is None else acc + part
    return acc


def _swiglu_pair(xa, xb, w1, w3, w1_terms, w3_terms, w2_terms, side_work):
    quarter = w1.shape[1] // 4
    tok = xa.shape[0]
    x_terms = [t.astype(_BF16) for t in _left_terms([_quarters(xa), _quarters(xb)])]
    x_rest = jnp.concatenate([xa[:, 4 * _QUARTER:], xb[:, 4 * _QUARTER:]], axis=0).astype(_BF16)

    def project(w, terms, lo):
        c = _combine(2, lambda i: _dot(x_terms[i], _unpack(terms[lo // _QUARTER, i])))
        rest = [_dot(x_rest, w[4 * _QUARTER:, j * quarter + lo:j * quarter + lo + _QUARTER])
                for j in range(4)]
        return [c[i][j] + rest[j][i * tok:(i + 1) * tok] for i in range(2) for j in range(4)]

    def hidden(lo):
        gates = [_silu(g) for g in project(w1, w1_terms, lo)]
        hid = [g * u for g, u in zip(gates, project(w3, w3_terms, lo))]
        return [t.astype(_BF16) for t in _left_terms([hid[:4], hid[4:]])]

    chunks = list(range(0, quarter, _PAIR_CHUNK))
    acc, hid = [None] * _PRODUCTS, None
    for n in range(len(chunks) + 1):
        prev = hid
        if n < len(chunks):
            tiles = [hidden(lo) for lo in range(chunks[n], chunks[n] + _PAIR_CHUNK, _QUARTER)]
            hid = [jnp.concatenate(t, axis=1) for t in zip(*tiles)]
        if n >= 1:
            first = chunks[n - 1] // _QUARTER
            for i in range(_PRODUCTS):
                left = [_unpack(w2_terms[first + c, i]) for c in range(_PAIR_CHUNK // _QUARTER)]
                part = _dot_nt(jnp.concatenate(left, axis=1), prev[i])
                acc[i] = part if acc[i] is None else acc[i] + part
        side_work(n)
    return [jnp.concatenate(row, axis=0) for row in _combine(2, acc.__getitem__)]


def _store_terms(w, terms, transposed):
    block_rows, block_cols = 2 * terms.shape[2], terms.shape[0] * _QUARTER

    def tile(j, carry):
        def block(r, c, lo):
            rows = pl.ds(pl.multiple_of(r * block_rows + j * 16, 16), 16)
            return pltpu.bitcast(
                w[rows, c * block_cols + lo:c * block_cols + lo + _QUARTER], jnp.uint32)

        for lo in range(0, block_cols, _QUARTER):
            words = [block(n, k, lo) if transposed else block(k, n, lo)
                     for k in range(4) for n in range(4)]
            even, odd = (_right_terms(rows) for rows in zip(*map(_split_words, words)))
            for i, pair in enumerate(zip(even, odd)):
                terms[lo // _QUARTER, i, pl.ds(pl.multiple_of(j * 8, 8), 8)] = (
                    pltpu.pack_elementwise(pair, packed_dtype=_BF16))
        return carry

    lax.fori_loop(0, block_rows // 16, tile, 0)


def _load_weights(sources, main, rest, wo_hbm, wo, wo_rest, stage, wo_stage, wsem, osem,
                  later_copies):
    _, n_heads, dh = sources[0].shape
    n_groups = n_heads // _GROUP
    main_chunks = _QUARTER // _WCHUNK
    per_weight = main_chunks + 1
    n_jobs = len(sources) * per_weight
    slots = stage.shape[0]
    rest_parts = 2 * rest.shape[2] // _WCHUNK

    def for_copies(src, job, action):
        c, slot = job % per_weight, job % slots

        def copy(row, n):
            action(pltpu.make_async_copy(src.at[pl.ds(row, _WCHUNK)], stage.at[slot, n],
                                         wsem.at[4 * slot + n]))

        @pl.when(c < main_chunks)
        def _():
            for n in range(4):
                copy(n * _QUARTER + c * _WCHUNK, n)

        @pl.when(c == main_chunks)
        def _():
            for n in range(rest_parts):
                copy(4 * _QUARTER + n * _WCHUNK, n)

    def start(job):
        for i, src in enumerate(sources):
            pl.when(job // per_weight == i)(
                functools.partial(for_copies, src, job, lambda c: c.start()))

    def wait(job):
        for i, src in enumerate(sources):
            pl.when(job // per_weight == i)(
                functools.partial(for_copies, src, job, lambda c: c.wait()))

    def split_heads(slot, n, j):
        rows = pl.ds(pl.multiple_of(j * 16, 16), 16)
        words = jnp.swapaxes(pltpu.bitcast(stage[slot, n, rows], jnp.uint32), 0, 1)
        return [half for p in range(n_heads // 2) for half in _split_words(words[p])]

    def output_group(g, carry):
        heads = [wo_stage[_GROUP * g + i, :4 * _QUARTER].T for i in range(_GROUP)]
        for r in range(0, dh, 16):
            blocks = [blk for h in heads for blk in _quarters(h[r:r + 16].astype(_F32))]
            rows = pl.ds(pl.multiple_of(g * (dh // 2) + r // 2, 8), 8)
            for i, t in enumerate(_right_terms(blocks)):
                wo[i, rows, :] = _pack(t)
        for i in range(_GROUP):
            head = _GROUP * g + i
            wo_rest[pl.ds(pl.multiple_of(head * (dh // 2), dh // 2), dh // 2), :] = _pack(
                wo_stage[head, 4 * _QUARTER:].astype(_F32).T)
        return carry

    wo_copy = pltpu.make_async_copy(wo_hbm, wo_stage, osem)
    lax.fori_loop(0, _INFLIGHT, lambda job, carry: start(job), None)
    wo_copy.start()

    def groups_done(job):
        return n_groups * jnp.maximum(job - _WO_FROM, 0) // (n_jobs - _WO_FROM)

    def run(job, carry):
        which, c, slot = job // per_weight, job % per_weight, job % slots
        wait(job)
        start(job + _INFLIGHT)

        @pl.when(job == n_jobs - _LATER_FROM)
        def _():
            for copy in later_copies:
                copy.start()


        def main_rows(j, carry):
            rows = pl.ds(pl.multiple_of(c * (_WCHUNK // 2) + j * 8, 8), 8)
            parts = [split_heads(slot, n, j) for n in range(4)]
            for g in range(n_groups):
                blocks = [h for part in parts for h in part[_GROUP * g:_GROUP * (g + 1)]]
                for n, t in enumerate(_right_terms(blocks)):
                    main[which, g, n, rows] = _pack(t)
            return carry

        def rest_rows(j, carry):
            rows = pl.ds(pl.multiple_of(j * 8, 8), 8)
            for h, t in enumerate(split_heads(slot, j // tiles, j % tiles)):
                rest[which, h, rows] = _pack(t)
            return carry

        tiles = _WCHUNK // 16
        lax.fori_loop(0, jnp.where(c < main_chunks, tiles, 0), main_rows, 0)
        lax.fori_loop(0, jnp.where(c < main_chunks, 0, rest_parts * tiles), rest_rows, 0)
        pl.when(job == _WO_FROM)(wo_copy.wait)
        lax.fori_loop(groups_done(job), groups_done(job + 1), output_group, 0)
        return carry

    lax.fori_loop(0, n_jobs, run, 0)


def _kernel(x0_ref, x_next_ref, mem0_ref, wq_hbm, wk_hbm, wv_hbm, wo_hbm, w1_hbm, w3_hbm,
            w2_hbm, out_ref,
            stage, wo_stage, qkv, qkv_rest, wo, wo_rest,
            w1, w3, w2_t, w1_terms, w3_terms, w2_terms, res, normed, mem, acc_t, wsem, osem, fsem, *, seg):
    b = pl.program_id(0)
    n_blocks = pl.num_programs(0) - 1
    _, n_heads, dh = wq_hbm.shape
    n_mem = mem0_ref.shape[0]
    n_chunks = w1.shape[1] // _FCHUNK
    steps = _TOK // seg
    ffn_copies = [pltpu.make_async_copy(s, d, fsem.at[i])
                  for i, (s, d) in enumerate(((w1_hbm, w1), (w3_hbm, w3), (w2_hbm, w2_t)))]

    def start_layer(slot, x):
        res[slot] = x
        normed[slot] = _layernorm(x)

    @pl.when(b == 0)
    def _():
        _load_weights((wq_hbm, wk_hbm, wv_hbm), qkv, qkv_rest, wo_hbm, wo, wo_rest,
                      stage, wo_stage, wsem, osem, ffn_copies)
        mem[0] = mem0_ref[...].astype(_F32)
        mem[1] = mem0_ref[...].astype(_F32)
        start_layer(0, x0_ref[...].astype(_F32).T)

    def run_attention(first, n_seq, unroll):
        keep, fill = _masks(n_mem, n_mem + seg, n_seq)

        def segment(j):
            rows = pl.ds(pl.multiple_of(j * seg, seg), seg)
            hs = [jnp.concatenate([mem[first + i], normed[first + i, rows]], axis=0)
                  for i in range(n_seq)]
            for i, out in enumerate(_attention(hs, keep, fill, qkv, qkv_rest, wo, wo_rest,
                                               n_heads, dh)):
                mem[first + i] = out[:n_mem]
                res[first + i, rows] += out[n_mem:]

        def step(j, carry):
            for u in range(unroll):
                segment(j * unroll + u)
            return carry

        lax.fori_loop(0, steps // unroll, step, 0)

    both = jnp.logical_and(b > 0, b < n_blocks)

    @pl.when(both)
    def _():
        run_attention(0, 2, _UNROLL)
        x1, x3 = res[0], res[1]

        def side_work(n):
            if n == 0:
                acc_t[...] = x3.T
                res[1] = x1
            if n == 1:
                start_layer(0, x_next_ref[...].astype(_F32).T)

        f2, f4 = _swiglu_pair(_layernorm(x1), _layernorm(x3), w1, w3,
                              w1_terms, w3_terms, w2_terms, side_work)
        start_layer(1, res[1] + f2.T)
        out_ref[...] = (acc_t[...] + f4).astype(out_ref.dtype)

    @pl.when(jnp.logical_not(both))
    def _():
        slot = jnp.where(b == 0, 0, 1)
        run_attention(slot, 1, 1)

        @pl.when(b == 0)
        def _():
            for c, w, terms in zip(ffn_copies, (w1, w3, w2_t), (w1_terms, w3_terms, w2_terms)):
                c.wait()
                _store_terms(w, terms, w is w2_t)

        x = res[slot]
        xn = _layernorm(x).astype(_BF16)
        acc_t[...] = x.T

        def part(i, carry):
            chunks = [pl.ds(pl.multiple_of((i * _EDGE_CHUNKS + c) * _FCHUNK, _FCHUNK), _FCHUNK)
                      for c in range(_EDGE_CHUNKS)]
            acc_t[...] += _swiglu_one(xn, w1, w3, w2_t, chunks)
            return carry

        lax.fori_loop(0, n_chunks // _EDGE_CHUNKS, part, 0)

        @pl.when(b == 0)
        def _():
            start_layer(1, acc_t[...].T)
            start_layer(0, x_next_ref[...].astype(_F32).T)

        @pl.when(b > 0)
        def _():
            out_ref[...] = acc_t[...].astype(out_ref.dtype)


@functools.partial(jax.jit, static_argnames=("A_seg_len",))
def pallas_interleave_layers__memory_aug_recurrent_mem_tr__glu_gated_swiglu__prompt_kernel(
    A_x: jax.Array,
    A_mem0: jax.Array,
    A_Wq: jax.Array,
    A_Wk: jax.Array,
    A_Wv: jax.Array,
    A_Wo: jax.Array,
    A_seg_len: int,
    B_x: jax.Array,
    B_w1: jax.Array,
    B_w3: jax.Array,
    B_w2: jax.Array,
):
    del B_x
    batch, seq, d_model = A_x.shape
    n_mem = A_mem0.shape[1]
    _, n_heads, dh = A_Wq.shape
    d_ff = B_w1.shape[1]
    seg = int(A_seg_len)
    assert batch == 1 and seq % _TOK == 0 and _TOK % seg == 0 and seg % 16 == 0
    assert n_mem == 8 and n_heads % _GROUP == 0 and d_ff % (_FCHUNK * _EDGE_CHUNKS) == 0
    d_rest = d_model - 4 * _QUARTER
    assert 0 < d_rest <= 4 * _WCHUNK and d_rest % _WCHUNK == 0 and d_model % 64 == 0
    assert dh == _QUARTER and d_ff % (4 * _PAIR_CHUNK) == 0
    ff_tiles = d_ff // (4 * _QUARTER)
    n_blocks = seq // _TOK

    x_t = A_x[0].T
    hbm = pl.BlockSpec(memory_space=pl.ANY)
    out_t = pl.pallas_call(
        functools.partial(_kernel, seg=seg),
        grid=(n_blocks + 1,),
        in_specs=[
            pl.BlockSpec((d_model, _TOK), lambda b: (0, 0)),
            pl.BlockSpec((d_model, _TOK), lambda b: (0, jnp.minimum(b + 1, n_blocks - 1))),
            pl.BlockSpec((n_mem, d_model), lambda b: (0, 0)),
            hbm, hbm, hbm, hbm, hbm, hbm, hbm,
        ],
        out_specs=pl.BlockSpec((d_model, _TOK), lambda b: (0, jnp.maximum(b - 1, 0))),
        out_shape=jax.ShapeDtypeStruct((d_model, seq), A_x.dtype),
        scratch_shapes=[
            pltpu.VMEM((_INFLIGHT + 1, 4, _WCHUNK, n_heads, dh), _BF16),
            pltpu.VMEM((n_heads, d_model, dh), _BF16),
            pltpu.VMEM((3, n_heads // _GROUP, _PRODUCTS, _QUARTER // 2, dh), jnp.uint32),
            pltpu.VMEM((3, n_heads, d_rest // 2, dh), jnp.uint32),
            pltpu.VMEM((_PRODUCTS, n_heads * dh // 8, _QUARTER), jnp.uint32),
            pltpu.VMEM((n_heads * dh // 2, d_rest), jnp.uint32),
            pltpu.VMEM((d_model, d_ff), _BF16),
            pltpu.VMEM((d_model, d_ff), _BF16),
            pltpu.VMEM((d_model, d_ff), _BF16),
            *2 * [pltpu.VMEM((ff_tiles, _PRODUCTS, _QUARTER // 2, _QUARTER), jnp.uint32)],
            pltpu.VMEM((ff_tiles, _PRODUCTS, d_model // 8, _QUARTER), jnp.uint32),
            pltpu.VMEM((2, _TOK, d_model), _F32),
            pltpu.VMEM((2, _TOK, d_model), _F32),
            pltpu.VMEM((2, n_mem, d_model), _F32),
            pltpu.VMEM((d_model, _TOK), _F32),
            pltpu.SemaphoreType.DMA((4 * (_INFLIGHT + 1),)),
            pltpu.SemaphoreType.DMA(()),
            pltpu.SemaphoreType.DMA((3,)),
        ],
        compiler_params=pltpu.CompilerParams(
            dimension_semantics=("arbitrary",),
            vmem_limit_bytes=112 * 1024 * 1024,
        ),
    )(x_t, x_t, A_mem0[0], A_Wq, A_Wk, A_Wv, jnp.transpose(A_Wo, (0, 2, 1)),
      B_w1, B_w3, B_w2.T)
    return out_t.T[None]
```

```python
import functools

import jax
import jax.numpy as jnp
import numpy as np
from jax import lax
import jax.experimental.pallas as pl
import jax.experimental.pallas.tpu as pltpu

_BF16 = jnp.bfloat16
_F32 = jnp.float32
_NT = (((1,), (1,)), ((), ()))
_TOK = 128
_GROUP = 4
_FCHUNK = 512
_WCHUNK = 32
_INFLIGHT = 3
_EDGE_CHUNKS = 3
_QUARTER = 128
_WO_FROM = 6
_PAIR_CHUNK = 384
_LATER_FROM = 1
_STAGE_ORDER = (((0, 1), 0), ("mix", 1), ((2,), 0), ("scores", 0), ("output", 2))
_MASKED = -1000000000.0


def _layernorm(x):
    m = jnp.mean(x, axis=-1, keepdims=True)
    c = x - m
    v = jnp.mean(c * c, axis=-1, keepdims=True)
    return c * lax.rsqrt(v + 1e-05)


def _dot(a, b):
    return lax.dot_general(a, b, (((1,), (0,)), ((), ())), preferred_element_type=_F32)


def _dot_nt(a, b):
    return lax.dot_general(a, b, _NT, preferred_element_type=_F32)


def _pack(x):
    return pltpu.bitcast(x.astype(_BF16), jnp.uint32)


def _split_words(words):
    return (pltpu.bitcast(words << 16, _F32),
            pltpu.bitcast(words & jnp.uint32(0xFFFF0000), _F32))


def _unpack(words):
    return pltpu.bitcast(words, _BF16)


_SCHEME = (
    "...+.... +.......++..--.. .-......",
    "..+++..+ +.........-..... ..-.+...",
    ".+++.... ....+++......... +..-....",
    ".+.+.+.. ...+.......+...- ...-.-.+",
    "++-..... ......+......... -.+++.--",
    "+...+..+ .+-.......-...+. ..-..++.",
    "+.-..... +.....+......... +.-.....",
    "..++..+. +....-..++..-... -+..+...",
    "+....... .+.............. .++..--.",
    ".+...+.. ....++++...+...- ...+....",
    "++-..+.. ...+..-......... ...++.--",
    "..++.-.. ...++++....+.... ...+-...",
    "+..++..+ +.........-...+. ..+.....",
    ".+.+..-. .....+.......... -+...-.+",
    "..++.... +...---.++...... +...-...",
    "..+...+. +....-..+...-... +-......",
    "......+. .....+...-...... -+..+-..",
    ".....+.. ...+..+-...+.... ...+...-",
    "++-.++-. ...+............ ....-.++",
    "....+..+ .+-.......-..... ..+...-.",
    ".+.+.+.+ ...+.+.....+...- .....+.-",
    "....+.-. ...+......+..... ....+.-.",
    ".....+++ ...+.+.....+.... ....-..+",
    "+...+... ..+.......+...-. .....++.",
    ".......+ .+-+.+....-+.-+- .....-..",
    "..++..++ +..-.-....---... ....-...",
)


def _sum_program(rows):
    n_in = len(rows[0])
    rows = [{i: c for i, c in enumerate(row) if c} for row in rows]
    steps, ready = [], list(range(n_in))

    def emit(a, b, sign):
        steps.append((a, b, sign))
        ready.append(max(ready[a], ready[b]))
        return len(ready) - 1

    while True:
        count = {}
        for row in rows:
            items = sorted(row.items())
            for n, (a, x) in enumerate(items):
                for b, y in items[n + 1:]:
                    count[a, b, x * y] = count.get((a, b, x * y), 0) + 1
        best = max(sorted(count), key=count.get, default=None)
        if best is None or count[best] < 2:
            break
        a, b, sign = best
        new = emit(a, b, sign)
        for row in rows:
            if a in row and b in row and row[a] * row[b] == sign:
                row[new] = row.pop(a)
                del row[b]
    outs = []
    for row in rows:
        items = sorted(row.items(), key=lambda item: (ready[item[0]], item[0]))
        at, sign = items[0]
        for b, y in items[1:]:
            if sign < 0 < y:
                at, sign = emit(b, at, -1), 1
            else:
                at = emit(at, b, sign * y)
        outs.append((at, sign))
    return n_in, steps, ready, outs


def _evaluate(program, make):
    n_in, steps, ready, outs = program
    vals = {}
    for i in range(n_in):
        vals[i] = make(i)
        for n, (a, b, sign) in enumerate(steps):
            if ready[n_in + n] == i:
                vals[n_in + n] = vals[a] + vals[b] if sign > 0 else vals[a] - vals[b]
    return [vals[i] if sign > 0 else -vals[i] for i, sign in outs]


def _programs():
    u, v, w = (np.array([[{"+": 1, ".": 0, "-": -1}[c] for c in line.split()[f]]
                         for line in _SCHEME]) for f in range(3))
    want = np.zeros((8, 16, 8), np.int64)
    for i in range(2):
        for k in range(4):
            for j in range(4):
                want[4 * i + k, 4 * k + j, 4 * i + j] = 1
    assert np.array_equal(np.einsum("ra,rb,rc->abc", u, v, w), want)
    assert np.array_equal(np.einsum("ra,rb,rc->abc", u[:16, :4], v[:16], w[:16, :4]),
                          want[:4, :, :4])
    left = {1: _sum_program(u[:16, :4].tolist()), 2: _sum_program(u.tolist())}
    out = {1: _sum_program(w[:16, :4].T.tolist()), 2: _sum_program(w.T.tolist())}
    return left, _sum_program(v.tolist()), out


_LEFT, _RIGHT, _OUT = _programs()
_PRODUCTS = len(_SCHEME)


def _left_terms(rows):
    blocks = [blk for row in rows for blk in row]
    return _evaluate(_LEFT[len(rows)], blocks.__getitem__)


def _right_terms(blocks):
    return _evaluate(_RIGHT, blocks.__getitem__)


def _combine(n_rows, product):
    c = _evaluate(_OUT[n_rows], product)
    return [c[4 * i:4 * i + 4] for i in range(n_rows)]


def _quarters(x):
    return [x[:, i * _QUARTER:(i + 1) * _QUARTER] for i in range(4)]


def _masks(n_mem, length, n_seq):
    rows = n_seq * length

    def describe(axis):
        i = lax.broadcasted_iota(jnp.int32, (rows, rows), axis)
        second = i >= length
        return jnp.where(second, 1, 0), jnp.where(second, i - length, i)

    (seq_r, idx_r), (seq_c, idx_c) = describe(0), describe(1)
    same = seq_r == seq_c
    keep = same & ((idx_r < n_mem) | (idx_r >= idx_c))
    fill = jnp.where(same, _MASKED, -jnp.inf).astype(_F32)
    return keep, fill


def _attention(hs, keep, fill, qkv, qkv_rest, wo, wo_rest, n_heads, dh):
    scale = dh ** -0.5
    width = _GROUP * dh
    n_groups = n_heads // _GROUP
    n_seq, length = len(hs), hs[0].shape[0]
    heads = [slice(i * dh, (i + 1) * dh) for i in range(_GROUP)]
    lhs_dtype = _BF16 if (n_seq * length) % 16 == 0 else _F32

    h_terms = _left_terms([_quarters(h) for h in hs])
    h_rest = jnp.concatenate([h[:, 4 * _QUARTER:] for h in hs], axis=0).astype(lhs_dtype)

    def project(ws, g):
        c = _combine(n_seq, lambda i: _dot(h_terms[i], jnp.concatenate(
            [_unpack(qkv[w, g, i]) for w in ws], axis=1)))
        return [jnp.concatenate(
            [jnp.concatenate([blk[:, n * dh:(n + 1) * dh] for blk in row], axis=1) for row in c],
            axis=0) + _dot(h_rest, jnp.concatenate(
                [_unpack(qkv_rest[w, g * _GROUP + i]) for i in range(_GROUP)], axis=1))
            for n, w in enumerate(ws)]

    def weights(q, k):
        out = []
        for cols in heads:
            s = jnp.where(keep, _dot_nt(q[:, cols], k[:, cols]) * scale, fill)
            e = jnp.exp(s - jnp.max(s, axis=-1, keepdims=True))
            out.append((e.astype(lhs_dtype), 1.0 / jnp.sum(e, axis=-1, keepdims=True)))
        return out

    def mix(p, v):
        return jnp.concatenate(
            [_dot(e, v[:, cols]) * inv for (e, inv), cols in zip(p, heads)], axis=1)

    def output(o, g):
        terms = _left_terms([_quarters(o[i * length:(i + 1) * length]) for i in range(n_seq)])
        m = [_dot(t, _unpack(wo[i, g * dh // 2:(g + 1) * dh // 2, :]))
             for i, t in enumerate(terms)]
        rest = _unpack(wo_rest[g * width // 2:(g + 1) * width // 2, :])
        return m + [_dot(o.astype(lhs_dtype), rest)]

    proj, p, o, acc = {}, {}, {}, None
    for stage in range(n_groups + max(lag for _, lag in _STAGE_ORDER)):
        for task, lag in _STAGE_ORDER:
            g = stage - lag
            if not 0 <= g < n_groups:
                continue
            if task == "scores":
                p[g] = weights(proj.pop((0, g)), proj.pop((1, g)))
            elif task == "mix":
                o[g] = mix(p.pop(g), proj.pop((2, g)))
            elif task == "output":
                part = output(o.pop(g), g)
                acc = part if acc is None else [x + y for x, y in zip(acc, part)]
            else:
                for w, x in zip(task, project(task, g)):
                    proj[w, g] = x.astype(lhs_dtype if w == 0 else _BF16)
    return [jnp.concatenate([*row, acc[-1][i * length:(i + 1) * length]], axis=1)
            for i, row in enumerate(_combine(n_seq, acc.__getitem__))]


def _silu(x):
    half = 0.5 * x
    return half + half * jnp.tanh(half)


def _swiglu_one(xn, w1, w3, w2_t, chunks):
    acc = hid = None
    for n in range(len(chunks) + 1):
        prev = hid
        if n < len(chunks):
            gate = _silu(_dot(xn, w1[:, chunks[n]]))
            hid = (gate * _dot(xn, w3[:, chunks[n]])).astype(_BF16)
        if n >= 1:
            part = _dot_nt(w2_t[:, chunks[n - 1]], prev)
            acc = part if acc is None else acc + part
    return acc


def _swiglu_pair(x_terms, x_rest, w1, w3, w1_terms, w3_terms, w2_terms, side_work):
    quarter = w1.shape[1] // 4
    tok = x_rest.shape[1]
    x_both = jnp.concatenate([x_rest[0], x_rest[1]], axis=0)

    def project(w, terms, lo):
        c = _combine(2, lambda i: _dot(x_terms[i], _unpack(terms[lo // _QUARTER, i])))
        rest = [_dot(x_both, w[4 * _QUARTER:, j * quarter + lo:j * quarter + lo + _QUARTER])
                for j in range(4)]
        return [c[i][j] + rest[j][i * tok:(i + 1) * tok] for i in range(2) for j in range(4)]

    def hidden(lo):
        gates = [_silu(g) for g in project(w1, w1_terms, lo)]
        hid = [g * u for g, u in zip(gates, project(w3, w3_terms, lo))]
        return [t.astype(_BF16) for t in _left_terms([hid[:4], hid[4:]])]

    chunks = list(range(0, quarter, _PAIR_CHUNK))
    acc, hid = [None] * _PRODUCTS, None
    for n in range(len(chunks) + 1):
        prev = hid
        if n < len(chunks):
            tiles = [hidden(lo) for lo in range(chunks[n], chunks[n] + _PAIR_CHUNK, _QUARTER)]
            hid = [jnp.concatenate(t, axis=1) for t in zip(*tiles)]
        if n >= 1:
            first = chunks[n - 1] // _QUARTER
            for i in range(_PRODUCTS):
                left = [_unpack(w2_terms[first + c, i]) for c in range(_PAIR_CHUNK // _QUARTER)]
                part = _dot_nt(jnp.concatenate(left, axis=1), prev[i])
                acc[i] = part if acc[i] is None else acc[i] + part
        side_work(n)
    return [jnp.concatenate(row, axis=0) for row in _combine(2, acc.__getitem__)]


def _store_terms(w, terms, transposed):
    block_rows, block_cols = 2 * terms.shape[2], terms.shape[0] * _QUARTER

    def tile(j, carry):
        def block(r, c, lo):
            rows = pl.ds(pl.multiple_of(r * block_rows + j * 16, 16), 16)
            return pltpu.bitcast(
                w[rows, c * block_cols + lo:c * block_cols + lo + _QUARTER], jnp.uint32)

        for lo in range(0, block_cols, _QUARTER):
            words = [block(n, k, lo) if transposed else block(k, n, lo)
                     for k in range(4) for n in range(4)]
            even, odd = (_right_terms(rows) for rows in zip(*map(_split_words, words)))
            for i, pair in enumerate(zip(even, odd)):
                terms[lo // _QUARTER, i, pl.ds(pl.multiple_of(j * 8, 8), 8)] = (
                    pltpu.pack_elementwise(pair, packed_dtype=_BF16))
        return carry

    lax.fori_loop(0, block_rows // 16, tile, 0)


def _load_weights(sources, main, rest, wo_hbm, wo, wo_rest, stage, wo_stage, wsem, osem,
                  later_copies):
    _, n_heads, dh = sources[0].shape
    n_groups = n_heads // _GROUP
    main_chunks = _QUARTER // _WCHUNK
    per_weight = main_chunks + 1
    n_jobs = len(sources) * per_weight
    slots = stage.shape[0]
    rest_parts = 2 * rest.shape[2] // _WCHUNK

    def for_copies(src, job, action):
        c, slot = job % per_weight, job % slots

        def copy(row, n):
            action(pltpu.make_async_copy(src.at[pl.ds(row, _WCHUNK)], stage.at[slot, n],
                                         wsem.at[4 * slot + n]))

        @pl.when(c < main_chunks)
        def _():
            for n in range(4):
                copy(n * _QUARTER + c * _WCHUNK, n)

        @pl.when(c == main_chunks)
        def _():
            for n in range(rest_parts):
                copy(4 * _QUARTER + n * _WCHUNK, n)

    def start(job):
        for i, src in enumerate(sources):
            pl.when(job // per_weight == i)(
                functools.partial(for_copies, src, job, lambda c: c.start()))

    def wait(job):
        for i, src in enumerate(sources):
            pl.when(job // per_weight == i)(
                functools.partial(for_copies, src, job, lambda c: c.wait()))

    def split_heads(slot, n, j):
        rows = pl.ds(pl.multiple_of(j * 16, 16), 16)
        words = jnp.swapaxes(pltpu.bitcast(stage[slot, n, rows], jnp.uint32), 0, 1)
        return [half for p in range(n_heads // 2) for half in _split_words(words[p])]

    def output_group(g, carry):
        heads = [wo_stage[_GROUP * g + i, :4 * _QUARTER].T for i in range(_GROUP)]
        for r in range(0, dh, 16):
            blocks = [blk for h in heads for blk in _quarters(h[r:r + 16].astype(_F32))]
            rows = pl.ds(pl.multiple_of(g * (dh // 2) + r // 2, 8), 8)
            for i, t in enumerate(_right_terms(blocks)):
                wo[i, rows, :] = _pack(t)
        for i in range(_GROUP):
            head = _GROUP * g + i
            wo_rest[pl.ds(pl.multiple_of(head * (dh // 2), dh // 2), dh // 2), :] = _pack(
                wo_stage[head, 4 * _QUARTER:].astype(_F32).T)
        return carry

    wo_copy = pltpu.make_async_copy(wo_hbm, wo_stage, osem)
    lax.fori_loop(0, _INFLIGHT, lambda job, carry: start(job), None)
    wo_copy.start()

    def groups_done(job):
        return n_groups * jnp.maximum(job - _WO_FROM, 0) // (n_jobs - _WO_FROM)

    def run(job, carry):
        which, c, slot = job // per_weight, job % per_weight, job % slots
        wait(job)
        start(job + _INFLIGHT)

        @pl.when(job == n_jobs - _LATER_FROM)
        def _():
            for copy in later_copies:
                copy.start()


        def main_rows(j, carry):
            rows = pl.ds(pl.multiple_of(c * (_WCHUNK // 2) + j * 8, 8), 8)
            parts = [split_heads(slot, n, j) for n in range(4)]
            for g in range(n_groups):
                blocks = [h for part in parts for h in part[_GROUP * g:_GROUP * (g + 1)]]
                for n, t in enumerate(_right_terms(blocks)):
                    main[which, g, n, rows] = _pack(t)
            return carry

        def rest_rows(j, carry):
            rows = pl.ds(pl.multiple_of(j * 8, 8), 8)
            for h, t in enumerate(split_heads(slot, j // tiles, j % tiles)):
                rest[which, h, rows] = _pack(t)
            return carry

        tiles = _WCHUNK // 16
        lax.fori_loop(0, jnp.where(c < main_chunks, tiles, 0), main_rows, 0)
        lax.fori_loop(0, jnp.where(c < main_chunks, 0, rest_parts * tiles), rest_rows, 0)
        pl.when(job == _WO_FROM)(wo_copy.wait)
        lax.fori_loop(groups_done(job), groups_done(job + 1), output_group, 0)
        return carry

    lax.fori_loop(0, n_jobs, run, 0)


def _kernel(x0_ref, x_next_ref, mem0_ref, wq_hbm, wk_hbm, wv_hbm, wo_hbm, w1_hbm, w3_hbm,
            w2_hbm, out_ref,
            stage, wo_stage, qkv, qkv_rest, wo, wo_rest,
            w1, w3, w2_t, w1_terms, w3_terms, w2_terms, res, normed, mem, acc_t, x_terms, x_rest, wsem, osem, fsem, *, seg):
    b = pl.program_id(0)
    n_blocks = pl.num_programs(0) - 1
    _, n_heads, dh = wq_hbm.shape
    n_mem = mem0_ref.shape[0]
    n_chunks = w1.shape[1] // _FCHUNK
    steps = _TOK // seg
    ffn_copies = [pltpu.make_async_copy(s, d, fsem.at[i])
                  for i, (s, d) in enumerate(((w1_hbm, w1), (w3_hbm, w3), (w2_hbm, w2_t)))]

    def start_layer(slot, x):
        res[slot] = x
        normed[slot] = _layernorm(x)

    def prepare_swiglu(rows):
        xs = [_layernorm(res[i, rows]) for i in range(2)]
        for i, t in enumerate(_left_terms([_quarters(x) for x in xs])):
            x_terms[i, rows] = t.astype(_BF16)
        for i, x in enumerate(xs):
            x_rest[i, rows] = x[:, 4 * _QUARTER:].astype(_BF16)

    @pl.when(b == 0)
    def _():
        _load_weights((wq_hbm, wk_hbm, wv_hbm), qkv, qkv_rest, wo_hbm, wo, wo_rest,
                      stage, wo_stage, wsem, osem, ffn_copies)
        mem[0] = mem0_ref[...].astype(_F32)
        mem[1] = mem0_ref[...].astype(_F32)
        start_layer(0, x0_ref[...].astype(_F32).T)

    def run_attention(first, n_seq):
        keep, fill = _masks(n_mem, n_mem + seg, n_seq)

        def segment(j, carry):
            rows = pl.ds(pl.multiple_of(j * seg, seg), seg)
            if n_seq == 2:
                done = pl.ds(pl.multiple_of(jnp.maximum(j - 1, 0) * seg, seg), seg)
                prepare_swiglu(done)
            hs = [jnp.concatenate([mem[first + i], normed[first + i, rows]], axis=0)
                  for i in range(n_seq)]
            for i, out in enumerate(_attention(hs, keep, fill, qkv, qkv_rest, wo, wo_rest,
                                               n_heads, dh)):
                mem[first + i] = out[:n_mem]
                res[first + i, rows] += out[n_mem:]
            return carry

        lax.fori_loop(0, steps, segment, 0)

    both = jnp.logical_and(b > 0, b < n_blocks)

    @pl.when(both)
    def _():
        run_attention(0, 2)
        prepare_swiglu(pl.ds(_TOK - seg, seg))

        def side_work(n):
            if n == 0:
                acc_t[...] = res[1].T
                res[1] = res[0]
            if n == 1:
                start_layer(0, x_next_ref[...].astype(_F32).T)

        f2, f4 = _swiglu_pair(x_terms, x_rest, w1, w3, w1_terms, w3_terms, w2_terms, side_work)
        start_layer(1, res[1] + f2.T)
        out_ref[...] = (acc_t[...] + f4).astype(out_ref.dtype)

    @pl.when(jnp.logical_not(both))
    def _():
        slot = jnp.where(b == 0, 0, 1)
        run_attention(slot, 1)

        @pl.when(b == 0)
        def _():
            for c, w, terms in zip(ffn_copies, (w1, w3, w2_t), (w1_terms, w3_terms, w2_terms)):
                c.wait()
                _store_terms(w, terms, w is w2_t)

        x = res[slot]
        xn = _layernorm(x).astype(_BF16)
        acc_t[...] = x.T

        def part(i, carry):
            chunks = [pl.ds(pl.multiple_of((i * _EDGE_CHUNKS + c) * _FCHUNK, _FCHUNK), _FCHUNK)
                      for c in range(_EDGE_CHUNKS)]
            acc_t[...] += _swiglu_one(xn, w1, w3, w2_t, chunks)
            return carry

        lax.fori_loop(0, n_chunks // _EDGE_CHUNKS, part, 0)

        @pl.when(b == 0)
        def _():
            start_layer(1, acc_t[...].T)
            start_layer(0, x_next_ref[...].astype(_F32).T)

        @pl.when(b > 0)
        def _():
            out_ref[...] = acc_t[...].astype(out_ref.dtype)


@functools.partial(jax.jit, static_argnames=("A_seg_len",))
def pallas_interleave_layers__memory_aug_recurrent_mem_tr__glu_gated_swiglu__prompt_kernel(
    A_x: jax.Array,
    A_mem0: jax.Array,
    A_Wq: jax.Array,
    A_Wk: jax.Array,
    A_Wv: jax.Array,
    A_Wo: jax.Array,
    A_seg_len: int,
    B_x: jax.Array,
    B_w1: jax.Array,
    B_w3: jax.Array,
    B_w2: jax.Array,
):
    del B_x
    batch, seq, d_model = A_x.shape
    n_mem = A_mem0.shape[1]
    _, n_heads, dh = A_Wq.shape
    d_ff = B_w1.shape[1]
    seg = int(A_seg_len)
    assert batch == 1 and seq % _TOK == 0 and _TOK % seg == 0 and seg % 16 == 0
    assert n_mem == 8 and n_heads % _GROUP == 0 and d_ff % (_FCHUNK * _EDGE_CHUNKS) == 0
    d_rest = d_model - 4 * _QUARTER
    assert 0 < d_rest <= 4 * _WCHUNK and d_rest % _WCHUNK == 0 and d_model % 64 == 0
    assert dh == _QUARTER and d_ff % (4 * _PAIR_CHUNK) == 0
    ff_tiles = d_ff // (4 * _QUARTER)
    n_blocks = seq // _TOK

    x_t = A_x[0].T
    hbm = pl.BlockSpec(memory_space=pl.ANY)
    out_t = pl.pallas_call(
        functools.partial(_kernel, seg=seg),
        grid=(n_blocks + 1,),
        in_specs=[
            pl.BlockSpec((d_model, _TOK), lambda b: (0, 0)),
            pl.BlockSpec((d_model, _TOK), lambda b: (0, jnp.minimum(b + 1, n_blocks - 1))),
            pl.BlockSpec((n_mem, d_model), lambda b: (0, 0)),
            hbm, hbm, hbm, hbm, hbm, hbm, hbm,
        ],
        out_specs=pl.BlockSpec((d_model, _TOK), lambda b: (0, jnp.maximum(b - 1, 0))),
        out_shape=jax.ShapeDtypeStruct((d_model, seq), A_x.dtype),
        scratch_shapes=[
            pltpu.VMEM((_INFLIGHT + 1, 4, _WCHUNK, n_heads, dh), _BF16),
            pltpu.VMEM((n_heads, d_model, dh), _BF16),
            pltpu.VMEM((3, n_heads // _GROUP, _PRODUCTS, _QUARTER // 2, dh), jnp.uint32),
            pltpu.VMEM((3, n_heads, d_rest // 2, dh), jnp.uint32),
            pltpu.VMEM((_PRODUCTS, n_heads * dh // 8, _QUARTER), jnp.uint32),
            pltpu.VMEM((n_heads * dh // 2, d_rest), jnp.uint32),
            pltpu.VMEM((d_model, d_ff), _BF16),
            pltpu.VMEM((d_model, d_ff), _BF16),
            pltpu.VMEM((d_model, d_ff), _BF16),
            *2 * [pltpu.VMEM((ff_tiles, _PRODUCTS, _QUARTER // 2, _QUARTER), jnp.uint32)],
            pltpu.VMEM((ff_tiles, _PRODUCTS, d_model // 8, _QUARTER), jnp.uint32),
            pltpu.VMEM((2, _TOK, d_model), _F32),
            pltpu.VMEM((2, _TOK, d_model), _F32),
            pltpu.VMEM((2, n_mem, d_model), _F32),
            pltpu.VMEM((d_model, _TOK), _F32),
            pltpu.VMEM((_PRODUCTS, _TOK, _QUARTER), _BF16),
            pltpu.VMEM((2, _TOK, d_rest), _BF16),
            pltpu.SemaphoreType.DMA((4 * (_INFLIGHT + 1),)),
            pltpu.SemaphoreType.DMA(()),
            pltpu.SemaphoreType.DMA((3,)),
        ],
        compiler_params=pltpu.CompilerParams(
            dimension_semantics=("arbitrary",),
            vmem_limit_bytes=112 * 1024 * 1024,
        ),
    )(x_t, x_t, A_mem0[0], A_Wq, A_Wk, A_Wv, jnp.transpose(A_Wo, (0, 2, 1)),
      B_w1, B_w3, B_w2.T)
    return out_t.T[None]
```

```python
import functools

import jax
import jax.numpy as jnp
import numpy as np
from jax import lax
import jax.experimental.pallas as pl
import jax.experimental.pallas.tpu as pltpu

_BF16 = jnp.bfloat16
_F32 = jnp.float32
_NT = (((1,), (1,)), ((), ()))
_TOK = 128
_GROUP = 4
_FCHUNK = 512
_WCHUNK = 32
_INFLIGHT = 3
_EDGE_CHUNKS = 3
_BLOCK = 128
_WO_FROM = 5
_PAIR_CHUNK = 384
_LATER_FROM = 1
_STAGE_ORDER = (((0, 1), 0), ("mix", 1), ((2,), 0), ("scores", 0), ("output", 2))
_MASKED = -1000000000.0


def _layernorm(x):
    m = jnp.mean(x, axis=-1, keepdims=True)
    c = x - m
    v = jnp.mean(c * c, axis=-1, keepdims=True)
    return c * lax.rsqrt(v + 1e-05)


def _dot(a, b):
    return lax.dot_general(a, b, (((1,), (0,)), ((), ())), preferred_element_type=_F32)


def _dot_nt(a, b):
    return lax.dot_general(a, b, _NT, preferred_element_type=_F32)


def _pack(x):
    return pltpu.bitcast(x.astype(_BF16), jnp.uint32)


def _split_words(words):
    return (pltpu.bitcast(words << 16, _F32),
            pltpu.bitcast(words & jnp.uint32(0xFFFF0000), _F32))


def _unpack(words):
    return pltpu.bitcast(words, _BF16)


_SCHEME_244 = (
    "...+.... +.......++..--.. .-......",
    "..+++..+ +.........-..... ..-.+...",
    ".+++.... ....+++......... +..-....",
    ".+.+.+.. ...+.......+...- ...-.-.+",
    "++-..... ......+......... -.+++.--",
    "+...+..+ .+-.......-...+. ..-..++.",
    "+.-..... +.....+......... +.-.....",
    "..++..+. +....-..++..-... -+..+...",
    "+....... .+.............. .++..--.",
    ".+...+.. ....++++...+...- ...+....",
    "++-..+.. ...+..-......... ...++.--",
    "..++.-.. ...++++....+.... ...+-...",
    "+..++..+ +.........-...+. ..+.....",
    ".+.+..-. .....+.......... -+...-.+",
    "..++.... +...---.++...... +...-...",
    "..+...+. +....-..+...-... +-......",
    "......+. .....+...-...... -+..+-..",
    ".....+.. ...+..+-...+.... ...+...-",
    "++-.++-. ...+............ ....-.++",
    "....+..+ .+-.......-..... ..+...-.",
    ".+.+.+.+ ...+.+.....+...- .....+.-",
    "....+.-. ...+......+..... ....+.-.",
    ".....+++ ...+.+.....+.... ....-..+",
    "+...+... ..+.......+...-. .....++.",
    ".......+ .+-+.+....-+.-+- .....-..",
    "..++..++ +..-.-....---... ....-...",
)
_SCHEME_254 = (
    "..+-.-..+. -.........+.....+... ..+.+...",
    "....+..... .-...............+.. .+...+..",
    ".++-...... ...-+-+....-...-.... +..+....",
    "....+..... ...................+ ...+....",
    "..+-...... .+-+-+-...-+-+-+-... +...+...",
    ".++....... ...-.......-...-.... .+.-.+.-",
    "+..-+..... .+-.......-...-.-... .++.....",
    "+...+..... ..-.......-...-..... +.-.+.-.",
    ".+....-... ...+-+-+............ ...+....",
    "+.-....... +.....-.........-... +.-.....",
    "....++..-. .-..............+.+. ..+..-..",
    "+--...+... ...+..-............. ...++.-+",
    ".++.....-. ...+.+.....+...+.... ++...+.-",
    "..+-....+. +-+-.-..+.+-+-+-.... ++..+...",
    "+...+...-. ..+.......+...+.+... ++..+.-.",
    "+..-.-..+. +-+................. ..+.....",
    "..+-..+... ...+-+-....+........ ...+-...",
    "..+....... -+-+....-+-+-+-+.... .+......",
    "...+....-. +..-.-..+..-+..--... ++......",
    "+--....... ......+............. +.-++.-+",
    ".....+..-. ..+.......+.......-. ..+...+.",
    "+...+-...- ................-... ....+.-.",
    "..+-...-+. ...+.+..-.-+........ ....+...",
    "........+. .+.+.+.....+.+.+.... ++..++..",
    ".....+..-+ ................+.+. .....++.",
    "......+... ...-..++...-........ ...+...+",
    ".....+.-.. ...-......+......... ....+.-.",
    "......++-. ...+.+.....+........ ....+..+",
    ".++...--.. .....-.............. .....+.-",
    ".......+.. .....-...+.......... .....+..",
    ".........+ ...................+ .......+",
    "+--..-++.. ...-................ ....+.-+",
    "....+....- ................+-+. .....+..",
)


def _sum_program(rows):
    n_in = len(rows[0])
    rows = [{i: c for i, c in enumerate(row) if c} for row in rows]
    steps, ready = [], list(range(n_in))

    def emit(a, b, sign):
        steps.append((a, b, sign))
        ready.append(max(ready[a], ready[b]))
        return len(ready) - 1

    while True:
        count = {}
        for row in rows:
            items = sorted(row.items())
            for n, (a, x) in enumerate(items):
                for b, y in items[n + 1:]:
                    count[a, b, x * y] = count.get((a, b, x * y), 0) + 1
        best = max(sorted(count), key=count.get, default=None)
        if best is None or count[best] < 2:
            break
        a, b, sign = best
        new = emit(a, b, sign)
        for row in rows:
            if a in row and b in row and row[a] * row[b] == sign:
                row[new] = row.pop(a)
                del row[b]
    outs = []
    for row in rows:
        items = sorted(row.items(), key=lambda item: (ready[item[0]], item[0]))
        at, sign = items[0]
        for b, y in items[1:]:
            if sign < 0 < y:
                at, sign = emit(b, at, -1), 1
            else:
                at = emit(at, b, sign * y)
        outs.append((at, sign))
    return n_in, steps, ready, outs


def _evaluate(program, make):
    n_in, steps, ready, outs = program
    vals = {}
    for i in range(n_in):
        vals[i] = make(i)
        for n, (a, b, sign) in enumerate(steps):
            if ready[n_in + n] == i:
                vals[n_in + n] = vals[a] + vals[b] if sign > 0 else vals[a] - vals[b]
    return [vals[i] if sign > 0 else -vals[i] for i, sign in outs]


class _Scheme:
    def __init__(self, u, v, w):
        self.products = len(u)
        self.inner, self.outer = k, n = u.shape[1] // 2, w.shape[1] // 2
        want = np.zeros((2 * k, k * n, 2 * n), np.int64)
        for i, a, j in np.ndindex(2, k, n):
            want[k * i + a, n * a + j, n * i + j] = 1
        first = (u[:k * n, :k], v[:k * n], w[:k * n, :n])
        assert np.array_equal(np.einsum("ra,rb,rc->abc", u, v, w), want)
        assert np.array_equal(np.einsum("ra,rb,rc->abc", *first), want[:k, :, :n])
        self._left = {1: _sum_program(first[0].tolist()), 2: _sum_program(u.tolist())}
        self._right = _sum_program(v.tolist())
        self._out = {1: _sum_program(first[2].T.tolist()), 2: _sum_program(w.T.tolist())}

    def left(self, rows):
        blocks = [blk for row in rows for blk in _column_blocks(row, self.inner)]
        return _evaluate(self._left[len(rows)], blocks.__getitem__)

    def right(self, blocks):
        return _evaluate(self._right, blocks.__getitem__)

    def combine(self, n_rows, product):
        c = _evaluate(self._out[n_rows], product)
        return [c[self.outer * i:self.outer * (i + 1)] for i in range(n_rows)]


def _parse(table):
    return [np.array([[{"+": 1, ".": 0, "-": -1}[c] for c in line.split()[f]]
                      for line in table]) for f in range(3)]


def _swap_inner_outer(u, v, w):
    k, n = u.shape[1] // 2, w.shape[1] // 2
    return w, v.reshape(-1, k, n).transpose(0, 2, 1).reshape(-1, k * n), u


_SQUARE = _Scheme(*_parse(_SCHEME_244))
_FROM_MODEL = _Scheme(*_parse(_SCHEME_254))
_TO_MODEL = _Scheme(*_swap_inner_outer(*_parse(_SCHEME_254)))


def _column_blocks(x, count):
    pad = count * _BLOCK - x.shape[1]
    if pad:
        x = jnp.concatenate([x, jnp.zeros((x.shape[0], pad), x.dtype)], axis=1)
    return [x[:, i * _BLOCK:(i + 1) * _BLOCK] for i in range(count)]


def _masks(n_mem, length, n_seq):
    rows = n_seq * length

    def describe(axis):
        i = lax.broadcasted_iota(jnp.int32, (rows, rows), axis)
        second = i >= length
        return jnp.where(second, 1, 0), jnp.where(second, i - length, i)

    (seq_r, idx_r), (seq_c, idx_c) = describe(0), describe(1)
    same = seq_r == seq_c
    keep = same & ((idx_r < n_mem) | (idx_r >= idx_c))
    fill = jnp.where(same, _MASKED, -jnp.inf).astype(_F32)
    return keep, fill


def _attention(hs, keep, fill, qkv, wo, n_heads, dh):
    scale = dh ** -0.5
    n_groups = n_heads // _GROUP
    n_seq, length = len(hs), hs[0].shape[0]
    heads = [slice(i * dh, (i + 1) * dh) for i in range(_GROUP)]
    lhs_dtype = _BF16 if (n_seq * length) % 16 == 0 else _F32

    h_terms = _FROM_MODEL.left(hs)

    def project(ws, g):
        c = _FROM_MODEL.combine(n_seq, lambda i: _dot(h_terms[i], jnp.concatenate(
            [_unpack(qkv[w, g, i]) for w in ws], axis=1)))
        return [jnp.concatenate(
            [jnp.concatenate([blk[:, n * dh:(n + 1) * dh] for blk in row], axis=1) for row in c],
            axis=0) for n in range(len(ws))]

    def weights(q, k):
        out = []
        for cols in heads:
            s = jnp.where(keep, _dot_nt(q[:, cols], k[:, cols]) * scale, fill)
            e = jnp.exp(s - jnp.max(s, axis=-1, keepdims=True))
            out.append((e.astype(lhs_dtype), 1.0 / jnp.sum(e, axis=-1, keepdims=True)))
        return out

    def mix(p, v):
        return jnp.concatenate(
            [_dot(e, v[:, cols]) * inv for (e, inv), cols in zip(p, heads)], axis=1)

    def output(o, g):
        terms = _TO_MODEL.left([o[i * length:(i + 1) * length] for i in range(n_seq)])
        return [_dot(t, _unpack(wo[g, i])) for i, t in enumerate(terms)]

    proj, p, o, acc = {}, {}, {}, None
    for stage in range(n_groups + max(lag for _, lag in _STAGE_ORDER)):
        for task, lag in _STAGE_ORDER:
            g = stage - lag
            if not 0 <= g < n_groups:
                continue
            if task == "scores":
                p[g] = weights(proj.pop((0, g)), proj.pop((1, g)))
            elif task == "mix":
                o[g] = mix(p.pop(g), proj.pop((2, g)))
            elif task == "output":
                part = output(o.pop(g), g)
                acc = part if acc is None else [x + y for x, y in zip(acc, part)]
            else:
                for w, x in zip(task, project(task, g)):
                    proj[w, g] = x.astype(lhs_dtype if w == 0 else _BF16)
    return [jnp.concatenate(row, axis=1)[:, :hs[0].shape[1]]
            for row in _TO_MODEL.combine(n_seq, acc.__getitem__)]


def _silu(x):
    half = 0.5 * x
    return half + half * jnp.tanh(half)


def _swiglu_one(xn, w1, w3, w2_t, chunks):
    acc = hid = None
    for n in range(len(chunks) + 1):
        prev = hid
        if n < len(chunks):
            gate = _silu(_dot(xn, w1[:, chunks[n]]))
            hid = (gate * _dot(xn, w3[:, chunks[n]])).astype(_BF16)
        if n >= 1:
            part = _dot_nt(w2_t[:, chunks[n - 1]], prev)
            acc = part if acc is None else acc + part
    return acc


def _swiglu_pair(x_terms, w1_terms, w3_terms, w2_terms, side_work):
    def project(terms, lo):
        c = _FROM_MODEL.combine(2, lambda i: _dot(x_terms[i], _unpack(terms[lo // _BLOCK, i])))
        return [jnp.concatenate(row, axis=1) for row in c]

    def hidden(lo):
        gates = [_silu(g) for g in project(w1_terms, lo)]
        hid = [g * u for g, u in zip(gates, project(w3_terms, lo))]
        return [t.astype(_BF16) for t in _SQUARE.left(hid)]

    chunks = list(range(0, w2_terms.shape[0] * _BLOCK, _PAIR_CHUNK))
    acc, hid = [None] * _SQUARE.products, None
    for n in range(len(chunks) + 1):
        prev = hid
        if n < len(chunks):
            tiles = [hidden(lo) for lo in range(chunks[n], chunks[n] + _PAIR_CHUNK, _BLOCK)]
            hid = [jnp.concatenate(t, axis=1) for t in zip(*tiles)]
        if n >= 1:
            first = chunks[n - 1] // _BLOCK
            for i in range(_SQUARE.products):
                left = [_unpack(w2_terms[first + c, i]) for c in range(_PAIR_CHUNK // _BLOCK)]
                part = _dot_nt(jnp.concatenate(left, axis=1), prev[i])
                acc[i] = part if acc[i] is None else acc[i] + part
        side_work(n)
    return [jnp.concatenate(row, axis=0) for row in _SQUARE.combine(2, acc.__getitem__)]


def _store_terms(w, terms, scheme, transposed):
    block_rows, block_cols = 2 * terms.shape[2], terms.shape[0] * _BLOCK

    def tile(j, carry):
        def block(r, c, lo):
            start = r * block_rows + j * 16
            rows = pl.ds(pl.multiple_of(jnp.minimum(start, w.shape[0] - 16), 16), 16)
            words = pltpu.bitcast(
                w[rows, c * block_cols + lo:c * block_cols + lo + _BLOCK], jnp.uint32)
            if (r + 1) * block_rows > w.shape[0]:
                words = jnp.where(start < w.shape[0], words, jnp.uint32(0))
            return words

        for lo in range(0, block_cols, _BLOCK):
            words = [block(n, k, lo) if transposed else block(k, n, lo)
                     for k in range(scheme.inner) for n in range(scheme.outer)]
            even, odd = (scheme.right(rows) for rows in zip(*map(_split_words, words)))
            for i, pair in enumerate(zip(even, odd)):
                terms[lo // _BLOCK, i, pl.ds(pl.multiple_of(j * 8, 8), 8)] = (
                    pltpu.pack_elementwise(pair, packed_dtype=_BF16))
        return carry

    lax.fori_loop(0, block_rows // 16, tile, 0)


def _load_weights(sources, qkv, wo_hbm, wo, stage, wo_stage, wsem, osem,
                  later_copies):
    d_model, n_heads, dh = sources[0].shape
    n_groups = n_heads // _GROUP
    per_weight = _BLOCK // _WCHUNK
    n_jobs = len(sources) * per_weight
    full = _FROM_MODEL.inner - 1
    ragged = (d_model - full * _BLOCK) // _WCHUNK
    stage[ragged:, full] = jnp.zeros((per_weight - ragged,) + stage.shape[2:], stage.dtype)

    def for_copies(src, job, action):
        c = job % per_weight

        def copy(n):
            action(pltpu.make_async_copy(src.at[pl.ds(n * _BLOCK + c * _WCHUNK, _WCHUNK)],
                                         stage.at[c, n], wsem.at[(full + 1) * c + n]))

        for n in range(full):
            copy(n)
        pl.when(c < ragged)(functools.partial(copy, full))

    def start(job):
        for i, src in enumerate(sources):
            pl.when(job // per_weight == i)(
                functools.partial(for_copies, src, job, lambda c: c.start()))

    def wait(job):
        for i, src in enumerate(sources):
            pl.when(job // per_weight == i)(
                functools.partial(for_copies, src, job, lambda c: c.wait()))

    def split_heads(slot, n, j):
        rows = pl.ds(pl.multiple_of(j * 16, 16), 16)
        words = jnp.swapaxes(pltpu.bitcast(stage[slot, n, rows], jnp.uint32), 0, 1)
        return [half for p in range(n_heads // 2) for half in _split_words(words[p])]

    def output_group(g, carry):
        def transposed(head):
            last = jnp.concatenate(
                [wo_stage[head, full * _BLOCK:],
                 jnp.zeros(((full + 1) * _BLOCK - d_model, dh), wo_stage.dtype)], axis=0)
            return jnp.concatenate([wo_stage[head, :full * _BLOCK].T, last.T], axis=1)

        heads = [transposed(_GROUP * g + i) for i in range(_GROUP)]
        for r in range(0, dh, 16):
            blocks = [blk for h in heads
                      for blk in _column_blocks(h[r:r + 16].astype(_F32), _TO_MODEL.outer)]
            for i, t in enumerate(_TO_MODEL.right(blocks)):
                wo[g, i, r // 2:r // 2 + 8] = _pack(t)
        return carry

    wo_copy = pltpu.make_async_copy(wo_hbm, wo_stage, osem)
    lax.fori_loop(0, _INFLIGHT, lambda job, carry: start(job), None)
    wo_copy.start()

    def groups_done(job):
        return n_groups * jnp.maximum(job - _WO_FROM, 0) // (n_jobs - _WO_FROM)

    def run(job, carry):
        which, c = job // per_weight, job % per_weight
        wait(job)
        start(job + _INFLIGHT)

        @pl.when(job == n_jobs - _LATER_FROM)
        def _():
            for copy in later_copies:
                copy.start()


        def main_rows(j, carry):
            rows = pl.ds(pl.multiple_of(c * (_WCHUNK // 2) + j * 8, 8), 8)
            parts = [split_heads(c, n, j) for n in range(full + 1)]
            for g in range(n_groups):
                blocks = [h for part in parts for h in part[_GROUP * g:_GROUP * (g + 1)]]
                for n, t in enumerate(_FROM_MODEL.right(blocks)):
                    qkv[which, g, n, rows] = _pack(t)
            return carry

        lax.fori_loop(0, _WCHUNK // 16, main_rows, 0)
        pl.when(job == _WO_FROM)(wo_copy.wait)
        lax.fori_loop(groups_done(job), groups_done(job + 1), output_group, 0)
        return carry

    lax.fori_loop(0, n_jobs, run, 0)


def _kernel(x0_ref, x_next_ref, mem0_ref, wq_hbm, wk_hbm, wv_hbm, wo_hbm, w1_hbm, w3_hbm,
            w2_hbm, out_ref,
            stage, wo_stage, qkv, wo,
            w1, w3, w2_t, w1_terms, w3_terms, w2_terms, res, normed, mem, acc_t, x_terms, wsem, osem, fsem, *, seg):
    b = pl.program_id(0)
    n_blocks = pl.num_programs(0) - 1
    _, n_heads, dh = wq_hbm.shape
    n_mem = mem0_ref.shape[0]
    n_chunks = w1.shape[1] // _FCHUNK
    steps = _TOK // seg
    ffn_copies = [pltpu.make_async_copy(s, d, fsem.at[i])
                  for i, (s, d) in enumerate(((w1_hbm, w1), (w3_hbm, w3), (w2_hbm, w2_t)))]

    def start_layer(slot, x):
        res[slot] = x
        normed[slot] = _layernorm(x)

    def prepare_swiglu(rows):
        xs = [_layernorm(res[i, rows]) for i in range(2)]
        for i, t in enumerate(_FROM_MODEL.left(xs)):
            x_terms[i, rows] = t.astype(_BF16)

    @pl.when(b == 0)
    def _():
        _load_weights((wq_hbm, wk_hbm, wv_hbm), qkv, wo_hbm, wo,
                      stage, wo_stage, wsem, osem, ffn_copies)
        mem[0] = mem0_ref[...].astype(_F32)
        mem[1] = mem0_ref[...].astype(_F32)
        start_layer(0, x0_ref[...].astype(_F32).T)

    def run_attention(first, n_seq):
        keep, fill = _masks(n_mem, n_mem + seg, n_seq)

        def segment(j, carry):
            rows = pl.ds(pl.multiple_of(j * seg, seg), seg)
            if n_seq == 2:
                done = pl.ds(pl.multiple_of(jnp.maximum(j - 1, 0) * seg, seg), seg)
                prepare_swiglu(done)
            hs = [jnp.concatenate([mem[first + i], normed[first + i, rows]], axis=0)
                  for i in range(n_seq)]
            for i, out in enumerate(_attention(hs, keep, fill, qkv, wo, n_heads, dh)):
                mem[first + i] = out[:n_mem]
                res[first + i, rows] += out[n_mem:]
            return carry

        lax.fori_loop(0, steps, segment, 0)

    both = jnp.logical_and(b > 0, b < n_blocks)

    @pl.when(both)
    def _():
        run_attention(0, 2)
        prepare_swiglu(pl.ds(_TOK - seg, seg))

        def side_work(n):
            if n == 0:
                acc_t[...] = res[1].T
                res[1] = res[0]
            if n == 1:
                start_layer(0, x_next_ref[...].astype(_F32).T)

        f2, f4 = _swiglu_pair(x_terms, w1_terms, w3_terms, w2_terms, side_work)
        start_layer(1, res[1] + f2.T)
        out_ref[...] = (acc_t[...] + f4).astype(out_ref.dtype)

    @pl.when(jnp.logical_not(both))
    def _():
        slot = jnp.where(b == 0, 0, 1)
        run_attention(slot, 1)

        @pl.when(b == 0)
        def _():
            for c, w, terms in zip(ffn_copies, (w1, w3, w2_t), (w1_terms, w3_terms, w2_terms)):
                c.wait()
                _store_terms(w, terms, _SQUARE if w is w2_t else _FROM_MODEL, w is w2_t)

        x = res[slot]
        xn = _layernorm(x).astype(_BF16)
        acc_t[...] = x.T

        def part(i, carry):
            chunks = [pl.ds(pl.multiple_of((i * _EDGE_CHUNKS + c) * _FCHUNK, _FCHUNK), _FCHUNK)
                      for c in range(_EDGE_CHUNKS)]
            acc_t[...] += _swiglu_one(xn, w1, w3, w2_t, chunks)
            return carry

        lax.fori_loop(0, n_chunks // _EDGE_CHUNKS, part, 0)

        @pl.when(b == 0)
        def _():
            start_layer(1, acc_t[...].T)
            start_layer(0, x_next_ref[...].astype(_F32).T)

        @pl.when(b > 0)
        def _():
            out_ref[...] = acc_t[...].astype(out_ref.dtype)


@functools.partial(jax.jit, static_argnames=("A_seg_len",))
def pallas_interleave_layers__memory_aug_recurrent_mem_tr__glu_gated_swiglu__prompt_kernel(
    A_x: jax.Array,
    A_mem0: jax.Array,
    A_Wq: jax.Array,
    A_Wk: jax.Array,
    A_Wv: jax.Array,
    A_Wo: jax.Array,
    A_seg_len: int,
    B_x: jax.Array,
    B_w1: jax.Array,
    B_w3: jax.Array,
    B_w2: jax.Array,
):
    del B_x
    batch, seq, d_model = A_x.shape
    n_mem = A_mem0.shape[1]
    _, n_heads, dh = A_Wq.shape
    d_ff = B_w1.shape[1]
    seg = int(A_seg_len)
    assert batch == 1 and seq % _TOK == 0 and _TOK % seg == 0 and seg % 16 == 0
    assert n_mem == 8 and n_heads % _GROUP == 0 and d_ff % (_FCHUNK * _EDGE_CHUNKS) == 0
    slots = _BLOCK // _WCHUNK
    assert _INFLIGHT < slots and d_model % 64 == 0
    assert (_FROM_MODEL.inner - 1) * _BLOCK < d_model < _FROM_MODEL.inner * _BLOCK
    assert dh == _BLOCK and d_ff % (4 * _PAIR_CHUNK) == 0
    ff_tiles = d_ff // (4 * _BLOCK)
    n_blocks = seq // _TOK

    x_t = A_x[0].T
    hbm = pl.BlockSpec(memory_space=pl.ANY)
    out_t = pl.pallas_call(
        functools.partial(_kernel, seg=seg),
        grid=(n_blocks + 1,),
        in_specs=[
            pl.BlockSpec((d_model, _TOK), lambda b: (0, 0)),
            pl.BlockSpec((d_model, _TOK), lambda b: (0, jnp.minimum(b + 1, n_blocks - 1))),
            pl.BlockSpec((n_mem, d_model), lambda b: (0, 0)),
            hbm, hbm, hbm, hbm, hbm, hbm, hbm,
        ],
        out_specs=pl.BlockSpec((d_model, _TOK), lambda b: (0, jnp.maximum(b - 1, 0))),
        out_shape=jax.ShapeDtypeStruct((d_model, seq), A_x.dtype),
        scratch_shapes=[
            pltpu.VMEM((slots, _FROM_MODEL.inner, _WCHUNK, n_heads, dh), _BF16),
            pltpu.VMEM((n_heads, d_model, dh), _BF16),
            pltpu.VMEM((3, n_heads // _GROUP, _FROM_MODEL.products, _BLOCK // 2, dh), jnp.uint32),
            pltpu.VMEM((n_heads // _GROUP, _TO_MODEL.products, dh // 2, _BLOCK), jnp.uint32),
            pltpu.VMEM((d_model, d_ff), _BF16),
            pltpu.VMEM((d_model, d_ff), _BF16),
            pltpu.VMEM((d_model, d_ff), _BF16),
            *2 * [pltpu.VMEM((ff_tiles, _FROM_MODEL.products, _BLOCK // 2, _BLOCK), jnp.uint32)],
            pltpu.VMEM((ff_tiles, _SQUARE.products, d_model // 8, _BLOCK), jnp.uint32),
            pltpu.VMEM((2, _TOK, d_model), _F32),
            pltpu.VMEM((2, _TOK, d_model), _F32),
            pltpu.VMEM((2, n_mem, d_model), _F32),
            pltpu.VMEM((d_model, _TOK), _F32),
            pltpu.VMEM((_FROM_MODEL.products, _TOK, _BLOCK), _BF16),
            pltpu.SemaphoreType.DMA((slots * _FROM_MODEL.inner,)),
            pltpu.SemaphoreType.DMA(()),
            pltpu.SemaphoreType.DMA((3,)),
        ],
        compiler_params=pltpu.CompilerParams(
            dimension_semantics=("arbitrary",),
            vmem_limit_bytes=112 * 1024 * 1024,
        ),
    )(x_t, x_t, A_mem0[0], A_Wq, A_Wk, A_Wv, jnp.transpose(A_Wo, (0, 2, 1)),
      B_w1, B_w3, B_w2.T)
    return out_t.T[None]
```

```python
import functools

import jax
import jax.numpy as jnp
import numpy as np
from jax import lax
import jax.experimental.pallas as pl
import jax.experimental.pallas.tpu as pltpu

_BF16 = jnp.bfloat16
_F32 = jnp.float32
_NT = (((1,), (1,)), ((), ()))
_TOK = 128
_GROUP = 4
_FCHUNK = 512
_WCHUNK = 32
_INFLIGHT = 3
_EDGE_CHUNKS = 3
_BLOCK = 128
_WO_FROM = 5
_PAIR_CHUNK = 384
_LATER_FROM = 1
_STAGE_ORDER = (((0, 1), 0), ("mix", 1), ((2,), 0), ("scores", 0), ("output", 2))
_LOG2E = float(np.log2(np.e))
_MASKED = -1000000000.0


def _layernorm(x):
    m = jnp.mean(x, axis=-1, keepdims=True)
    c = x - m
    v = jnp.mean(c * c, axis=-1, keepdims=True)
    return c * lax.rsqrt(v + 1e-05)


def _dot(a, b):
    return lax.dot_general(a, b, (((1,), (0,)), ((), ())), preferred_element_type=_F32)


def _dot_nt(a, b):
    return lax.dot_general(a, b, _NT, preferred_element_type=_F32)


def _pack(x):
    return pltpu.bitcast(x.astype(_BF16), jnp.uint32)


def _split_words(words):
    return (pltpu.bitcast(words << 16, _F32),
            pltpu.bitcast(words & jnp.uint32(0xFFFF0000), _F32))


def _unpack(words):
    return pltpu.bitcast(words, _BF16)


_SCHEME_244 = (
    "...+.... +.......++..--.. .-......",
    "..+++..+ +.........-..... ..-.+...",
    ".+++.... ....+++......... +..-....",
    ".+.+.+.. ...+.......+...- ...-.-.+",
    "++-..... ......+......... -.+++.--",
    "+...+..+ .+-.......-...+. ..-..++.",
    "+.-..... +.....+......... +.-.....",
    "..++..+. +....-..++..-... -+..+...",
    "+....... .+.............. .++..--.",
    ".+...+.. ....++++...+...- ...+....",
    "++-..+.. ...+..-......... ...++.--",
    "..++.-.. ...++++....+.... ...+-...",
    "+..++..+ +.........-...+. ..+.....",
    ".+.+..-. .....+.......... -+...-.+",
    "..++.... +...---.++...... +...-...",
    "..+...+. +....-..+...-... +-......",
    "......+. .....+...-...... -+..+-..",
    ".....+.. ...+..+-...+.... ...+...-",
    "++-.++-. ...+............ ....-.++",
    "....+..+ .+-.......-..... ..+...-.",
    ".+.+.+.+ ...+.+.....+...- .....+.-",
    "....+.-. ...+......+..... ....+.-.",
    ".....+++ ...+.+.....+.... ....-..+",
    "+...+... ..+.......+...-. .....++.",
    ".......+ .+-+.+....-+.-+- .....-..",
    "..++..++ +..-.-....---... ....-...",
)
_SCHEME_254 = (
    "..+-.-..+. -.........+.....+... ..+.+...",
    "....+..... .-...............+.. .+...+..",
    ".++-...... ...-+-+....-...-.... +..+....",
    "....+..... ...................+ ...+....",
    "..+-...... .+-+-+-...-+-+-+-... +...+...",
    ".++....... ...-.......-...-.... .+.-.+.-",
    "+..-+..... .+-.......-...-.-... .++.....",
    "+...+..... ..-.......-...-..... +.-.+.-.",
    ".+....-... ...+-+-+............ ...+....",
    "+.-....... +.....-.........-... +.-.....",
    "....++..-. .-..............+.+. ..+..-..",
    "+--...+... ...+..-............. ...++.-+",
    ".++.....-. ...+.+.....+...+.... ++...+.-",
    "..+-....+. +-+-.-..+.+-+-+-.... ++..+...",
    "+...+...-. ..+.......+...+.+... ++..+.-.",
    "+..-.-..+. +-+................. ..+.....",
    "..+-..+... ...+-+-....+........ ...+-...",
    "..+....... -+-+....-+-+-+-+.... .+......",
    "...+....-. +..-.-..+..-+..--... ++......",
    "+--....... ......+............. +.-++.-+",
    ".....+..-. ..+.......+.......-. ..+...+.",
    "+...+-...- ................-... ....+.-.",
    "..+-...-+. ...+.+..-.-+........ ....+...",
    "........+. .+.+.+.....+.+.+.... ++..++..",
    ".....+..-+ ................+.+. .....++.",
    "......+... ...-..++...-........ ...+...+",
    ".....+.-.. ...-......+......... ....+.-.",
    "......++-. ...+.+.....+........ ....+..+",
    ".++...--.. .....-.............. .....+.-",
    ".......+.. .....-...+.......... .....+..",
    ".........+ ...................+ .......+",
    "+--..-++.. ...-................ ....+.-+",
    "....+....- ................+-+. .....+..",
)


def _sum_program(rows):
    n_in = len(rows[0])
    rows = [{i: c for i, c in enumerate(row) if c} for row in rows]
    steps, ready = [], list(range(n_in))

    def emit(a, b, sign):
        steps.append((a, b, sign))
        ready.append(max(ready[a], ready[b]))
        return len(ready) - 1

    while True:
        count = {}
        for row in rows:
            items = sorted(row.items())
            for n, (a, x) in enumerate(items):
                for b, y in items[n + 1:]:
                    count[a, b, x * y] = count.get((a, b, x * y), 0) + 1
        best = max(sorted(count), key=count.get, default=None)
        if best is None or count[best] < 2:
            break
        a, b, sign = best
        new = emit(a, b, sign)
        for row in rows:
            if a in row and b in row and row[a] * row[b] == sign:
                row[new] = row.pop(a)
                del row[b]
    outs = []
    for row in rows:
        items = sorted(row.items(), key=lambda item: (ready[item[0]], item[0]))
        at, sign = items[0]
        for b, y in items[1:]:
            if sign < 0 < y:
                at, sign = emit(b, at, -1), 1
            else:
                at = emit(at, b, sign * y)
        outs.append((at, sign))
    return n_in, steps, ready, outs


def _evaluate(program, make):
    n_in, steps, ready, outs = program
    vals = {}
    for i in range(n_in):
        vals[i] = make(i)
        for n, (a, b, sign) in enumerate(steps):
            if ready[n_in + n] == i:
                vals[n_in + n] = vals[a] + vals[b] if sign > 0 else vals[a] - vals[b]
    return [vals[i] if sign > 0 else -vals[i] for i, sign in outs]


class _Scheme:
    def __init__(self, u, v, w):
        self.products = len(u)
        self.inner, self.outer = k, n = u.shape[1] // 2, w.shape[1] // 2
        want = np.zeros((2 * k, k * n, 2 * n), np.int64)
        for i, a, j in np.ndindex(2, k, n):
            want[k * i + a, n * a + j, n * i + j] = 1
        first = (u[:k * n, :k], v[:k * n], w[:k * n, :n])
        assert np.array_equal(np.einsum("ra,rb,rc->abc", u, v, w), want)
        assert np.array_equal(np.einsum("ra,rb,rc->abc", *first), want[:k, :, :n])
        self._left = {1: _sum_program(first[0].tolist()), 2: _sum_program(u.tolist())}
        self._right = _sum_program(v.tolist())
        self._out = {1: _sum_program(first[2].T.tolist()), 2: _sum_program(w.T.tolist())}

    def left(self, rows):
        blocks = [blk for row in rows for blk in _column_blocks(row, self.inner)]
        return _evaluate(self._left[len(rows)], blocks.__getitem__)

    def right(self, blocks):
        return _evaluate(self._right, blocks.__getitem__)

    def combine(self, n_rows, product):
        c = _evaluate(self._out[n_rows], product)
        return [c[self.outer * i:self.outer * (i + 1)] for i in range(n_rows)]


def _parse(table):
    return [np.array([[{"+": 1, ".": 0, "-": -1}[c] for c in line.split()[f]]
                      for line in table]) for f in range(3)]


def _swap_inner_outer(u, v, w):
    k, n = u.shape[1] // 2, w.shape[1] // 2
    return w, v.reshape(-1, k, n).transpose(0, 2, 1).reshape(-1, k * n), u


_SQUARE = _Scheme(*_parse(_SCHEME_244))
_FROM_MODEL = _Scheme(*_parse(_SCHEME_254))
_TO_MODEL = _Scheme(*_swap_inner_outer(*_parse(_SCHEME_254)))


def _column_blocks(x, count):
    pad = count * _BLOCK - x.shape[1]
    if pad:
        x = jnp.concatenate([x, jnp.zeros((x.shape[0], pad), x.dtype)], axis=1)
    return [x[:, i * _BLOCK:(i + 1) * _BLOCK] for i in range(count)]


def _masks(n_mem, length, n_seq):
    rows = n_seq * length

    def describe(axis):
        i = lax.broadcasted_iota(jnp.int32, (rows, rows), axis)
        second = i >= length
        return jnp.where(second, 1, 0), jnp.where(second, i - length, i)

    (seq_r, idx_r), (seq_c, idx_c) = describe(0), describe(1)
    same = seq_r == seq_c
    keep = same & ((idx_r < n_mem) | (idx_r >= idx_c))
    fill = jnp.where(same, _MASKED * _LOG2E, -jnp.inf).astype(_F32)
    return keep, fill


def _attention(hs, keep, fill, qkv, wo, n_heads, dh):
    scale = dh ** -0.5
    n_groups = n_heads // _GROUP
    n_seq, length = len(hs), hs[0].shape[0]
    heads = [slice(i * dh, (i + 1) * dh) for i in range(_GROUP)]
    lhs_dtype = _BF16 if (n_seq * length) % 16 == 0 else _F32

    h_terms = _FROM_MODEL.left(hs)

    def project(ws, g):
        c = _FROM_MODEL.combine(n_seq, lambda i: _dot(h_terms[i], jnp.concatenate(
            [_unpack(qkv[w, g, i]) for w in ws], axis=1)))
        return [jnp.concatenate(
            [jnp.concatenate([blk[:, n * dh:(n + 1) * dh] for blk in row], axis=1) for row in c],
            axis=0) for n in range(len(ws))]

    def weights(q, k):
        out = []
        for cols in heads:
            s = jnp.where(keep, _dot_nt(q[:, cols], k[:, cols]) * (scale * _LOG2E), fill)
            e = jnp.exp2(s - jnp.max(s, axis=-1, keepdims=True))
            out.append((e.astype(lhs_dtype), 1.0 / jnp.sum(e, axis=-1, keepdims=True)))
        return out

    def mix(p, v):
        return jnp.concatenate(
            [_dot(e, v[:, cols]) * inv for (e, inv), cols in zip(p, heads)], axis=1)

    def output(o, g, acc):
        terms = _TO_MODEL.left([o[i * length:(i + 1) * length] for i in range(n_seq)])

        def product(i):
            part = _dot(terms[i], _unpack(wo[g, i]))
            return part if acc is None else acc[i] + part

        if g < n_groups - 1:
            return [product(i) for i in range(len(terms))]
        return _TO_MODEL.combine(n_seq, product)

    proj, p, o, acc = {}, {}, {}, None
    for stage in range(n_groups + max(lag for _, lag in _STAGE_ORDER)):
        for task, lag in _STAGE_ORDER:
            g = stage - lag
            if not 0 <= g < n_groups:
                continue
            if task == "scores":
                p[g] = weights(proj.pop((0, g)), proj.pop((1, g)))
            elif task == "mix":
                o[g] = mix(p.pop(g), proj.pop((2, g)))
            elif task == "output":
                acc = output(o.pop(g), g, acc)
            else:
                for w, x in zip(task, project(task, g)):
                    proj[w, g] = x.astype(lhs_dtype if w == 0 else _BF16)
    return [jnp.concatenate(row, axis=1)[:, :hs[0].shape[1]] for row in acc]


def _silu(x):
    half = 0.5 * x
    return half + half * jnp.tanh(half)


def _swiglu_one(xn, w1, w3, w2_t, chunks):
    acc = hid = None
    for n in range(len(chunks) + 1):
        prev = hid
        if n < len(chunks):
            gate = _silu(_dot(xn, w1[:, chunks[n]]))
            hid = (gate * _dot(xn, w3[:, chunks[n]])).astype(_BF16)
        if n >= 1:
            part = _dot_nt(w2_t[:, chunks[n - 1]], prev)
            acc = part if acc is None else acc + part
    return acc


def _swiglu_pair(x_terms, w1_terms, w3_terms, w2_terms, side_work):
    def project(terms, lo):
        c = _FROM_MODEL.combine(2, lambda i: _dot(x_terms[i], _unpack(terms[lo // _BLOCK, i])))
        return [jnp.concatenate(row, axis=1) for row in c]

    def hidden(lo):
        gates = [_silu(g) for g in project(w1_terms, lo)]
        hid = [g * u for g, u in zip(gates, project(w3_terms, lo))]
        return [t.astype(_BF16) for t in _SQUARE.left(hid)]

    chunks = list(range(0, w2_terms.shape[0] * _BLOCK, _PAIR_CHUNK))
    acc = hid = None
    for n in range(len(chunks) + 1):
        prev = hid
        if n < len(chunks):
            tiles = [hidden(lo) for lo in range(chunks[n], chunks[n] + _PAIR_CHUNK, _BLOCK)]
            hid = [jnp.concatenate(t, axis=1) for t in zip(*tiles)]
        if n >= 1:
            first = chunks[n - 1] // _BLOCK

            def product(i, first=first, prev=prev, acc=acc):
                left = [_unpack(w2_terms[first + c, i]) for c in range(_PAIR_CHUNK // _BLOCK)]
                part = _dot_nt(jnp.concatenate(left, axis=1), prev[i])
                return part if acc is None else acc[i] + part

            if n < len(chunks):
                acc = [product(i) for i in range(_SQUARE.products)]
            else:
                acc = _SQUARE.combine(2, product)
        side_work(n)
    return [jnp.concatenate(row, axis=0) for row in acc]


def _store_terms(w, terms, scheme, transposed):
    block_rows, block_cols = 2 * terms.shape[2], terms.shape[0] * _BLOCK

    def tile(j, carry):
        def block(r, c, lo):
            start = r * block_rows + j * 16
            rows = pl.ds(pl.multiple_of(jnp.minimum(start, w.shape[0] - 16), 16), 16)
            words = pltpu.bitcast(
                w[rows, c * block_cols + lo:c * block_cols + lo + _BLOCK], jnp.uint32)
            if (r + 1) * block_rows > w.shape[0]:
                words = jnp.where(start < w.shape[0], words, jnp.uint32(0))
            return words

        for lo in range(0, block_cols, _BLOCK):
            words = [block(n, k, lo) if transposed else block(k, n, lo)
                     for k in range(scheme.inner) for n in range(scheme.outer)]
            even, odd = (scheme.right(rows) for rows in zip(*map(_split_words, words)))
            for i, pair in enumerate(zip(even, odd)):
                terms[lo // _BLOCK, i, pl.ds(pl.multiple_of(j * 8, 8), 8)] = (
                    pltpu.pack_elementwise(pair, packed_dtype=_BF16))
        return carry

    lax.fori_loop(0, block_rows // 16, tile, 0)


def _load_weights(sources, qkv, wo_hbm, wo, stage, wo_stage, wsem, osem,
                  later_copies):
    d_model, n_heads, dh = sources[0].shape
    n_groups = n_heads // _GROUP
    per_weight = _BLOCK // _WCHUNK
    n_jobs = len(sources) * per_weight
    full = _FROM_MODEL.inner - 1
    ragged = (d_model - full * _BLOCK) // _WCHUNK
    stage[ragged:, full] = jnp.zeros((per_weight - ragged,) + stage.shape[2:], stage.dtype)

    def for_copies(src, job, action):
        c = job % per_weight

        def copy(n):
            action(pltpu.make_async_copy(src.at[pl.ds(n * _BLOCK + c * _WCHUNK, _WCHUNK)],
                                         stage.at[c, n], wsem.at[(full + 1) * c + n]))

        for n in range(full):
            copy(n)
        pl.when(c < ragged)(functools.partial(copy, full))

    def start(job):
        for i, src in enumerate(sources):
            pl.when(job // per_weight == i)(
                functools.partial(for_copies, src, job, lambda c: c.start()))

    def wait(job):
        for i, src in enumerate(sources):
            pl.when(job // per_weight == i)(
                functools.partial(for_copies, src, job, lambda c: c.wait()))

    def split_heads(slot, n, j):
        rows = pl.ds(pl.multiple_of(j * 16, 16), 16)
        words = jnp.swapaxes(pltpu.bitcast(stage[slot, n, rows], jnp.uint32), 0, 1)
        return [half for p in range(n_heads // 2) for half in _split_words(words[p])]

    def output_group(g, carry):
        def transposed(head):
            last = jnp.concatenate(
                [wo_stage[head, full * _BLOCK:],
                 jnp.zeros(((full + 1) * _BLOCK - d_model, dh), wo_stage.dtype)], axis=0)
            return jnp.concatenate([wo_stage[head, :full * _BLOCK].T, last.T], axis=1)

        heads = [transposed(_GROUP * g + i) for i in range(_GROUP)]
        for r in range(0, dh, 16):
            blocks = [blk for h in heads
                      for blk in _column_blocks(h[r:r + 16].astype(_F32), _TO_MODEL.outer)]
            for i, t in enumerate(_TO_MODEL.right(blocks)):
                wo[g, i, r // 2:r // 2 + 8] = _pack(t)
        return carry

    wo_copy = pltpu.make_async_copy(wo_hbm, wo_stage, osem)
    lax.fori_loop(0, _INFLIGHT, lambda job, carry: start(job), None)
    wo_copy.start()

    def groups_done(job):
        return jnp.minimum(2 * jnp.maximum(job - _WO_FROM, 0), n_groups)

    def run(job, carry):
        which, c = job // per_weight, job % per_weight
        wait(job)
        start(job + _INFLIGHT)

        @pl.when(job == n_jobs - _LATER_FROM)
        def _():
            for copy in later_copies:
                copy.start()


        def main_rows(j, carry):
            rows = pl.ds(pl.multiple_of(c * (_WCHUNK // 2) + j * 8, 8), 8)
            parts = [split_heads(c, n, j) for n in range(full + 1)]
            for g in range(n_groups):
                blocks = [h for part in parts for h in part[_GROUP * g:_GROUP * (g + 1)]]
                for n, t in enumerate(_FROM_MODEL.right(blocks)):
                    qkv[which, g, n, rows] = _pack(t)
            return carry

        lax.fori_loop(0, _WCHUNK // 16, main_rows, 0)
        pl.when(job == _WO_FROM)(wo_copy.wait)
        lax.fori_loop(groups_done(job), groups_done(job + 1), output_group, 0)
        return carry

    lax.fori_loop(0, n_jobs, run, 0)


def _kernel(x0_ref, x_next_ref, mem0_ref, wq_hbm, wk_hbm, wv_hbm, wo_hbm, w1_hbm, w3_hbm,
            w2_hbm, out_ref,
            stage, wo_stage, qkv, wo,
            w1, w3, w2_t, w1_terms, w3_terms, w2_terms, res, normed, mem, acc_t, x_terms, wsem, osem, fsem, *, seg):
    b = pl.program_id(0)
    n_blocks = pl.num_programs(0) - 1
    _, n_heads, dh = wq_hbm.shape
    n_mem = mem0_ref.shape[0]
    n_chunks = w1.shape[1] // _FCHUNK
    steps = _TOK // seg
    ffn_copies = [pltpu.make_async_copy(s, d, fsem.at[i])
                  for i, (s, d) in enumerate(((w1_hbm, w1), (w3_hbm, w3), (w2_hbm, w2_t)))]

    def start_layer(slot, x):
        res[slot] = x
        normed[slot] = _layernorm(x)

    def prepare_swiglu(rows):
        xs = [_layernorm(res[i, rows]) for i in range(2)]
        for i, t in enumerate(_FROM_MODEL.left(xs)):
            x_terms[i, rows] = t.astype(_BF16)

    @pl.when(b == 0)
    def _():
        _load_weights((wq_hbm, wk_hbm, wv_hbm), qkv, wo_hbm, wo,
                      stage, wo_stage, wsem, osem, ffn_copies)
        mem[0] = mem0_ref[...].astype(_F32)
        mem[1] = mem0_ref[...].astype(_F32)
        start_layer(0, x0_ref[...].astype(_F32).T)

    def run_attention(first, n_seq):
        keep, fill = _masks(n_mem, n_mem + seg, n_seq)

        def segment(j, carry):
            rows = pl.ds(pl.multiple_of(j * seg, seg), seg)
            if n_seq == 2:
                done = pl.ds(pl.multiple_of(jnp.maximum(j - 1, 0) * seg, seg), seg)
                prepare_swiglu(done)
            hs = [jnp.concatenate([mem[first + i], normed[first + i, rows]], axis=0)
                  for i in range(n_seq)]
            for i, out in enumerate(_attention(hs, keep, fill, qkv, wo, n_heads, dh)):
                mem[first + i] = out[:n_mem]
                res[first + i, rows] += out[n_mem:]
            return carry

        lax.fori_loop(0, steps, segment, 0)

    both = jnp.logical_and(b > 0, b < n_blocks)

    @pl.when(both)
    def _():
        run_attention(0, 2)
        prepare_swiglu(pl.ds(_TOK - seg, seg))

        def side_work(n):
            if n == 0:
                acc_t[...] = res[1].T
                res[1] = res[0]
            if n == 1:
                start_layer(0, x_next_ref[...].astype(_F32).T)

        f2, f4 = _swiglu_pair(x_terms, w1_terms, w3_terms, w2_terms, side_work)
        start_layer(1, res[1] + f2.T)
        out_ref[...] = (acc_t[...] + f4).astype(out_ref.dtype)

    @pl.when(jnp.logical_not(both))
    def _():
        slot = jnp.where(b == 0, 0, 1)
        run_attention(slot, 1)

        @pl.when(b == 0)
        def _():
            for c, w, terms in zip(ffn_copies, (w1, w3, w2_t), (w1_terms, w3_terms, w2_terms)):
                c.wait()
                _store_terms(w, terms, _SQUARE if w is w2_t else _FROM_MODEL, w is w2_t)

        x = res[slot]
        xn = _layernorm(x).astype(_BF16)
        acc_t[...] = x.T

        def part(i, carry):
            chunks = [pl.ds(pl.multiple_of((i * _EDGE_CHUNKS + c) * _FCHUNK, _FCHUNK), _FCHUNK)
                      for c in range(_EDGE_CHUNKS)]
            acc_t[...] += _swiglu_one(xn, w1, w3, w2_t, chunks)
            return carry

        lax.fori_loop(0, n_chunks // _EDGE_CHUNKS, part, 0)

        @pl.when(b == 0)
        def _():
            start_layer(1, acc_t[...].T)
            start_layer(0, x_next_ref[...].astype(_F32).T)

        @pl.when(b > 0)
        def _():
            out_ref[...] = acc_t[...].astype(out_ref.dtype)


@functools.partial(jax.jit, static_argnames=("A_seg_len",))
def pallas_interleave_layers__memory_aug_recurrent_mem_tr__glu_gated_swiglu__prompt_kernel(
    A_x: jax.Array,
    A_mem0: jax.Array,
    A_Wq: jax.Array,
    A_Wk: jax.Array,
    A_Wv: jax.Array,
    A_Wo: jax.Array,
    A_seg_len: int,
    B_x: jax.Array,
    B_w1: jax.Array,
    B_w3: jax.Array,
    B_w2: jax.Array,
):
    del B_x
    batch, seq, d_model = A_x.shape
    n_mem = A_mem0.shape[1]
    _, n_heads, dh = A_Wq.shape
    d_ff = B_w1.shape[1]
    seg = int(A_seg_len)
    assert batch == 1 and seq % _TOK == 0 and _TOK % seg == 0 and seg % 16 == 0
    assert n_mem == 8 and n_heads % _GROUP == 0 and d_ff % (_FCHUNK * _EDGE_CHUNKS) == 0
    slots = _BLOCK // _WCHUNK
    assert _INFLIGHT < slots and d_model % 64 == 0
    assert (_FROM_MODEL.inner - 1) * _BLOCK < d_model < _FROM_MODEL.inner * _BLOCK
    assert dh == _BLOCK and d_ff % (4 * _PAIR_CHUNK) == 0
    ff_tiles = d_ff // (4 * _BLOCK)
    n_blocks = seq // _TOK

    x_t = A_x[0].T
    hbm = pl.BlockSpec(memory_space=pl.ANY)
    out_t = pl.pallas_call(
        functools.partial(_kernel, seg=seg),
        grid=(n_blocks + 1,),
        in_specs=[
            pl.BlockSpec((d_model, _TOK), lambda b: (0, 0)),
            pl.BlockSpec((d_model, _TOK), lambda b: (0, jnp.minimum(b + 1, n_blocks - 1))),
            pl.BlockSpec((n_mem, d_model), lambda b: (0, 0)),
            hbm, hbm, hbm, hbm, hbm, hbm, hbm,
        ],
        out_specs=pl.BlockSpec((d_model, _TOK), lambda b: (0, jnp.maximum(b - 1, 0))),
        out_shape=jax.ShapeDtypeStruct((d_model, seq), A_x.dtype),
        scratch_shapes=[
            pltpu.VMEM((slots, _FROM_MODEL.inner, _WCHUNK, n_heads, dh), _BF16),
            pltpu.VMEM((n_heads, d_model, dh), _BF16),
            pltpu.VMEM((3, n_heads // _GROUP, _FROM_MODEL.products, _BLOCK // 2, dh), jnp.uint32),
            pltpu.VMEM((n_heads // _GROUP, _TO_MODEL.products, dh // 2, _BLOCK), jnp.uint32),
            pltpu.VMEM((d_model, d_ff), _BF16),
            pltpu.VMEM((d_model, d_ff), _BF16),
            pltpu.VMEM((d_model, d_ff), _BF16),
            *2 * [pltpu.VMEM((ff_tiles, _FROM_MODEL.products, _BLOCK // 2, _BLOCK), jnp.uint32)],
            pltpu.VMEM((ff_tiles, _SQUARE.products, d_model // 8, _BLOCK), jnp.uint32),
            pltpu.VMEM((2, _TOK, d_model), _F32),
            pltpu.VMEM((2, _TOK, d_model), _F32),
            pltpu.VMEM((2, n_mem, d_model), _F32),
            pltpu.VMEM((d_model, _TOK), _F32),
            pltpu.VMEM((_FROM_MODEL.products, _TOK, _BLOCK), _BF16),
            pltpu.SemaphoreType.DMA((slots * _FROM_MODEL.inner,)),
            pltpu.SemaphoreType.DMA(()),
            pltpu.SemaphoreType.DMA((3,)),
        ],
        compiler_params=pltpu.CompilerParams(
            dimension_semantics=("arbitrary",),
            vmem_limit_bytes=112 * 1024 * 1024,
        ),
    )(x_t, x_t, A_mem0[0], A_Wq, A_Wk, A_Wv, jnp.transpose(A_Wo, (0, 2, 1)),
      B_w1, B_w3, B_w2.T)
    return out_t.T[None]
```

```python
import functools

import jax
import jax.numpy as jnp
import numpy as np
from jax import lax
import jax.experimental.pallas as pl
import jax.experimental.pallas.tpu as pltpu

_BF16 = jnp.bfloat16
_F32 = jnp.float32
_NT = (((1,), (1,)), ((), ()))
_TOK = 128
_GROUP = 4
_WCHUNK = 32
_INFLIGHT = 3
_EDGE_TILES = 3
_BLOCK = 128
_WO_FROM = 5
_PAIR_CHUNK = 384
_LATER_FROM = 1
_STAGE_ORDER = (((0, 1), 0), ("mix", 1), ((2,), 0), ("scores", 0), ("output", 2))
_LOG2E = float(np.log2(np.e))
_MASKED = -1000000000.0


def _layernorm(x):
    m = jnp.mean(x, axis=-1, keepdims=True)
    c = x - m
    v = jnp.mean(c * c, axis=-1, keepdims=True)
    return c * lax.rsqrt(v + 1e-05)


def _dot(a, b):
    return lax.dot_general(a, b, (((1,), (0,)), ((), ())), preferred_element_type=_F32)


def _dot_nt(a, b):
    return lax.dot_general(a, b, _NT, preferred_element_type=_F32)


def _pack(x):
    return pltpu.bitcast(x.astype(_BF16), jnp.uint32)


def _split_words(words):
    return (pltpu.bitcast(words << 16, _F32),
            pltpu.bitcast(words & jnp.uint32(0xFFFF0000), _F32))


def _unpack(words):
    return pltpu.bitcast(words, _BF16)


_SCHEME_244 = (
    "...+.... +.......++..--.. .-......",
    "..+++..+ +.........-..... ..-.+...",
    ".+++.... ....+++......... +..-....",
    ".+.+.+.. ...+.......+...- ...-.-.+",
    "++-..... ......+......... -.+++.--",
    "+...+..+ .+-.......-...+. ..-..++.",
    "+.-..... +.....+......... +.-.....",
    "..++..+. +....-..++..-... -+..+...",
    "+....... .+.............. .++..--.",
    ".+...+.. ....++++...+...- ...+....",
    "++-..+.. ...+..-......... ...++.--",
    "..++.-.. ...++++....+.... ...+-...",
    "+..++..+ +.........-...+. ..+.....",
    ".+.+..-. .....+.......... -+...-.+",
    "..++.... +...---.++...... +...-...",
    "..+...+. +....-..+...-... +-......",
    "......+. .....+...-...... -+..+-..",
    ".....+.. ...+..+-...+.... ...+...-",
    "++-.++-. ...+............ ....-.++",
    "....+..+ .+-.......-..... ..+...-.",
    ".+.+.+.+ ...+.+.....+...- .....+.-",
    "....+.-. ...+......+..... ....+.-.",
    ".....+++ ...+.+.....+.... ....-..+",
    "+...+... ..+.......+...-. .....++.",
    ".......+ .+-+.+....-+.-+- .....-..",
    "..++..++ +..-.-....---... ....-...",
)
_SCHEME_254 = (
    "..+-.-..+. -.........+.....+... ..+.+...",
    "....+..... .-...............+.. .+...+..",
    ".++-...... ...-+-+....-...-.... +..+....",
    "....+..... ...................+ ...+....",
    "..+-...... .+-+-+-...-+-+-+-... +...+...",
    ".++....... ...-.......-...-.... .+.-.+.-",
    "+..-+..... .+-.......-...-.-... .++.....",
    "+...+..... ..-.......-...-..... +.-.+.-.",
    ".+....-... ...+-+-+............ ...+....",
    "+.-....... +.....-.........-... +.-.....",
    "....++..-. .-..............+.+. ..+..-..",
    "+--...+... ...+..-............. ...++.-+",
    ".++.....-. ...+.+.....+...+.... ++...+.-",
    "..+-....+. +-+-.-..+.+-+-+-.... ++..+...",
    "+...+...-. ..+.......+...+.+... ++..+.-.",
    "+..-.-..+. +-+................. ..+.....",
    "..+-..+... ...+-+-....+........ ...+-...",
    "..+....... -+-+....-+-+-+-+.... .+......",
    "...+....-. +..-.-..+..-+..--... ++......",
    "+--....... ......+............. +.-++.-+",
    ".....+..-. ..+.......+.......-. ..+...+.",
    "+...+-...- ................-... ....+.-.",
    "..+-...-+. ...+.+..-.-+........ ....+...",
    "........+. .+.+.+.....+.+.+.... ++..++..",
    ".....+..-+ ................+.+. .....++.",
    "......+... ...-..++...-........ ...+...+",
    ".....+.-.. ...-......+......... ....+.-.",
    "......++-. ...+.+.....+........ ....+..+",
    ".++...--.. .....-.............. .....+.-",
    ".......+.. .....-...+.......... .....+..",
    ".........+ ...................+ .......+",
    "+--..-++.. ...-................ ....+.-+",
    "....+....- ................+-+. .....+..",
)


def _sum_program(rows):
    n_in = len(rows[0])
    rows = [{i: c for i, c in enumerate(row) if c} for row in rows]
    steps, ready = [], list(range(n_in))

    def emit(a, b, sign):
        steps.append((a, b, sign))
        ready.append(max(ready[a], ready[b]))
        return len(ready) - 1

    while True:
        count = {}
        for row in rows:
            items = sorted(row.items())
            for n, (a, x) in enumerate(items):
                for b, y in items[n + 1:]:
                    count[a, b, x * y] = count.get((a, b, x * y), 0) + 1
        best = max(sorted(count), key=count.get, default=None)
        if best is None or count[best] < 2:
            break
        a, b, sign = best
        new = emit(a, b, sign)
        for row in rows:
            if a in row and b in row and row[a] * row[b] == sign:
                row[new] = row.pop(a)
                del row[b]
    outs = []
    for row in rows:
        items = sorted(row.items(), key=lambda item: (ready[item[0]], item[0]))
        at, sign = items[0]
        for b, y in items[1:]:
            if sign < 0 < y:
                at, sign = emit(b, at, -1), 1
            else:
                at = emit(at, b, sign * y)
        outs.append((at, sign))
    return n_in, steps, ready, outs


def _evaluate(program, make):
    n_in, steps, ready, outs = program
    vals = {}
    for i in range(n_in):
        vals[i] = make(i)
        for n, (a, b, sign) in enumerate(steps):
            if ready[n_in + n] == i:
                vals[n_in + n] = vals[a] + vals[b] if sign > 0 else vals[a] - vals[b]
    return [vals[i] if sign > 0 else -vals[i] for i, sign in outs]


class _Scheme:
    def __init__(self, u, v, w):
        self.products = len(u)
        self.inner, self.outer = k, n = u.shape[1] // 2, w.shape[1] // 2
        want = np.zeros((2 * k, k * n, 2 * n), np.int64)
        for i, a, j in np.ndindex(2, k, n):
            want[k * i + a, n * a + j, n * i + j] = 1
        first = (u[:k * n, :k], v[:k * n], w[:k * n, :n])
        assert np.array_equal(np.einsum("ra,rb,rc->abc", u, v, w), want)
        assert np.array_equal(np.einsum("ra,rb,rc->abc", *first), want[:k, :, :n])
        self._left = {1: _sum_program(first[0].tolist()), 2: _sum_program(u.tolist())}
        self._right = _sum_program(v.tolist())
        self._out = {1: _sum_program(first[2].T.tolist()), 2: _sum_program(w.T.tolist())}

    def left(self, rows):
        blocks = [blk for row in rows for blk in _column_blocks(row, self.inner)]
        return _evaluate(self._left[len(rows)], blocks.__getitem__)

    def right(self, blocks):
        return _evaluate(self._right, blocks.__getitem__)

    def combine(self, n_rows, product):
        c = _evaluate(self._out[n_rows], product)
        return [c[self.outer * i:self.outer * (i + 1)] for i in range(n_rows)]


def _parse(table):
    return [np.array([[{"+": 1, ".": 0, "-": -1}[c] for c in line.split()[f]]
                      for line in table]) for f in range(3)]


def _swap_inner_outer(u, v, w):
    k, n = u.shape[1] // 2, w.shape[1] // 2
    return w, v.reshape(-1, k, n).transpose(0, 2, 1).reshape(-1, k * n), u


_SQUARE = _Scheme(*_parse(_SCHEME_244))
_FROM_MODEL = _Scheme(*_parse(_SCHEME_254))
_TO_MODEL = _Scheme(*_swap_inner_outer(*_parse(_SCHEME_254)))


def _column_blocks(x, count):
    pad = count * _BLOCK - x.shape[1]
    if pad:
        x = jnp.concatenate([x, jnp.zeros((x.shape[0], pad), x.dtype)], axis=1)
    return [x[:, i * _BLOCK:(i + 1) * _BLOCK] for i in range(count)]


def _masks(n_mem, length, n_seq):
    rows = n_seq * length

    def describe(axis):
        i = lax.broadcasted_iota(jnp.int32, (rows, rows), axis)
        second = i >= length
        return jnp.where(second, 1, 0), jnp.where(second, i - length, i)

    (seq_r, idx_r), (seq_c, idx_c) = describe(0), describe(1)
    same = seq_r == seq_c
    keep = same & ((idx_r < n_mem) | (idx_r >= idx_c))
    fill = jnp.where(same, _MASKED * _LOG2E, -jnp.inf).astype(_F32)
    return keep, fill


def _attention(hs, keep, fill, qkv, wo, n_heads, dh):
    scale = dh ** -0.5
    n_groups = n_heads // _GROUP
    n_seq, length = len(hs), hs[0].shape[0]
    heads = [slice(i * dh, (i + 1) * dh) for i in range(_GROUP)]
    lhs_dtype = _BF16 if (n_seq * length) % 16 == 0 else _F32

    h_terms = _FROM_MODEL.left(hs)

    def project(ws, g):
        c = _FROM_MODEL.combine(n_seq, lambda i: _dot(h_terms[i], jnp.concatenate(
            [_unpack(qkv[w, g, i]) for w in ws], axis=1)))
        return [jnp.concatenate(
            [jnp.concatenate([blk[:, n * dh:(n + 1) * dh] for blk in row], axis=1) for row in c],
            axis=0) for n in range(len(ws))]

    def weights(q, k):
        out = []
        for cols in heads:
            s = jnp.where(keep, _dot_nt(q[:, cols], k[:, cols]) * (scale * _LOG2E), fill)
            e = jnp.exp2(s - jnp.max(s, axis=-1, keepdims=True))
            out.append((e.astype(lhs_dtype), 1.0 / jnp.sum(e, axis=-1, keepdims=True)))
        return out

    def mix(p, v):
        return jnp.concatenate(
            [_dot(e, v[:, cols]) * inv for (e, inv), cols in zip(p, heads)], axis=1)

    def output(o, g, acc):
        terms = _TO_MODEL.left([o[i * length:(i + 1) * length] for i in range(n_seq)])

        def product(i):
            part = _dot(terms[i], _unpack(wo[g, i]))
            return part if acc is None else acc[i] + part

        if g < n_groups - 1:
            return [product(i) for i in range(len(terms))]
        return _TO_MODEL.combine(n_seq, product)

    proj, p, o, acc = {}, {}, {}, None
    for stage in range(n_groups + max(lag for _, lag in _STAGE_ORDER)):
        for task, lag in _STAGE_ORDER:
            g = stage - lag
            if not 0 <= g < n_groups:
                continue
            if task == "scores":
                p[g] = weights(proj.pop((0, g)), proj.pop((1, g)))
            elif task == "mix":
                o[g] = mix(p.pop(g), proj.pop((2, g)))
            elif task == "output":
                acc = output(o.pop(g), g, acc)
            else:
                for w, x in zip(task, project(task, g)):
                    proj[w, g] = x.astype(lhs_dtype if w == 0 else _BF16)
    return [jnp.concatenate(row, axis=1)[:, :hs[0].shape[1]] for row in acc]


def _silu(x):
    half = 0.5 * x
    return half + half * jnp.tanh(half)


def _swiglu_one(x_terms, w1_terms, w3_terms, w2_t, tiles):
    quarter = w2_t.shape[1] // _FROM_MODEL.outer

    def project(terms, tile):
        c = _FROM_MODEL.combine(2, lambda i: _dot(x_terms[i], _unpack(terms[tile, i])))
        return jnp.concatenate([jnp.concatenate(row, axis=1) for row in c], axis=0)

    acc = hid = None
    for n in range(len(tiles) + 1):
        prev = hid
        if n < len(tiles):
            gate = _silu(project(w1_terms, tiles[n]))
            hid = (gate * project(w3_terms, tiles[n])).astype(_BF16)
        if n >= 1:
            starts = [pl.multiple_of(j * quarter + tiles[n - 1] * _BLOCK, _BLOCK)
                      for j in range(_FROM_MODEL.outer)]
            part = _dot_nt(
                jnp.concatenate([w2_t[:, pl.ds(c, _BLOCK)] for c in starts], axis=1), prev)
            acc = part if acc is None else acc + part
    return acc


def _swiglu_pair(x_terms, w1_terms, w3_terms, w2_terms, side_work):
    def project(terms, lo):
        c = _FROM_MODEL.combine(2, lambda i: _dot(x_terms[i], _unpack(terms[lo // _BLOCK, i])))
        return [jnp.concatenate(row, axis=1) for row in c]

    def hidden(lo):
        gates = [_silu(g) for g in project(w1_terms, lo)]
        hid = [g * u for g, u in zip(gates, project(w3_terms, lo))]
        return [t.astype(_BF16) for t in _SQUARE.left(hid)]

    chunks = list(range(0, w2_terms.shape[0] * _BLOCK, _PAIR_CHUNK))
    acc = hid = None
    for n in range(len(chunks) + 1):
        prev = hid
        if n < len(chunks):
            tiles = [hidden(lo) for lo in range(chunks[n], chunks[n] + _PAIR_CHUNK, _BLOCK)]
            hid = [jnp.concatenate(t, axis=1) for t in zip(*tiles)]
        if n >= 1:
            first = chunks[n - 1] // _BLOCK

            def product(i, first=first, prev=prev, acc=acc):
                left = [_unpack(w2_terms[first + c, i]) for c in range(_PAIR_CHUNK // _BLOCK)]
                part = _dot_nt(jnp.concatenate(left, axis=1), prev[i])
                return part if acc is None else acc[i] + part

            if n < len(chunks):
                acc = [product(i) for i in range(_SQUARE.products)]
            else:
                acc = _SQUARE.combine(2, product)
        side_work(n)
    return [jnp.concatenate(row, axis=0) for row in acc]


def _store_terms(w, terms, scheme, transposed):
    block_rows, block_cols = 2 * terms.shape[2], terms.shape[0] * _BLOCK

    def tile(j, carry):
        def block(r, c, lo):
            start = r * block_rows + j * 16
            rows = pl.ds(pl.multiple_of(jnp.minimum(start, w.shape[0] - 16), 16), 16)
            words = pltpu.bitcast(
                w[rows, c * block_cols + lo:c * block_cols + lo + _BLOCK], jnp.uint32)
            if (r + 1) * block_rows > w.shape[0]:
                words = jnp.where(start < w.shape[0], words, jnp.uint32(0))
            return words

        for lo in range(0, block_cols, _BLOCK):
            words = [block(n, k, lo) if transposed else block(k, n, lo)
                     for k in range(scheme.inner) for n in range(scheme.outer)]
            even, odd = (scheme.right(rows) for rows in zip(*map(_split_words, words)))
            for i, pair in enumerate(zip(even, odd)):
                terms[lo // _BLOCK, i, pl.ds(pl.multiple_of(j * 8, 8), 8)] = (
                    pltpu.pack_elementwise(pair, packed_dtype=_BF16))
        return carry

    lax.fori_loop(0, block_rows // 16, tile, 0)


def _load_weights(sources, qkv, wo_hbm, wo, stage, wo_stage, wsem, osem,
                  later_copies):
    d_model, n_heads, dh = sources[0].shape
    n_groups = n_heads // _GROUP
    per_weight = _BLOCK // _WCHUNK
    n_jobs = len(sources) * per_weight
    full = _FROM_MODEL.inner - 1
    ragged = (d_model - full * _BLOCK) // _WCHUNK
    stage[ragged:, full] = jnp.zeros((per_weight - ragged,) + stage.shape[2:], stage.dtype)

    def for_copies(src, job, action):
        c = job % per_weight

        def copy(n):
            action(pltpu.make_async_copy(src.at[pl.ds(n * _BLOCK + c * _WCHUNK, _WCHUNK)],
                                         stage.at[c, n], wsem.at[(full + 1) * c + n]))

        for n in range(full):
            copy(n)
        pl.when(c < ragged)(functools.partial(copy, full))

    def start(job):
        for i, src in enumerate(sources):
            pl.when(job // per_weight == i)(
                functools.partial(for_copies, src, job, lambda c: c.start()))

    def wait(job):
        for i, src in enumerate(sources):
            pl.when(job // per_weight == i)(
                functools.partial(for_copies, src, job, lambda c: c.wait()))

    def split_heads(slot, n, j):
        rows = pl.ds(pl.multiple_of(j * 16, 16), 16)
        words = jnp.swapaxes(pltpu.bitcast(stage[slot, n, rows], jnp.uint32), 0, 1)
        return [half for p in range(n_heads // 2) for half in _split_words(words[p])]

    def output_group(g, carry):
        def transposed(head):
            last = jnp.concatenate(
                [wo_stage[head, full * _BLOCK:],
                 jnp.zeros(((full + 1) * _BLOCK - d_model, dh), wo_stage.dtype)], axis=0)
            return jnp.concatenate([wo_stage[head, :full * _BLOCK].T, last.T], axis=1)

        heads = [transposed(_GROUP * g + i) for i in range(_GROUP)]
        for r in range(0, dh, 16):
            blocks = [blk for h in heads
                      for blk in _column_blocks(h[r:r + 16].astype(_F32), _TO_MODEL.outer)]
            for i, t in enumerate(_TO_MODEL.right(blocks)):
                wo[g, i, r // 2:r // 2 + 8] = _pack(t)
        return carry

    wo_copy = pltpu.make_async_copy(wo_hbm, wo_stage, osem)
    lax.fori_loop(0, _INFLIGHT, lambda job, carry: start(job), None)
    wo_copy.start()

    def groups_done(job):
        return jnp.minimum(2 * jnp.maximum(job - _WO_FROM, 0), n_groups)

    def run(job, carry):
        which, c = job // per_weight, job % per_weight
        wait(job)
        start(job + _INFLIGHT)

        @pl.when(job == n_jobs - _LATER_FROM)
        def _():
            for copy in later_copies:
                copy.start()


        def main_rows(j, carry):
            rows = pl.ds(pl.multiple_of(c * (_WCHUNK // 2) + j * 8, 8), 8)
            parts = [split_heads(c, n, j) for n in range(full + 1)]
            for g in range(n_groups):
                blocks = [h for part in parts for h in part[_GROUP * g:_GROUP * (g + 1)]]
                for n, t in enumerate(_FROM_MODEL.right(blocks)):
                    qkv[which, g, n, rows] = _pack(t)
            return carry

        lax.fori_loop(0, _WCHUNK // 16, main_rows, 0)
        pl.when(job == _WO_FROM)(wo_copy.wait)
        lax.fori_loop(groups_done(job), groups_done(job + 1), output_group, 0)
        return carry

    lax.fori_loop(0, n_jobs, run, 0)


def _kernel(x0_ref, x_next_ref, mem0_ref, wq_hbm, wk_hbm, wv_hbm, wo_hbm, w1_hbm, w3_hbm,
            w2_hbm, out_ref,
            stage, wo_stage, qkv, wo,
            w1, w3, w2_t, w1_terms, w3_terms, w2_terms, res, normed, mem, acc_t, x_terms, wsem, osem, fsem, *, seg):
    b = pl.program_id(0)
    n_blocks = pl.num_programs(0) - 1
    _, n_heads, dh = wq_hbm.shape
    n_mem = mem0_ref.shape[0]
    steps = _TOK // seg
    ffn_copies = [pltpu.make_async_copy(s, d, fsem.at[i])
                  for i, (s, d) in enumerate(((w1_hbm, w1), (w3_hbm, w3), (w2_hbm, w2_t)))]

    def start_layer(slot, x):
        res[slot] = x
        normed[slot] = _layernorm(x)

    def prepare_swiglu(j):
        rows = pl.ds(pl.multiple_of(j * seg, seg), seg)
        for i, t in enumerate(_FROM_MODEL.left([_layernorm(res[n, rows]) for n in range(2)])):
            x_terms[i, rows] = t.astype(_BF16)

    @pl.when(b == 0)
    def _():
        _load_weights((wq_hbm, wk_hbm, wv_hbm), qkv, wo_hbm, wo,
                      stage, wo_stage, wsem, osem, ffn_copies)
        mem[0] = mem0_ref[...].astype(_F32)
        mem[1] = mem0_ref[...].astype(_F32)
        start_layer(0, x0_ref[...].astype(_F32).T)

    def run_attention(first, n_seq):
        keep, fill = _masks(n_mem, n_mem + seg, n_seq)

        def segment(j, carry):
            rows = pl.ds(pl.multiple_of(j * seg, seg), seg)
            if n_seq == 2:
                prepare_swiglu(jnp.maximum(j - 1, 0))
            hs = [jnp.concatenate([mem[first + i], normed[first + i, rows]], axis=0)
                  for i in range(n_seq)]
            for i, out in enumerate(_attention(hs, keep, fill, qkv, wo, n_heads, dh)):
                mem[first + i] = out[:n_mem]
                res[first + i, rows] += out[n_mem:]
            return carry

        lax.fori_loop(0, steps, segment, 0)

    both = jnp.logical_and(b > 0, b < n_blocks)

    @pl.when(both)
    def _():
        run_attention(0, 2)
        prepare_swiglu(steps - 1)

        def side_work(n):
            if n == 0:
                acc_t[...] = res[1].T
                res[1] = res[0]
            if n == 1:
                start_layer(0, x_next_ref[...].astype(_F32).T)

        f2, f4 = _swiglu_pair(x_terms, w1_terms, w3_terms, w2_terms, side_work)
        start_layer(1, res[1] + f2.T)
        out_ref[...] = (acc_t[...] + f4).astype(out_ref.dtype)

    @pl.when(jnp.logical_not(both))
    def _():
        slot = jnp.where(b == 0, 0, 1)
        run_attention(slot, 1)

        @pl.when(b == 0)
        def _():
            for c, w, terms in zip(ffn_copies, (w1, w3, w2_t), (w1_terms, w3_terms, w2_terms)):
                c.wait()
                _store_terms(w, terms, _SQUARE if w is w2_t else _FROM_MODEL, w is w2_t)

        x = res[slot]
        xn = _layernorm(x)
        terms = [t.astype(_BF16) for t in _FROM_MODEL.left([xn[:_TOK // 2], xn[_TOK // 2:]])]
        acc_t[...] = x.T

        def part(i, carry):
            tiles = [i * _EDGE_TILES + t for t in range(_EDGE_TILES)]
            acc_t[...] += _swiglu_one(terms, w1_terms, w3_terms, w2_t, tiles)
            return carry

        lax.fori_loop(0, w1_terms.shape[0] // _EDGE_TILES, part, 0)

        @pl.when(b == 0)
        def _():
            start_layer(1, acc_t[...].T)
            start_layer(0, x_next_ref[...].astype(_F32).T)

        @pl.when(b > 0)
        def _():
            out_ref[...] = acc_t[...].astype(out_ref.dtype)


@functools.partial(jax.jit, static_argnames=("A_seg_len",))
def pallas_interleave_layers__memory_aug_recurrent_mem_tr__glu_gated_swiglu__prompt_kernel(
    A_x: jax.Array,
    A_mem0: jax.Array,
    A_Wq: jax.Array,
    A_Wk: jax.Array,
    A_Wv: jax.Array,
    A_Wo: jax.Array,
    A_seg_len: int,
    B_x: jax.Array,
    B_w1: jax.Array,
    B_w3: jax.Array,
    B_w2: jax.Array,
):
    del B_x
    batch, seq, d_model = A_x.shape
    n_mem = A_mem0.shape[1]
    _, n_heads, dh = A_Wq.shape
    d_ff = B_w1.shape[1]
    seg = int(A_seg_len)
    assert batch == 1 and seq % _TOK == 0 and _TOK % seg == 0 and seg % 16 == 0
    assert n_mem == 8 and n_heads % _GROUP == 0 and d_ff % (4 * _BLOCK * _EDGE_TILES) == 0
    slots = _BLOCK // _WCHUNK
    assert _INFLIGHT < slots and d_model % 64 == 0
    assert (_FROM_MODEL.inner - 1) * _BLOCK < d_model < _FROM_MODEL.inner * _BLOCK
    assert dh == _BLOCK and d_ff % (4 * _PAIR_CHUNK) == 0
    ff_tiles = d_ff // (4 * _BLOCK)
    n_blocks = seq // _TOK

    x_t = A_x[0].T
    hbm = pl.BlockSpec(memory_space=pl.ANY)
    out_t = pl.pallas_call(
        functools.partial(_kernel, seg=seg),
        grid=(n_blocks + 1,),
        in_specs=[
            pl.BlockSpec((d_model, _TOK), lambda b: (0, 0)),
            pl.BlockSpec((d_model, _TOK), lambda b: (0, jnp.minimum(b + 1, n_blocks - 1))),
            pl.BlockSpec((n_mem, d_model), lambda b: (0, 0)),
            hbm, hbm, hbm, hbm, hbm, hbm, hbm,
        ],
        out_specs=pl.BlockSpec((d_model, _TOK), lambda b: (0, jnp.maximum(b - 1, 0))),
        out_shape=jax.ShapeDtypeStruct((d_model, seq), A_x.dtype),
        scratch_shapes=[
            pltpu.VMEM((slots, _FROM_MODEL.inner, _WCHUNK, n_heads, dh), _BF16),
            pltpu.VMEM((n_heads, d_model, dh), _BF16),
            pltpu.VMEM((3, n_heads // _GROUP, _FROM_MODEL.products, _BLOCK // 2, dh), jnp.uint32),
            pltpu.VMEM((n_heads // _GROUP, _TO_MODEL.products, dh // 2, _BLOCK), jnp.uint32),
            pltpu.VMEM((d_model, d_ff), _BF16),
            pltpu.VMEM((d_model, d_ff), _BF16),
            pltpu.VMEM((d_model, d_ff), _BF16),
            *2 * [pltpu.VMEM((ff_tiles, _FROM_MODEL.products, _BLOCK // 2, _BLOCK), jnp.uint32)],
            pltpu.VMEM((ff_tiles, _SQUARE.products, d_model // 8, _BLOCK), jnp.uint32),
            pltpu.VMEM((2, _TOK, d_model), _F32),
            pltpu.VMEM((2, _TOK, d_model), _F32),
            pltpu.VMEM((2, n_mem, d_model), _F32),
            pltpu.VMEM((d_model, _TOK), _F32),
            pltpu.VMEM((_FROM_MODEL.products, _TOK, _BLOCK), _BF16),
            pltpu.SemaphoreType.DMA((slots * _FROM_MODEL.inner,)),
            pltpu.SemaphoreType.DMA(()),
            pltpu.SemaphoreType.DMA((3,)),
        ],
        compiler_params=pltpu.CompilerParams(
            dimension_semantics=("arbitrary",),
            vmem_limit_bytes=112 * 1024 * 1024,
        ),
    )(x_t, x_t, A_mem0[0], A_Wq, A_Wk, A_Wv, jnp.transpose(A_Wo, (0, 2, 1)),
      B_w1, B_w3, B_w2.T)
    return out_t.T[None]
```

```python
import functools

import jax
import jax.numpy as jnp
import numpy as np
from jax import lax
import jax.experimental.pallas as pl
import jax.experimental.pallas.tpu as pltpu

_BF16 = jnp.bfloat16
_F32 = jnp.float32
_NT = (((1,), (1,)), ((), ()))
_TOK = 128
_GROUP = 4
_WCHUNK = 32
_INFLIGHT = 3
_EDGE_TILES = 3
_BLOCK = 128
_WO_FROM = 5
_PAIR_CHUNK = 384
_LATER_FROM = 1
_STAGE_ORDER = (((0, 1), 0), ("mix", 1), ((2,), 0), ("scores", 0), ("output", 2))
_LOG2E = float(np.log2(np.e))
_MASKED = -1000000000.0


def _layernorm(x):
    m = jnp.mean(x, axis=-1, keepdims=True)
    c = x - m
    v = jnp.mean(c * c, axis=-1, keepdims=True)
    return c * lax.rsqrt(v + 1e-05)


def _dot(a, b):
    return lax.dot_general(a, b, (((1,), (0,)), ((), ())), preferred_element_type=_F32)


def _dot_nt(a, b):
    return lax.dot_general(a, b, _NT, preferred_element_type=_F32)


def _pack(x):
    return pltpu.bitcast(x.astype(_BF16), jnp.uint32)


def _split_words(words):
    return (pltpu.bitcast(words << 16, _F32),
            pltpu.bitcast(words & jnp.uint32(0xFFFF0000), _F32))


def _unpack(words):
    return pltpu.bitcast(words, _BF16)


_SCHEME_244 = (
    "...+.... +.......++..--.. .-......",
    "..+++..+ +.........-..... ..-.+...",
    ".+++.... ....+++......... +..-....",
    ".+.+.+.. ...+.......+...- ...-.-.+",
    "++-..... ......+......... -.+++.--",
    "+...+..+ .+-.......-...+. ..-..++.",
    "+.-..... +.....+......... +.-.....",
    "..++..+. +....-..++..-... -+..+...",
    "+....... .+.............. .++..--.",
    ".+...+.. ....++++...+...- ...+....",
    "++-..+.. ...+..-......... ...++.--",
    "..++.-.. ...++++....+.... ...+-...",
    "+..++..+ +.........-...+. ..+.....",
    ".+.+..-. .....+.......... -+...-.+",
    "..++.... +...---.++...... +...-...",
    "..+...+. +....-..+...-... +-......",
    "......+. .....+...-...... -+..+-..",
    ".....+.. ...+..+-...+.... ...+...-",
    "++-.++-. ...+............ ....-.++",
    "....+..+ .+-.......-..... ..+...-.",
    ".+.+.+.+ ...+.+.....+...- .....+.-",
    "....+.-. ...+......+..... ....+.-.",
    ".....+++ ...+.+.....+.... ....-..+",
    "+...+... ..+.......+...-. .....++.",
    ".......+ .+-+.+....-+.-+- .....-..",
    "..++..++ +..-.-....---... ....-...",
)
_SCHEME_254 = (
    "..+-.-..+. -.........+.....+... ..+.+...",
    "....+..... .-...............+.. .+...+..",
    ".++-...... ...-+-+....-...-.... +..+....",
    "....+..... ...................+ ...+....",
    "..+-...... .+-+-+-...-+-+-+-... +...+...",
    ".++....... ...-.......-...-.... .+.-.+.-",
    "+..-+..... .+-.......-...-.-... .++.....",
    "+...+..... ..-.......-...-..... +.-.+.-.",
    ".+....-... ...+-+-+............ ...+....",
    "+.-....... +.....-.........-... +.-.....",
    "....++..-. .-..............+.+. ..+..-..",
    "+--...+... ...+..-............. ...++.-+",
    ".++.....-. ...+.+.....+...+.... ++...+.-",
    "..+-....+. +-+-.-..+.+-+-+-.... ++..+...",
    "+...+...-. ..+.......+...+.+... ++..+.-.",
    "+..-.-..+. +-+................. ..+.....",
    "..+-..+... ...+-+-....+........ ...+-...",
    "..+....... -+-+....-+-+-+-+.... .+......",
    "...+....-. +..-.-..+..-+..--... ++......",
    "+--....... ......+............. +.-++.-+",
    ".....+..-. ..+.......+.......-. ..+...+.",
    "+...+-...- ................-... ....+.-.",
    "..+-...-+. ...+.+..-.-+........ ....+...",
    "........+. .+.+.+.....+.+.+.... ++..++..",
    ".....+..-+ ................+.+. .....++.",
    "......+... ...-..++...-........ ...+...+",
    ".....+.-.. ...-......+......... ....+.-.",
    "......++-. ...+.+.....+........ ....+..+",
    ".++...--.. .....-.............. .....+.-",
    ".......+.. .....-...+.......... .....+..",
    ".........+ ...................+ .......+",
    "+--..-++.. ...-................ ....+.-+",
    "....+....- ................+-+. .....+..",
)


def _sum_program(rows):
    n_in = len(rows[0])
    rows = [{i: c for i, c in enumerate(row) if c} for row in rows]
    steps, ready = [], list(range(n_in))

    def emit(a, b, sign):
        steps.append((a, b, sign))
        ready.append(max(ready[a], ready[b]))
        return len(ready) - 1

    while True:
        count = {}
        for row in rows:
            items = sorted(row.items())
            for n, (a, x) in enumerate(items):
                for b, y in items[n + 1:]:
                    count[a, b, x * y] = count.get((a, b, x * y), 0) + 1
        best = max(sorted(count), key=count.get, default=None)
        if best is None or count[best] < 2:
            break
        a, b, sign = best
        new = emit(a, b, sign)
        for row in rows:
            if a in row and b in row and row[a] * row[b] == sign:
                row[new] = row.pop(a)
                del row[b]
    outs = []
    for row in rows:
        items = sorted(row.items(), key=lambda item: (ready[item[0]], item[0]))
        at, sign = items[0]
        for b, y in items[1:]:
            if sign < 0 < y:
                at, sign = emit(b, at, -1), 1
            else:
                at = emit(at, b, sign * y)
        outs.append((at, sign))
    return n_in, steps, ready, outs


def _evaluate(program, make):
    n_in, steps, ready, outs = program
    vals = {}
    for i in range(n_in):
        vals[i] = make(i)
        for n, (a, b, sign) in enumerate(steps):
            if ready[n_in + n] == i:
                vals[n_in + n] = vals[a] + vals[b] if sign > 0 else vals[a] - vals[b]
    return [vals[i] if sign > 0 else -vals[i] for i, sign in outs]


class _Scheme:
    def __init__(self, u, v, w):
        self.products = len(u)
        self.inner, self.outer = k, n = u.shape[1] // 2, w.shape[1] // 2
        want = np.zeros((2 * k, k * n, 2 * n), np.int64)
        for i, a, j in np.ndindex(2, k, n):
            want[k * i + a, n * a + j, n * i + j] = 1
        first = (u[:k * n, :k], v[:k * n], w[:k * n, :n])
        assert np.array_equal(np.einsum("ra,rb,rc->abc", u, v, w), want)
        assert np.array_equal(np.einsum("ra,rb,rc->abc", *first), want[:k, :, :n])
        self._left = {1: _sum_program(first[0].tolist()), 2: _sum_program(u.tolist())}
        self._right = _sum_program(v.tolist())
        self._out = {1: _sum_program(first[2].T.tolist()), 2: _sum_program(w.T.tolist())}

    def left(self, rows):
        blocks = [blk for row in rows for blk in _column_blocks(row, self.inner)]
        return _evaluate(self._left[len(rows)], blocks.__getitem__)

    def right(self, blocks):
        return _evaluate(self._right, blocks.__getitem__)

    def combine(self, n_rows, product):
        c = _evaluate(self._out[n_rows], product)
        return [c[self.outer * i:self.outer * (i + 1)] for i in range(n_rows)]


def _parse(table):
    return [np.array([[{"+": 1, ".": 0, "-": -1}[c] for c in line.split()[f]]
                      for line in table]) for f in range(3)]


def _swap_inner_outer(u, v, w):
    k, n = u.shape[1] // 2, w.shape[1] // 2
    return w, v.reshape(-1, k, n).transpose(0, 2, 1).reshape(-1, k * n), u


_SQUARE = _Scheme(*_parse(_SCHEME_244))
_FROM_MODEL = _Scheme(*_parse(_SCHEME_254))
_TO_MODEL = _Scheme(*_swap_inner_outer(*_parse(_SCHEME_254)))


def _column_blocks(x, count):
    pad = count * _BLOCK - x.shape[1]
    if pad:
        x = jnp.concatenate([x, jnp.zeros((x.shape[0], pad), x.dtype)], axis=1)
    return [x[:, i * _BLOCK:(i + 1) * _BLOCK] for i in range(count)]


def _masks(n_mem, length, n_seq):
    rows = n_seq * length

    def describe(axis):
        i = lax.broadcasted_iota(jnp.int32, (rows, rows), axis)
        second = i >= length
        return jnp.where(second, 1, 0), jnp.where(second, i - length, i)

    (seq_r, idx_r), (seq_c, idx_c) = describe(0), describe(1)
    same = seq_r == seq_c
    keep = same & ((idx_r < n_mem) | (idx_r >= idx_c))
    fill = jnp.where(same, _MASKED * _LOG2E, -jnp.inf).astype(_F32)
    return keep, fill


def _attention(hs, keep, fill, qkv, wo, h_terms, n_heads, dh):
    scale = dh ** -0.5
    n_groups = n_heads // _GROUP
    n_seq, length = len(hs), hs[0].shape[0]
    heads = [slice(i * dh, (i + 1) * dh) for i in range(_GROUP)]
    lhs_dtype = _BF16 if (n_seq * length) % 16 == 0 else _F32

    for i, t in enumerate(_FROM_MODEL.left(hs)):
        h_terms[i] = t

    def project(ws, g):
        c = _FROM_MODEL.combine(n_seq, lambda i: _dot(h_terms[i], jnp.concatenate(
            [_unpack(qkv[w, g, i]) for w in ws], axis=1)))
        return [jnp.concatenate(
            [jnp.concatenate([blk[:, n * dh:(n + 1) * dh] for blk in row], axis=1) for row in c],
            axis=0) for n in range(len(ws))]

    def weights(q, k):
        out = []
        for cols in heads:
            s = jnp.where(keep, _dot_nt(q[:, cols], k[:, cols]) * (scale * _LOG2E), fill)
            e = jnp.exp2(s - jnp.max(s, axis=-1, keepdims=True))
            out.append((e.astype(lhs_dtype), 1.0 / jnp.sum(e, axis=-1, keepdims=True)))
        return out

    def mix(p, v):
        return jnp.concatenate(
            [_dot(e, v[:, cols]) * inv for (e, inv), cols in zip(p, heads)], axis=1)

    def output(o, g, acc):
        terms = _TO_MODEL.left([o[i * length:(i + 1) * length] for i in range(n_seq)])

        def product(i):
            part = _dot(terms[i], _unpack(wo[g, i]))
            return part if acc is None else acc[i] + part

        if g < n_groups - 1:
            return [product(i) for i in range(len(terms))]
        return _TO_MODEL.combine(n_seq, product)

    proj, p, o, acc = {}, {}, {}, None
    for stage in range(n_groups + max(lag for _, lag in _STAGE_ORDER)):
        for task, lag in _STAGE_ORDER:
            g = stage - lag
            if not 0 <= g < n_groups:
                continue
            if task == "scores":
                p[g] = weights(proj.pop((0, g)), proj.pop((1, g)))
            elif task == "mix":
                o[g] = mix(p.pop(g), proj.pop((2, g)))
            elif task == "output":
                acc = output(o.pop(g), g, acc)
            else:
                for w, x in zip(task, project(task, g)):
                    proj[w, g] = x.astype(lhs_dtype if w == 0 else _BF16)
    return [jnp.concatenate(row, axis=1)[:, :hs[0].shape[1]] for row in acc]


def _silu(x):
    half = 0.5 * x
    return half + half * jnp.tanh(half)


def _swiglu_one(x_terms, w1_terms, w3_terms, w2_t, tiles):
    quarter = w2_t.shape[1] // _FROM_MODEL.outer

    def project(terms, tile):
        c = _FROM_MODEL.combine(2, lambda i: _dot(x_terms[i], _unpack(terms[tile, i])))
        return jnp.concatenate([jnp.concatenate(row, axis=1) for row in c], axis=0)

    acc = hid = None
    for n in range(len(tiles) + 1):
        prev = hid
        if n < len(tiles):
            gate = _silu(project(w1_terms, tiles[n]))
            hid = (gate * project(w3_terms, tiles[n])).astype(_BF16)
        if n >= 1:
            starts = [pl.multiple_of(j * quarter + tiles[n - 1] * _BLOCK, _BLOCK)
                      for j in range(_FROM_MODEL.outer)]
            part = _dot_nt(
                jnp.concatenate([w2_t[:, pl.ds(c, _BLOCK)] for c in starts], axis=1), prev)
            acc = part if acc is None else acc + part
    return acc


def _swiglu_pair(x_terms, w1_terms, w3_terms, w2_terms, side_work):
    def project(terms, lo):
        c = _FROM_MODEL.combine(2, lambda i: _dot(x_terms[i], _unpack(terms[lo // _BLOCK, i])))
        return [jnp.concatenate(row, axis=1) for row in c]

    def hidden(lo):
        gates = [_silu(g) for g in project(w1_terms, lo)]
        hid = [g * u for g, u in zip(gates, project(w3_terms, lo))]
        return [t.astype(_BF16) for t in _SQUARE.left(hid)]

    chunks = list(range(0, w2_terms.shape[0] * _BLOCK, _PAIR_CHUNK))
    acc = hid = None
    for n in range(len(chunks) + 1):
        prev = hid
        if n < len(chunks):
            tiles = [hidden(lo) for lo in range(chunks[n], chunks[n] + _PAIR_CHUNK, _BLOCK)]
            hid = [jnp.concatenate(t, axis=1) for t in zip(*tiles)]
        if n >= 1:
            first = chunks[n - 1] // _BLOCK

            def product(i, first=first, prev=prev, acc=acc):
                left = [_unpack(w2_terms[first + c, i]) for c in range(_PAIR_CHUNK // _BLOCK)]
                part = _dot_nt(jnp.concatenate(left, axis=1), prev[i])
                return part if acc is None else acc[i] + part

            if n < len(chunks):
                acc = [product(i) for i in range(_SQUARE.products)]
            else:
                acc = _SQUARE.combine(2, product)
        side_work(n)
    return [jnp.concatenate(row, axis=0) for row in acc]


def _store_terms(w, terms, scheme, transposed):
    block_rows, block_cols = 2 * terms.shape[2], terms.shape[0] * _BLOCK

    def tile(j, carry):
        def block(r, c, lo):
            start = r * block_rows + j * 16
            rows = pl.ds(pl.multiple_of(jnp.minimum(start, w.shape[0] - 16), 16), 16)
            words = pltpu.bitcast(
                w[rows, c * block_cols + lo:c * block_cols + lo + _BLOCK], jnp.uint32)
            if (r + 1) * block_rows > w.shape[0]:
                words = jnp.where(start < w.shape[0], words, jnp.uint32(0))
            return words

        for lo in range(0, block_cols, _BLOCK):
            words = [block(n, k, lo) if transposed else block(k, n, lo)
                     for k in range(scheme.inner) for n in range(scheme.outer)]
            even, odd = (scheme.right(rows) for rows in zip(*map(_split_words, words)))
            for i, pair in enumerate(zip(even, odd)):
                terms[lo // _BLOCK, i, pl.ds(pl.multiple_of(j * 8, 8), 8)] = (
                    pltpu.pack_elementwise(pair, packed_dtype=_BF16))
        return carry

    lax.fori_loop(0, block_rows // 16, tile, 0)


def _load_weights(sources, qkv, wo_hbm, wo, stage, wo_stage, wsem, osem,
                  later_copies):
    d_model, n_heads, dh = sources[0].shape
    n_groups = n_heads // _GROUP
    per_weight = _BLOCK // _WCHUNK
    n_jobs = len(sources) * per_weight
    full = _FROM_MODEL.inner - 1
    ragged = (d_model - full * _BLOCK) // _WCHUNK
    stage[ragged:, full] = jnp.zeros((per_weight - ragged,) + stage.shape[2:], stage.dtype)

    def for_copies(src, job, action):
        c = job % per_weight

        def copy(n):
            action(pltpu.make_async_copy(src.at[pl.ds(n * _BLOCK + c * _WCHUNK, _WCHUNK)],
                                         stage.at[c, n], wsem.at[(full + 1) * c + n]))

        for n in range(full):
            copy(n)
        pl.when(c < ragged)(functools.partial(copy, full))

    def start(job):
        for i, src in enumerate(sources):
            pl.when(job // per_weight == i)(
                functools.partial(for_copies, src, job, lambda c: c.start()))

    def wait(job):
        for i, src in enumerate(sources):
            pl.when(job // per_weight == i)(
                functools.partial(for_copies, src, job, lambda c: c.wait()))

    def split_heads(slot, n, j):
        rows = pl.ds(pl.multiple_of(j * 16, 16), 16)
        words = jnp.swapaxes(pltpu.bitcast(stage[slot, n, rows], jnp.uint32), 0, 1)
        return [half for p in range(n_heads // 2) for half in _split_words(words[p])]

    def output_group(g, carry):
        def transposed(head):
            last = jnp.concatenate(
                [wo_stage[head, full * _BLOCK:],
                 jnp.zeros(((full + 1) * _BLOCK - d_model, dh), wo_stage.dtype)], axis=0)
            return jnp.concatenate([wo_stage[head, :full * _BLOCK].T, last.T], axis=1)

        heads = [transposed(_GROUP * g + i) for i in range(_GROUP)]
        for r in range(0, dh, 16):
            blocks = [blk for h in heads
                      for blk in _column_blocks(h[r:r + 16].astype(_F32), _TO_MODEL.outer)]
            for i, t in enumerate(_TO_MODEL.right(blocks)):
                wo[g, i, r // 2:r // 2 + 8] = _pack(t)
        return carry

    wo_copy = pltpu.make_async_copy(wo_hbm, wo_stage, osem)
    lax.fori_loop(0, _INFLIGHT, lambda job, carry: start(job), None)
    wo_copy.start()

    def groups_done(job):
        return jnp.minimum(2 * jnp.maximum(job - _WO_FROM, 0), n_groups)

    def run(job, carry):
        which, c = job // per_weight, job % per_weight
        wait(job)
        start(job + _INFLIGHT)

        @pl.when(job == n_jobs - _LATER_FROM)
        def _():
            for copy in later_copies:
                copy.start()


        def main_rows(j, carry):
            rows = pl.ds(pl.multiple_of(c * (_WCHUNK // 2) + j * 8, 8), 8)
            parts = [split_heads(c, n, j) for n in range(full + 1)]
            for g in range(n_groups):
                blocks = [h for part in parts for h in part[_GROUP * g:_GROUP * (g + 1)]]
                for n, t in enumerate(_FROM_MODEL.right(blocks)):
                    qkv[which, g, n, rows] = _pack(t)
            return carry

        lax.fori_loop(0, _WCHUNK // 16, main_rows, 0)
        pl.when(job == _WO_FROM)(wo_copy.wait)
        lax.fori_loop(groups_done(job), groups_done(job + 1), output_group, 0)
        return carry

    lax.fori_loop(0, n_jobs, run, 0)


def _kernel(x0_ref, x_next_ref, mem0_ref, wq_hbm, wk_hbm, wv_hbm, wo_hbm, w1_hbm, w3_hbm,
            w2_hbm, out_ref,
            stage, wo_stage, qkv, wo,
            w1, w3, w2_t, w1_terms, w3_terms, w2_terms, res, normed, mem, acc_t, x_terms, h_terms, wsem, osem, fsem, *, seg):
    b = pl.program_id(0)
    n_blocks = pl.num_programs(0) - 1
    _, n_heads, dh = wq_hbm.shape
    n_mem = mem0_ref.shape[0]
    steps = _TOK // seg
    ffn_copies = [pltpu.make_async_copy(s, d, fsem.at[i])
                  for i, (s, d) in enumerate(((w1_hbm, w1), (w3_hbm, w3), (w2_hbm, w2_t)))]

    def start_layer(slot, x):
        res[slot] = x
        normed[slot] = _layernorm(x)

    def prepare_swiglu(j):
        rows = pl.ds(pl.multiple_of(j * seg, seg), seg)
        for i, t in enumerate(_FROM_MODEL.left([_layernorm(res[n, rows]) for n in range(2)])):
            x_terms[i, rows] = t.astype(_BF16)

    @pl.when(b == 0)
    def _():
        _load_weights((wq_hbm, wk_hbm, wv_hbm), qkv, wo_hbm, wo,
                      stage, wo_stage, wsem, osem, ffn_copies)
        mem[0] = mem0_ref[...].astype(_F32)
        mem[1] = mem0_ref[...].astype(_F32)
        start_layer(0, x0_ref[...].astype(_F32).T)

    def run_attention(first, n_seq):
        keep, fill = _masks(n_mem, n_mem + seg, n_seq)

        def segment(j, carry):
            rows = pl.ds(pl.multiple_of(j * seg, seg), seg)
            if n_seq == 2:
                prepare_swiglu(jnp.maximum(j - 1, 0))
            hs = [jnp.concatenate([mem[first + i], normed[first + i, rows]], axis=0)
                  for i in range(n_seq)]
            for i, out in enumerate(_attention(hs, keep, fill, qkv, wo, h_terms, n_heads, dh)):
                mem[first + i] = out[:n_mem]
                res[first + i, rows] += out[n_mem:]
            return carry

        lax.fori_loop(0, steps, segment, 0)

    both = jnp.logical_and(b > 0, b < n_blocks)

    @pl.when(both)
    def _():
        run_attention(0, 2)
        prepare_swiglu(steps - 1)

        def side_work(n):
            if n == 0:
                acc_t[...] = res[1].T
                res[1] = res[0]
            if n == 1:
                start_layer(0, x_next_ref[...].astype(_F32).T)

        f2, f4 = _swiglu_pair(x_terms, w1_terms, w3_terms, w2_terms, side_work)
        start_layer(1, res[1] + f2.T)
        out_ref[...] = (acc_t[...] + f4).astype(out_ref.dtype)

    @pl.when(jnp.logical_not(both))
    def _():
        slot = jnp.where(b == 0, 0, 1)
        run_attention(slot, 1)

        @pl.when(b == 0)
        def _():
            for c, w, terms in zip(ffn_copies, (w1, w3, w2_t), (w1_terms, w3_terms, w2_terms)):
                c.wait()
                _store_terms(w, terms, _SQUARE if w is w2_t else _FROM_MODEL, w is w2_t)

        x = res[slot]
        xn = _layernorm(x)
        terms = [t.astype(_BF16) for t in _FROM_MODEL.left([xn[:_TOK // 2], xn[_TOK // 2:]])]
        acc_t[...] = x.T

        def part(i, carry):
            tiles = [i * _EDGE_TILES + t for t in range(_EDGE_TILES)]
            acc_t[...] += _swiglu_one(terms, w1_terms, w3_terms, w2_t, tiles)
            return carry

        lax.fori_loop(0, w1_terms.shape[0] // _EDGE_TILES, part, 0)

        @pl.when(b == 0)
        def _():
            start_layer(1, acc_t[...].T)
            start_layer(0, x_next_ref[...].astype(_F32).T)

        @pl.when(b > 0)
        def _():
            out_ref[...] = acc_t[...].astype(out_ref.dtype)


@functools.partial(jax.jit, static_argnames=("A_seg_len",))
def pallas_interleave_layers__memory_aug_recurrent_mem_tr__glu_gated_swiglu__prompt_kernel(
    A_x: jax.Array,
    A_mem0: jax.Array,
    A_Wq: jax.Array,
    A_Wk: jax.Array,
    A_Wv: jax.Array,
    A_Wo: jax.Array,
    A_seg_len: int,
    B_x: jax.Array,
    B_w1: jax.Array,
    B_w3: jax.Array,
    B_w2: jax.Array,
):
    del B_x
    batch, seq, d_model = A_x.shape
    n_mem = A_mem0.shape[1]
    _, n_heads, dh = A_Wq.shape
    d_ff = B_w1.shape[1]
    seg = int(A_seg_len)
    assert batch == 1 and seq % _TOK == 0 and _TOK % seg == 0 and seg % 16 == 0
    assert n_mem == 8 and n_heads % _GROUP == 0 and d_ff % (4 * _BLOCK * _EDGE_TILES) == 0
    slots = _BLOCK // _WCHUNK
    assert _INFLIGHT < slots and d_model % 64 == 0
    assert (_FROM_MODEL.inner - 1) * _BLOCK < d_model < _FROM_MODEL.inner * _BLOCK
    assert dh == _BLOCK and d_ff % (4 * _PAIR_CHUNK) == 0
    ff_tiles = d_ff // (4 * _BLOCK)
    n_blocks = seq // _TOK

    x_t = A_x[0].T
    hbm = pl.BlockSpec(memory_space=pl.ANY)
    out_t = pl.pallas_call(
        functools.partial(_kernel, seg=seg),
        grid=(n_blocks + 1,),
        in_specs=[
            pl.BlockSpec((d_model, _TOK), lambda b: (0, 0)),
            pl.BlockSpec((d_model, _TOK), lambda b: (0, jnp.minimum(b + 1, n_blocks - 1))),
            pl.BlockSpec((n_mem, d_model), lambda b: (0, 0)),
            hbm, hbm, hbm, hbm, hbm, hbm, hbm,
        ],
        out_specs=pl.BlockSpec((d_model, _TOK), lambda b: (0, jnp.maximum(b - 1, 0))),
        out_shape=jax.ShapeDtypeStruct((d_model, seq), A_x.dtype),
        scratch_shapes=[
            pltpu.VMEM((slots, _FROM_MODEL.inner, _WCHUNK, n_heads, dh), _BF16),
            pltpu.VMEM((n_heads, d_model, dh), _BF16),
            pltpu.VMEM((3, n_heads // _GROUP, _FROM_MODEL.products, _BLOCK // 2, dh), jnp.uint32),
            pltpu.VMEM((n_heads // _GROUP, _TO_MODEL.products, dh // 2, _BLOCK), jnp.uint32),
            pltpu.VMEM((d_model, d_ff), _BF16),
            pltpu.VMEM((d_model, d_ff), _BF16),
            pltpu.VMEM((d_model, d_ff), _BF16),
            *2 * [pltpu.VMEM((ff_tiles, _FROM_MODEL.products, _BLOCK // 2, _BLOCK), jnp.uint32)],
            pltpu.VMEM((ff_tiles, _SQUARE.products, d_model // 8, _BLOCK), jnp.uint32),
            pltpu.VMEM((2, _TOK, d_model), _F32),
            pltpu.VMEM((2, _TOK, d_model), _F32),
            pltpu.VMEM((2, n_mem, d_model), _F32),
            pltpu.VMEM((d_model, _TOK), _F32),
            pltpu.VMEM((_FROM_MODEL.products, _TOK, _BLOCK), _BF16),
            pltpu.VMEM((_FROM_MODEL.products, n_mem + seg, _BLOCK), _F32),
            pltpu.SemaphoreType.DMA((slots * _FROM_MODEL.inner,)),
            pltpu.SemaphoreType.DMA(()),
            pltpu.SemaphoreType.DMA((3,)),
        ],
        compiler_params=pltpu.CompilerParams(
            dimension_semantics=("arbitrary",),
            vmem_limit_bytes=112 * 1024 * 1024,
        ),
    )(x_t, x_t, A_mem0[0], A_Wq, A_Wk, A_Wv, jnp.transpose(A_Wo, (0, 2, 1)),
      B_w1, B_w3, B_w2.T)
    return out_t.T[None]
```

```python
import functools

import jax
import jax.numpy as jnp
import numpy as np
from jax import lax
import jax.experimental.pallas as pl
import jax.experimental.pallas.tpu as pltpu

_BF16 = jnp.bfloat16
_F32 = jnp.float32
_NT = (((1,), (1,)), ((), ()))
_TOK = 128
_GROUP = 4
_WCHUNK = 32
_INFLIGHT = 3
_EDGE_TILES = 3
_BLOCK = 128
_WO_FROM = 5
_PAIR_CHUNK = 384
_LATER_FROM = 1
_STAGE_ORDER = (((0, 1), 0), ((2,), 0), ("mix", 1), ("scores", 0), ("output", 2))
_LOG2E = float(np.log2(np.e))
_MASKED = -1000000000.0


def _layernorm(x):
    m = jnp.mean(x, axis=-1, keepdims=True)
    c = x - m
    v = jnp.mean(c * c, axis=-1, keepdims=True)
    return c * lax.rsqrt(v + 1e-05)


def _dot(a, b):
    return lax.dot_general(a, b, (((1,), (0,)), ((), ())), preferred_element_type=_F32)


def _dot_nt(a, b):
    return lax.dot_general(a, b, _NT, preferred_element_type=_F32)


def _pack(x):
    return pltpu.bitcast(x.astype(_BF16), jnp.uint32)


def _split_words(words):
    return (pltpu.bitcast(words << 16, _F32),
            pltpu.bitcast(words & jnp.uint32(0xFFFF0000), _F32))


def _unpack(words):
    return pltpu.bitcast(words, _BF16)


_SCHEME_244 = (
    "...+.... +.......++..--.. .-......",
    "..+++..+ +.........-..... ..-.+...",
    ".+++.... ....+++......... +..-....",
    ".+.+.+.. ...+.......+...- ...-.-.+",
    "++-..... ......+......... -.+++.--",
    "+...+..+ .+-.......-...+. ..-..++.",
    "+.-..... +.....+......... +.-.....",
    "..++..+. +....-..++..-... -+..+...",
    "+....... .+.............. .++..--.",
    ".+...+.. ....++++...+...- ...+....",
    "++-..+.. ...+..-......... ...++.--",
    "..++.-.. ...++++....+.... ...+-...",
    "+..++..+ +.........-...+. ..+.....",
    ".+.+..-. .....+.......... -+...-.+",
    "..++.... +...---.++...... +...-...",
    "..+...+. +....-..+...-... +-......",
    "......+. .....+...-...... -+..+-..",
    ".....+.. ...+..+-...+.... ...+...-",
    "++-.++-. ...+............ ....-.++",
    "....+..+ .+-.......-..... ..+...-.",
    ".+.+.+.+ ...+.+.....+...- .....+.-",
    "....+.-. ...+......+..... ....+.-.",
    ".....+++ ...+.+.....+.... ....-..+",
    "+...+... ..+.......+...-. .....++.",
    ".......+ .+-+.+....-+.-+- .....-..",
    "..++..++ +..-.-....---... ....-...",
)
_SCHEME_254 = (
    "..+-.-..+. -.........+.....+... ..+.+...",
    "....+..... .-...............+.. .+...+..",
    ".++-...... ...-+-+....-...-.... +..+....",
    "....+..... ...................+ ...+....",
    "..+-...... .+-+-+-...-+-+-+-... +...+...",
    ".++....... ...-.......-...-.... .+.-.+.-",
    "+..-+..... .+-.......-...-.-... .++.....",
    "+...+..... ..-.......-...-..... +.-.+.-.",
    ".+....-... ...+-+-+............ ...+....",
    "+.-....... +.....-.........-... +.-.....",
    "....++..-. .-..............+.+. ..+..-..",
    "+--...+... ...+..-............. ...++.-+",
    ".++.....-. ...+.+.....+...+.... ++...+.-",
    "..+-....+. +-+-.-..+.+-+-+-.... ++..+...",
    "+...+...-. ..+.......+...+.+... ++..+.-.",
    "+..-.-..+. +-+................. ..+.....",
    "..+-..+... ...+-+-....+........ ...+-...",
    "..+....... -+-+....-+-+-+-+.... .+......",
    "...+....-. +..-.-..+..-+..--... ++......",
    "+--....... ......+............. +.-++.-+",
    ".....+..-. ..+.......+.......-. ..+...+.",
    "+...+-...- ................-... ....+.-.",
    "..+-...-+. ...+.+..-.-+........ ....+...",
    "........+. .+.+.+.....+.+.+.... ++..++..",
    ".....+..-+ ................+.+. .....++.",
    "......+... ...-..++...-........ ...+...+",
    ".....+.-.. ...-......+......... ....+.-.",
    "......++-. ...+.+.....+........ ....+..+",
    ".++...--.. .....-.............. .....+.-",
    ".......+.. .....-...+.......... .....+..",
    ".........+ ...................+ .......+",
    "+--..-++.. ...-................ ....+.-+",
    "....+....- ................+-+. .....+..",
)


def _sum_program(rows):
    n_in = len(rows[0])
    rows = [{i: c for i, c in enumerate(row) if c} for row in rows]
    steps, ready = [], list(range(n_in))

    def emit(a, b, sign):
        steps.append((a, b, sign))
        ready.append(max(ready[a], ready[b]))
        return len(ready) - 1

    while True:
        count = {}
        for row in rows:
            items = sorted(row.items())
            for n, (a, x) in enumerate(items):
                for b, y in items[n + 1:]:
                    count[a, b, x * y] = count.get((a, b, x * y), 0) + 1
        best = max(sorted(count), key=count.get, default=None)
        if best is None or count[best] < 2:
            break
        a, b, sign = best
        new = emit(a, b, sign)
        for row in rows:
            if a in row and b in row and row[a] * row[b] == sign:
                row[new] = row.pop(a)
                del row[b]
    outs = []
    for row in rows:
        items = sorted(row.items(), key=lambda item: (ready[item[0]], item[0]))
        at, sign = items[0]
        for b, y in items[1:]:
            if sign < 0 < y:
                at, sign = emit(b, at, -1), 1
            else:
                at = emit(at, b, sign * y)
        outs.append((at, sign))
    return n_in, steps, ready, outs


def _evaluate(program, make):
    n_in, steps, ready, outs = program
    vals = {}
    for i in range(n_in):
        vals[i] = make(i)
        for n, (a, b, sign) in enumerate(steps):
            if ready[n_in + n] == i:
                vals[n_in + n] = vals[a] + vals[b] if sign > 0 else vals[a] - vals[b]
    return [vals[i] if sign > 0 else -vals[i] for i, sign in outs]


class _Scheme:
    def __init__(self, u, v, w):
        self.products = len(u)
        self.inner, self.outer = k, n = u.shape[1] // 2, w.shape[1] // 2
        want = np.zeros((2 * k, k * n, 2 * n), np.int64)
        for i, a, j in np.ndindex(2, k, n):
            want[k * i + a, n * a + j, n * i + j] = 1
        first = (u[:k * n, :k], v[:k * n], w[:k * n, :n])
        assert np.array_equal(np.einsum("ra,rb,rc->abc", u, v, w), want)
        assert np.array_equal(np.einsum("ra,rb,rc->abc", *first), want[:k, :, :n])
        self._left = {1: _sum_program(first[0].tolist()), 2: _sum_program(u.tolist())}
        self._right = _sum_program(v.tolist())
        self._out = {1: _sum_program(first[2].T.tolist()), 2: _sum_program(w.T.tolist())}

    def left(self, rows):
        blocks = [blk for row in rows for blk in _column_blocks(row, self.inner)]
        return _evaluate(self._left[len(rows)], blocks.__getitem__)

    def right(self, blocks):
        return _evaluate(self._right, blocks.__getitem__)

    def combine(self, n_rows, product):
        c = _evaluate(self._out[n_rows], product)
        return [c[self.outer * i:self.outer * (i + 1)] for i in range(n_rows)]


def _parse(table):
    return [np.array([[{"+": 1, ".": 0, "-": -1}[c] for c in line.split()[f]]
                      for line in table]) for f in range(3)]


def _swap_inner_outer(u, v, w):
    k, n = u.shape[1] // 2, w.shape[1] // 2
    return w, v.reshape(-1, k, n).transpose(0, 2, 1).reshape(-1, k * n), u


_SQUARE = _Scheme(*_parse(_SCHEME_244))
_FROM_MODEL = _Scheme(*_parse(_SCHEME_254))
_TO_MODEL = _Scheme(*_swap_inner_outer(*_parse(_SCHEME_254)))


def _column_blocks(x, count):
    pad = count * _BLOCK - x.shape[1]
    if pad:
        x = jnp.concatenate([x, jnp.zeros((x.shape[0], pad), x.dtype)], axis=1)
    return [x[:, i * _BLOCK:(i + 1) * _BLOCK] for i in range(count)]


def _masks(n_mem, length, n_seq):
    rows = n_seq * length

    def describe(axis):
        i = lax.broadcasted_iota(jnp.int32, (rows, rows), axis)
        second = i >= length
        return jnp.where(second, 1, 0), jnp.where(second, i - length, i)

    (seq_r, idx_r), (seq_c, idx_c) = describe(0), describe(1)
    same = seq_r == seq_c
    keep = same & ((idx_r < n_mem) | (idx_r >= idx_c))
    fill = jnp.where(same, _MASKED * _LOG2E, -jnp.inf).astype(_F32)
    return keep, fill


def _attention(hs, keep, fill, qkv, wo, h_terms, o_sums,
               n_heads, dh):
    scale = dh ** -0.5
    n_groups = n_heads // _GROUP
    n_seq, length = len(hs), hs[0].shape[0]
    heads = [slice(i * dh, (i + 1) * dh) for i in range(_GROUP)]
    lhs_dtype = _BF16 if (n_seq * length) % 16 == 0 else _F32

    for i, t in enumerate(_FROM_MODEL.left(hs)):
        h_terms[i] = t

    def project(ws, g):
        c = _FROM_MODEL.combine(n_seq, lambda i: _dot(h_terms[i], jnp.concatenate(
            [_unpack(qkv[w, g, i]) for w in ws], axis=1)))
        return [jnp.concatenate(
            [jnp.concatenate([blk[:, n * dh:(n + 1) * dh] for blk in row], axis=1) for row in c],
            axis=0) for n in range(len(ws))]

    def weights(q, k):
        out = []
        for cols in heads:
            s = jnp.where(keep, _dot_nt(q[:, cols], k[:, cols]) * (scale * _LOG2E), fill)
            e = jnp.exp2(s - jnp.max(s, axis=-1, keepdims=True))
            out.append((e.astype(lhs_dtype), 1.0 / jnp.sum(e, axis=-1, keepdims=True)))
        return out

    def mix(p, v):
        return jnp.concatenate(
            [_dot(e, v[:, cols]) * inv for (e, inv), cols in zip(p, heads)], axis=1)

    def output(o, g):
        terms = _TO_MODEL.left([o[i * length:(i + 1) * length] for i in range(n_seq)])

        def product(i):
            part = _dot(terms[i], _unpack(wo[g, i]))
            return part if g == 0 else o_sums[i] + part

        if g == n_groups - 1:
            return _TO_MODEL.combine(n_seq, product)
        for i in range(len(terms)):
            o_sums[i] = product(i)

    proj, p, o, acc = {}, {}, {}, None
    for stage in range(n_groups + max(lag for _, lag in _STAGE_ORDER)):
        for task, lag in _STAGE_ORDER:
            g = stage - lag
            if not 0 <= g < n_groups:
                continue
            if task == "scores":
                p[g] = weights(proj.pop((0, g)), proj.pop((1, g)))
            elif task == "mix":
                o[g] = mix(p.pop(g), proj.pop((2, g)))
            elif task == "output":
                acc = output(o.pop(g), g)
            else:
                for w, x in zip(task, project(task, g)):
                    proj[w, g] = x.astype(lhs_dtype if w == 0 else _BF16)
    return [jnp.concatenate(row, axis=1)[:, :hs[0].shape[1]] for row in acc]


def _silu(x):
    half = 0.5 * x
    return half + half * jnp.tanh(half)


def _swiglu_one(x_terms, w1_terms, w3_terms, w2_t, tiles):
    quarter = w2_t.shape[1] // _FROM_MODEL.outer

    def project(terms, tile):
        c = _FROM_MODEL.combine(2, lambda i: _dot(x_terms[i], _unpack(terms[tile, i])))
        return jnp.concatenate([jnp.concatenate(row, axis=1) for row in c], axis=0)

    acc = hid = None
    for n in range(len(tiles) + 1):
        prev = hid
        if n < len(tiles):
            gate = _silu(project(w1_terms, tiles[n]))
            hid = (gate * project(w3_terms, tiles[n])).astype(_BF16)
        if n >= 1:
            starts = [pl.multiple_of(j * quarter + tiles[n - 1] * _BLOCK, _BLOCK)
                      for j in range(_FROM_MODEL.outer)]
            part = _dot_nt(
                jnp.concatenate([w2_t[:, pl.ds(c, _BLOCK)] for c in starts], axis=1), prev)
            acc = part if acc is None else acc + part
    return acc


def _swiglu_pair(x_terms, w1_terms, w3_terms, w2_terms, side_work):
    def project(terms, lo):
        c = _FROM_MODEL.combine(2, lambda i: _dot(x_terms[i], _unpack(terms[lo // _BLOCK, i])))
        return [jnp.concatenate(row, axis=1) for row in c]

    def hidden(lo):
        gates = [_silu(g) for g in project(w1_terms, lo)]
        hid = [g * u for g, u in zip(gates, project(w3_terms, lo))]
        return [t.astype(_BF16) for t in _SQUARE.left(hid)]

    chunks = list(range(0, w2_terms.shape[0] * _BLOCK, _PAIR_CHUNK))
    acc = hid = None
    for n in range(len(chunks) + 1):
        prev = hid
        if n < len(chunks):
            tiles = [hidden(lo) for lo in range(chunks[n], chunks[n] + _PAIR_CHUNK, _BLOCK)]
            hid = [jnp.concatenate(t, axis=1) for t in zip(*tiles)]
        if n >= 1:
            first = chunks[n - 1] // _BLOCK

            def product(i, first=first, prev=prev, acc=acc):
                left = [_unpack(w2_terms[first + c, i]) for c in range(_PAIR_CHUNK // _BLOCK)]
                part = _dot_nt(jnp.concatenate(left, axis=1), prev[i])
                return part if acc is None else acc[i] + part

            if n < len(chunks):
                acc = [product(i) for i in range(_SQUARE.products)]
            else:
                acc = _SQUARE.combine(2, product)
        side_work(n)
    return [jnp.concatenate(row, axis=0) for row in acc]


def _store_terms(w, terms, scheme, transposed):
    block_rows, block_cols = 2 * terms.shape[2], terms.shape[0] * _BLOCK

    def tile(j, carry):
        def block(r, c, lo):
            start = r * block_rows + j * 16
            rows = pl.ds(pl.multiple_of(jnp.minimum(start, w.shape[0] - 16), 16), 16)
            words = pltpu.bitcast(
                w[rows, c * block_cols + lo:c * block_cols + lo + _BLOCK], jnp.uint32)
            if (r + 1) * block_rows > w.shape[0]:
                words = jnp.where(start < w.shape[0], words, jnp.uint32(0))
            return words

        for lo in range(0, block_cols, _BLOCK):
            words = [block(n, k, lo) if transposed else block(k, n, lo)
                     for k in range(scheme.inner) for n in range(scheme.outer)]
            even, odd = (scheme.right(rows) for rows in zip(*map(_split_words, words)))
            for i, pair in enumerate(zip(even, odd)):
                terms[lo // _BLOCK, i, pl.ds(pl.multiple_of(j * 8, 8), 8)] = (
                    pltpu.pack_elementwise(pair, packed_dtype=_BF16))
        return carry

    lax.fori_loop(0, block_rows // 16, tile, 0)


def _load_weights(sources, qkv, wo_hbm, wo, stage, wo_stage, wsem, osem,
                  later_copies):
    d_model, n_heads, dh = sources[0].shape
    n_groups = n_heads // _GROUP
    per_weight = _BLOCK // _WCHUNK
    n_jobs = len(sources) * per_weight
    full = _FROM_MODEL.inner - 1
    ragged = (d_model - full * _BLOCK) // _WCHUNK
    stage[ragged:, full] = jnp.zeros((per_weight - ragged,) + stage.shape[2:], stage.dtype)

    def for_copies(src, job, action):
        c = job % per_weight

        def copy(n):
            action(pltpu.make_async_copy(src.at[pl.ds(n * _BLOCK + c * _WCHUNK, _WCHUNK)],
                                         stage.at[c, n], wsem.at[(full + 1) * c + n]))

        for n in range(full):
            copy(n)
        pl.when(c < ragged)(functools.partial(copy, full))

    def start(job):
        for i, src in enumerate(sources):
            pl.when(job // per_weight == i)(
                functools.partial(for_copies, src, job, lambda c: c.start()))

    def wait(job):
        for i, src in enumerate(sources):
            pl.when(job // per_weight == i)(
                functools.partial(for_copies, src, job, lambda c: c.wait()))

    def split_heads(slot, n, j):
        rows = pl.ds(pl.multiple_of(j * 16, 16), 16)
        words = jnp.swapaxes(pltpu.bitcast(stage[slot, n, rows], jnp.uint32), 0, 1)
        return [half for p in range(n_heads // 2) for half in _split_words(words[p])]

    def output_group(g, carry):
        def transposed(head):
            last = jnp.concatenate(
                [wo_stage[head, full * _BLOCK:],
                 jnp.zeros(((full + 1) * _BLOCK - d_model, dh), wo_stage.dtype)], axis=0)
            return jnp.concatenate([wo_stage[head, :full * _BLOCK].T, last.T], axis=1)

        heads = [transposed(_GROUP * g + i) for i in range(_GROUP)]
        for r in range(0, dh, 16):
            blocks = [blk for h in heads
                      for blk in _column_blocks(h[r:r + 16].astype(_F32), _TO_MODEL.outer)]
            for i, t in enumerate(_TO_MODEL.right(blocks)):
                wo[g, i, r // 2:r // 2 + 8] = _pack(t)
        return carry

    wo_copy = pltpu.make_async_copy(wo_hbm, wo_stage, osem)
    lax.fori_loop(0, _INFLIGHT, lambda job, carry: start(job), None)
    wo_copy.start()

    def groups_done(job):
        return jnp.minimum(2 * jnp.maximum(job - _WO_FROM, 0), n_groups)

    def run(job, carry):
        which, c = job // per_weight, job % per_weight
        wait(job)
        start(job + _INFLIGHT)

        @pl.when(job == n_jobs - _LATER_FROM)
        def _():
            for copy in later_copies:
                copy.start()


        def main_rows(j, carry):
            rows = pl.ds(pl.multiple_of(c * (_WCHUNK // 2) + j * 8, 8), 8)
            parts = [split_heads(c, n, j) for n in range(full + 1)]
            for g in range(n_groups):
                blocks = [h for part in parts for h in part[_GROUP * g:_GROUP * (g + 1)]]
                for n, t in enumerate(_FROM_MODEL.right(blocks)):
                    qkv[which, g, n, rows] = _pack(t)
            return carry

        lax.fori_loop(0, _WCHUNK // 16, main_rows, 0)
        pl.when(job == _WO_FROM)(wo_copy.wait)
        lax.fori_loop(groups_done(job), groups_done(job + 1), output_group, 0)
        return carry

    lax.fori_loop(0, n_jobs, run, 0)


def _kernel(x0_ref, x_next_ref, mem0_ref, wq_hbm, wk_hbm, wv_hbm, wo_hbm, w1_hbm, w3_hbm,
            w2_hbm, out_ref,
            stage, wo_stage, qkv, wo,
            w1, w3, w2_t, w1_terms, w3_terms, w2_terms, res, normed, mem, acc_t, x_terms, h_terms, o_sums, wsem, osem, fsem, *, seg):
    b = pl.program_id(0)
    n_blocks = pl.num_programs(0) - 1
    _, n_heads, dh = wq_hbm.shape
    n_mem = mem0_ref.shape[0]
    steps = _TOK // seg
    ffn_copies = [pltpu.make_async_copy(s, d, fsem.at[i])
                  for i, (s, d) in enumerate(((w1_hbm, w1), (w3_hbm, w3), (w2_hbm, w2_t)))]

    def start_layer(slot, x):
        res[slot] = x
        normed[slot] = _layernorm(x)

    def prepare_swiglu(j):
        rows = pl.ds(pl.multiple_of(j * seg, seg), seg)
        for i, t in enumerate(_FROM_MODEL.left([_layernorm(res[n, rows]) for n in range(2)])):
            x_terms[i, rows] = t.astype(_BF16)

    @pl.when(b == 0)
    def _():
        _load_weights((wq_hbm, wk_hbm, wv_hbm), qkv, wo_hbm, wo,
                      stage, wo_stage, wsem, osem, ffn_copies)
        mem[0] = mem0_ref[...].astype(_F32)
        mem[1] = mem0_ref[...].astype(_F32)
        start_layer(0, x0_ref[...].astype(_F32).T)

    def run_attention(first, n_seq):
        keep, fill = _masks(n_mem, n_mem + seg, n_seq)

        def segment(j, carry):
            rows = pl.ds(pl.multiple_of(j * seg, seg), seg)
            if n_seq == 2:
                prepare_swiglu(jnp.maximum(j - 1, 0))
            hs = [jnp.concatenate([mem[first + i], normed[first + i, rows]], axis=0)
                  for i in range(n_seq)]
            for i, out in enumerate(_attention(hs, keep, fill, qkv, wo, h_terms, o_sums,
               n_heads, dh)):
                mem[first + i] = out[:n_mem]
                res[first + i, rows] += out[n_mem:]
            return carry

        lax.fori_loop(0, steps, segment, 0)

    both = jnp.logical_and(b > 0, b < n_blocks)

    @pl.when(both)
    def _():
        run_attention(0, 2)
        prepare_swiglu(steps - 1)

        def side_work(n):
            if n == 0:
                acc_t[...] = res[1].T
                res[1] = res[0]
            if n == 1:
                start_layer(0, x_next_ref[...].astype(_F32).T)

        f2, f4 = _swiglu_pair(x_terms, w1_terms, w3_terms, w2_terms, side_work)
        start_layer(1, res[1] + f2.T)
        out_ref[...] = (acc_t[...] + f4).astype(out_ref.dtype)

    @pl.when(jnp.logical_not(both))
    def _():
        slot = jnp.where(b == 0, 0, 1)
        run_attention(slot, 1)

        @pl.when(b == 0)
        def _():
            for c, w, terms in zip(ffn_copies, (w1, w3, w2_t), (w1_terms, w3_terms, w2_terms)):
                c.wait()
                _store_terms(w, terms, _SQUARE if w is w2_t else _FROM_MODEL, w is w2_t)

        x = res[slot]
        xn = _layernorm(x)
        terms = [t.astype(_BF16) for t in _FROM_MODEL.left([xn[:_TOK // 2], xn[_TOK // 2:]])]
        acc_t[...] = x.T

        def part(i, carry):
            tiles = [i * _EDGE_TILES + t for t in range(_EDGE_TILES)]
            acc_t[...] += _swiglu_one(terms, w1_terms, w3_terms, w2_t, tiles)
            return carry

        lax.fori_loop(0, w1_terms.shape[0] // _EDGE_TILES, part, 0)

        @pl.when(b == 0)
        def _():
            start_layer(1, acc_t[...].T)
            start_layer(0, x_next_ref[...].astype(_F32).T)

        @pl.when(b > 0)
        def _():
            out_ref[...] = acc_t[...].astype(out_ref.dtype)


@functools.partial(jax.jit, static_argnames=("A_seg_len",))
def pallas_interleave_layers__memory_aug_recurrent_mem_tr__glu_gated_swiglu__prompt_kernel(
    A_x: jax.Array,
    A_mem0: jax.Array,
    A_Wq: jax.Array,
    A_Wk: jax.Array,
    A_Wv: jax.Array,
    A_Wo: jax.Array,
    A_seg_len: int,
    B_x: jax.Array,
    B_w1: jax.Array,
    B_w3: jax.Array,
    B_w2: jax.Array,
):
    del B_x
    batch, seq, d_model = A_x.shape
    n_mem = A_mem0.shape[1]
    _, n_heads, dh = A_Wq.shape
    d_ff = B_w1.shape[1]
    seg = int(A_seg_len)
    assert batch == 1 and seq % _TOK == 0 and _TOK % seg == 0 and seg % 16 == 0
    assert n_mem == 8 and n_heads % _GROUP == 0 and d_ff % (4 * _BLOCK * _EDGE_TILES) == 0
    slots = _BLOCK // _WCHUNK
    assert _INFLIGHT < slots and d_model % 64 == 0
    assert (_FROM_MODEL.inner - 1) * _BLOCK < d_model < _FROM_MODEL.inner * _BLOCK
    assert dh == _BLOCK and d_ff % (4 * _PAIR_CHUNK) == 0
    ff_tiles = d_ff // (4 * _BLOCK)
    n_blocks = seq // _TOK

    x_t = A_x[0].T
    hbm = pl.BlockSpec(memory_space=pl.ANY)
    out_t = pl.pallas_call(
        functools.partial(_kernel, seg=seg),
        grid=(n_blocks + 1,),
        in_specs=[
            pl.BlockSpec((d_model, _TOK), lambda b: (0, 0)),
            pl.BlockSpec((d_model, _TOK), lambda b: (0, jnp.minimum(b + 1, n_blocks - 1))),
            pl.BlockSpec((n_mem, d_model), lambda b: (0, 0)),
            hbm, hbm, hbm, hbm, hbm, hbm, hbm,
        ],
        out_specs=pl.BlockSpec((d_model, _TOK), lambda b: (0, jnp.maximum(b - 1, 0))),
        out_shape=jax.ShapeDtypeStruct((d_model, seq), A_x.dtype),
        scratch_shapes=[
            pltpu.VMEM((slots, _FROM_MODEL.inner, _WCHUNK, n_heads, dh), _BF16),
            pltpu.VMEM((n_heads, d_model, dh), _BF16),
            pltpu.VMEM((3, n_heads // _GROUP, _FROM_MODEL.products, _BLOCK // 2, dh), jnp.uint32),
            pltpu.VMEM((n_heads // _GROUP, _TO_MODEL.products, dh // 2, _BLOCK), jnp.uint32),
            pltpu.VMEM((d_model, d_ff), _BF16),
            pltpu.VMEM((d_model, d_ff), _BF16),
            pltpu.VMEM((d_model, d_ff), _BF16),
            *2 * [pltpu.VMEM((ff_tiles, _FROM_MODEL.products, _BLOCK // 2, _BLOCK), jnp.uint32)],
            pltpu.VMEM((ff_tiles, _SQUARE.products, d_model // 8, _BLOCK), jnp.uint32),
            pltpu.VMEM((2, _TOK, d_model), _F32),
            pltpu.VMEM((2, _TOK, d_model), _F32),
            pltpu.VMEM((2, n_mem, d_model), _F32),
            pltpu.VMEM((d_model, _TOK), _F32),
            pltpu.VMEM((_FROM_MODEL.products, _TOK, _BLOCK), _BF16),
            pltpu.VMEM((_FROM_MODEL.products, n_mem + seg, _BLOCK), _F32),
            pltpu.VMEM((_TO_MODEL.products, n_mem + seg, _BLOCK), _F32),
            pltpu.SemaphoreType.DMA((slots * _FROM_MODEL.inner,)),
            pltpu.SemaphoreType.DMA(()),
            pltpu.SemaphoreType.DMA((3,)),
        ],
        compiler_params=pltpu.CompilerParams(
            dimension_semantics=("arbitrary",),
            vmem_limit_bytes=112 * 1024 * 1024,
        ),
    )(x_t, x_t, A_mem0[0], A_Wq, A_Wk, A_Wv, jnp.transpose(A_Wo, (0, 2, 1)),
      B_w1, B_w3, B_w2.T)
    return out_t.T[None]
```

```python
import functools

import jax
import jax.numpy as jnp
import numpy as np
from jax import lax
import jax.experimental.pallas as pl
import jax.experimental.pallas.tpu as pltpu

_BF16 = jnp.bfloat16
_F32 = jnp.float32
_NT = (((1,), (1,)), ((), ()))
_TOK = 128
_GROUP = 4
_WCHUNK = 32
_INFLIGHT = 3
_EDGE_TILES = 3
_BLOCK = 128
_WO_FROM = 5
_PAIR_CHUNK = 384
_LATER_FROM = 1
_STAGE_ORDER = (((0, 1), 0), ((2,), 0), ("mix", 1), ("scores", 0), ("output", 2))
_LOG2E = float(np.log2(np.e))
_MASKED = -1000000000.0


def _layernorm(x):
    m = jnp.mean(x, axis=-1, keepdims=True)
    c = x - m
    v = jnp.mean(c * c, axis=-1, keepdims=True)
    return c * lax.rsqrt(v + 1e-05)


def _dot(a, b):
    return lax.dot_general(a, b, (((1,), (0,)), ((), ())), preferred_element_type=_F32)


def _dot_nt(a, b):
    return lax.dot_general(a, b, _NT, preferred_element_type=_F32)


def _pack(x):
    return pltpu.bitcast(x.astype(_BF16), jnp.uint32)


def _split_words(words):
    return (pltpu.bitcast(words << 16, _F32),
            pltpu.bitcast(words & jnp.uint32(0xFFFF0000), _F32))


def _unpack(words):
    return pltpu.bitcast(words, _BF16)


_SCHEME_244 = (
    "...+.... +.......++..--.. .-......",
    "..+++..+ +.........-..... ..-.+...",
    ".+++.... ....+++......... +..-....",
    ".+.+.+.. ...+.......+...- ...-.-.+",
    "++-..... ......+......... -.+++.--",
    "+...+..+ .+-.......-...+. ..-..++.",
    "+.-..... +.....+......... +.-.....",
    "..++..+. +....-..++..-... -+..+...",
    "+....... .+.............. .++..--.",
    ".+...+.. ....++++...+...- ...+....",
    "++-..+.. ...+..-......... ...++.--",
    "..++.-.. ...++++....+.... ...+-...",
    "+..++..+ +.........-...+. ..+.....",
    ".+.+..-. .....+.......... -+...-.+",
    "..++.... +...---.++...... +...-...",
    "..+...+. +....-..+...-... +-......",
    "......+. .....+...-...... -+..+-..",
    ".....+.. ...+..+-...+.... ...+...-",
    "++-.++-. ...+............ ....-.++",
    "....+..+ .+-.......-..... ..+...-.",
    ".+.+.+.+ ...+.+.....+...- .....+.-",
    "....+.-. ...+......+..... ....+.-.",
    ".....+++ ...+.+.....+.... ....-..+",
    "+...+... ..+.......+...-. .....++.",
    ".......+ .+-+.+....-+.-+- .....-..",
    "..++..++ +..-.-....---... ....-...",
)
_SCHEME_254 = (
    "..+-.-..+. -.........+.....+... ..+.+...",
    "....+..... .-...............+.. .+...+..",
    ".++-...... ...-+-+....-...-.... +..+....",
    "....+..... ...................+ ...+....",
    "..+-...... .+-+-+-...-+-+-+-... +...+...",
    ".++....... ...-.......-...-.... .+.-.+.-",
    "+..-+..... .+-.......-...-.-... .++.....",
    "+...+..... ..-.......-...-..... +.-.+.-.",
    ".+....-... ...+-+-+............ ...+....",
    "+.-....... +.....-.........-... +.-.....",
    "....++..-. .-..............+.+. ..+..-..",
    "+--...+... ...+..-............. ...++.-+",
    ".++.....-. ...+.+.....+...+.... ++...+.-",
    "..+-....+. +-+-.-..+.+-+-+-.... ++..+...",
    "+...+...-. ..+.......+...+.+... ++..+.-.",
    "+..-.-..+. +-+................. ..+.....",
    "..+-..+... ...+-+-....+........ ...+-...",
    "..+....... -+-+....-+-+-+-+.... .+......",
    "...+....-. +..-.-..+..-+..--... ++......",
    "+--....... ......+............. +.-++.-+",
    ".....+..-. ..+.......+.......-. ..+...+.",
    "+...+-...- ................-... ....+.-.",
    "..+-...-+. ...+.+..-.-+........ ....+...",
    "........+. .+.+.+.....+.+.+.... ++..++..",
    ".....+..-+ ................+.+. .....++.",
    "......+... ...-..++...-........ ...+...+",
    ".....+.-.. ...-......+......... ....+.-.",
    "......++-. ...+.+.....+........ ....+..+",
    ".++...--.. .....-.............. .....+.-",
    ".......+.. .....-...+.......... .....+..",
    ".........+ ...................+ .......+",
    "+--..-++.. ...-................ ....+.-+",
    "....+....- ................+-+. .....+..",
)


def _sum_program(rows):
    n_in = len(rows[0])
    rows = [{i: c for i, c in enumerate(row) if c} for row in rows]
    steps, ready = [], list(range(n_in))

    def emit(a, b, sign):
        steps.append((a, b, sign))
        ready.append(max(ready[a], ready[b]))
        return len(ready) - 1

    while True:
        count = {}
        for row in rows:
            items = sorted(row.items())
            for n, (a, x) in enumerate(items):
                for b, y in items[n + 1:]:
                    count[a, b, x * y] = count.get((a, b, x * y), 0) + 1
        best = max(sorted(count), key=count.get, default=None)
        if best is None or count[best] < 2:
            break
        a, b, sign = best
        new = emit(a, b, sign)
        for row in rows:
            if a in row and b in row and row[a] * row[b] == sign:
                row[new] = row.pop(a)
                del row[b]
    outs = []
    for row in rows:
        items = sorted(row.items(), key=lambda item: (ready[item[0]], item[0]))
        at, sign = items[0]
        for b, y in items[1:]:
            if sign < 0 < y:
                at, sign = emit(b, at, -1), 1
            else:
                at = emit(at, b, sign * y)
        outs.append((at, sign))
    return n_in, steps, ready, outs


def _evaluate(program, make):
    n_in, steps, ready, outs = program
    vals = {}
    for i in range(n_in):
        vals[i] = make(i)
        for n, (a, b, sign) in enumerate(steps):
            if ready[n_in + n] == i:
                vals[n_in + n] = vals[a] + vals[b] if sign > 0 else vals[a] - vals[b]
    return [vals[i] if sign > 0 else -vals[i] for i, sign in outs]


class _Scheme:
    def __init__(self, u, v, w):
        self.products = len(u)
        self.inner, self.outer = k, n = u.shape[1] // 2, w.shape[1] // 2
        want = np.zeros((2 * k, k * n, 2 * n), np.int64)
        for i, a, j in np.ndindex(2, k, n):
            want[k * i + a, n * a + j, n * i + j] = 1
        first = (u[:k * n, :k], v[:k * n], w[:k * n, :n])
        assert np.array_equal(np.einsum("ra,rb,rc->abc", u, v, w), want)
        assert np.array_equal(np.einsum("ra,rb,rc->abc", *first), want[:k, :, :n])
        self._left = {1: _sum_program(first[0].tolist()), 2: _sum_program(u.tolist())}
        self._right = _sum_program(v.tolist())
        self._out = {1: _sum_program(first[2].T.tolist()), 2: _sum_program(w.T.tolist())}

    def left(self, rows):
        blocks = [blk for row in rows for blk in _column_blocks(row, self.inner)]
        return _evaluate(self._left[len(rows)], blocks.__getitem__)

    def right(self, blocks):
        return _evaluate(self._right, blocks.__getitem__)

    def combine(self, n_rows, product):
        c = _evaluate(self._out[n_rows], product)
        return [c[self.outer * i:self.outer * (i + 1)] for i in range(n_rows)]


def _parse(table):
    return [np.array([[{"+": 1, ".": 0, "-": -1}[c] for c in line.split()[f]]
                      for line in table]) for f in range(3)]


def _swap_inner_outer(u, v, w):
    k, n = u.shape[1] // 2, w.shape[1] // 2
    return w, v.reshape(-1, k, n).transpose(0, 2, 1).reshape(-1, k * n), u


_SQUARE = _Scheme(*_parse(_SCHEME_244))
_FROM_MODEL = _Scheme(*_parse(_SCHEME_254))
_TO_MODEL = _Scheme(*_swap_inner_outer(*_parse(_SCHEME_254)))


def _column_blocks(x, count):
    pad = count * _BLOCK - x.shape[1]
    if pad:
        x = jnp.concatenate([x, jnp.zeros((x.shape[0], pad), x.dtype)], axis=1)
    return [x[:, i * _BLOCK:(i + 1) * _BLOCK] for i in range(count)]


def _masks(n_mem, length, n_seq):
    rows = n_seq * length

    def describe(axis):
        i = lax.broadcasted_iota(jnp.int32, (rows, rows), axis)
        second = i >= length
        return jnp.where(second, 1, 0), jnp.where(second, i - length, i)

    (seq_r, idx_r), (seq_c, idx_c) = describe(0), describe(1)
    same = seq_r == seq_c
    keep = same & ((idx_r < n_mem) | (idx_r >= idx_c))
    fill = jnp.where(same, _MASKED * _LOG2E, -jnp.inf).astype(_F32)
    return keep, fill


def _attention(hs, keep, fill, qkv, wo, h_terms, o_sums,
               n_heads, dh):
    scale = dh ** -0.5
    n_groups = n_heads // _GROUP
    n_seq, length = len(hs), hs[0].shape[0]
    heads = [slice(i * dh, (i + 1) * dh) for i in range(_GROUP)]
    lhs_dtype = _BF16 if (n_seq * length) % 16 == 0 else _F32

    for i, t in enumerate(_FROM_MODEL.left(hs)):
        h_terms[i] = t

    def project(ws, g):
        c = _FROM_MODEL.combine(n_seq, lambda i: _dot(h_terms[i], jnp.concatenate(
            [_unpack(qkv[w, g, i]) for w in ws], axis=1)))
        return [jnp.concatenate(
            [jnp.concatenate([blk[:, n * dh:(n + 1) * dh] for blk in row], axis=1) for row in c],
            axis=0) for n in range(len(ws))]

    def weights(q, k):
        out = []
        for cols in heads:
            s = jnp.where(keep, _dot_nt(q[:, cols], k[:, cols]) * (scale * _LOG2E), fill)
            e = jnp.exp2(s - jnp.max(s, axis=-1, keepdims=True))
            out.append((e.astype(lhs_dtype), 1.0 / jnp.sum(e, axis=-1, keepdims=True)))
        return out

    def mix(p, v):
        return jnp.concatenate(
            [_dot(e, v[:, cols]) * inv for (e, inv), cols in zip(p, heads)], axis=1)

    def output(o, g):
        terms = _TO_MODEL.left([o[i * length:(i + 1) * length] for i in range(n_seq)])

        def product(i):
            part = _dot(terms[i], _unpack(wo[g, i]))
            return part if g == 0 else o_sums[i] + part

        if g == n_groups - 1:
            return _TO_MODEL.combine(n_seq, product)
        for i in range(len(terms)):
            o_sums[i] = product(i)

    proj, p, o, acc = {}, {}, {}, None
    for stage in range(n_groups + max(lag for _, lag in _STAGE_ORDER)):
        for task, lag in _STAGE_ORDER:
            g = stage - lag
            if not 0 <= g < n_groups:
                continue
            if task == "scores":
                p[g] = weights(proj.pop((0, g)), proj.pop((1, g)))
            elif task == "mix":
                o[g] = mix(p.pop(g), proj.pop((2, g)))
            elif task == "output":
                acc = output(o.pop(g), g)
            else:
                for w, x in zip(task, project(task, g)):
                    proj[w, g] = x.astype(lhs_dtype if w == 0 else _BF16)
    return [jnp.concatenate(row, axis=1)[:, :hs[0].shape[1]] for row in acc]


def _silu(x):
    half = 0.5 * x
    return half + half * jnp.tanh(half)


def _swiglu_one(x_terms, w1_terms, w3_terms, w2_t, tiles):
    quarter = w2_t.shape[1] // _FROM_MODEL.outer

    def project(terms, tile):
        c = _FROM_MODEL.combine(2, lambda i: _dot(x_terms[i], _unpack(terms[tile, i])))
        return jnp.concatenate([jnp.concatenate(row, axis=1) for row in c], axis=0)

    acc = hid = None
    for n in range(len(tiles) + 1):
        prev = hid
        if n < len(tiles):
            gate = _silu(project(w1_terms, tiles[n]))
            hid = (gate * project(w3_terms, tiles[n])).astype(_BF16)
        if n >= 1:
            starts = [pl.multiple_of(j * quarter + tiles[n - 1] * _BLOCK, _BLOCK)
                      for j in range(_FROM_MODEL.outer)]
            part = _dot_nt(
                jnp.concatenate([w2_t[:, pl.ds(c, _BLOCK)] for c in starts], axis=1), prev)
            acc = part if acc is None else acc + part
    return acc


def _swiglu_pair(x_terms, w1_terms, w3_terms, w2_terms, side_work):
    def project(terms, lo):
        c = _FROM_MODEL.combine(2, lambda i: _dot(x_terms[i], _unpack(terms[lo // _BLOCK, i])))
        return [jnp.concatenate(row, axis=1) for row in c]

    def hidden(lo):
        gates = [_silu(g) for g in project(w1_terms, lo)]
        hid = [g * u for g, u in zip(gates, project(w3_terms, lo))]
        return [t.astype(_BF16) for t in _SQUARE.left(hid)]

    chunks = list(range(0, w2_terms.shape[0] * _BLOCK, _PAIR_CHUNK))
    acc = hid = None
    for n in range(len(chunks) + 1):
        prev = hid
        if n < len(chunks):
            tiles = [hidden(lo) for lo in range(chunks[n], chunks[n] + _PAIR_CHUNK, _BLOCK)]
            hid = [jnp.concatenate(t, axis=1) for t in zip(*tiles)]
        if n >= 1:
            first = chunks[n - 1] // _BLOCK

            def product(i, first=first, prev=prev, acc=acc):
                left = [_unpack(w2_terms[first + c, i]) for c in range(_PAIR_CHUNK // _BLOCK)]
                part = _dot_nt(jnp.concatenate(left, axis=1), prev[i])
                return part if acc is None else acc[i] + part

            if n < len(chunks):
                acc = [product(i) for i in range(_SQUARE.products)]
            else:
                acc = _SQUARE.combine(2, product)
        side_work(n)
    return [jnp.concatenate(row, axis=0) for row in acc]


def _store_terms(w, terms, scheme, transposed):
    block_rows, block_cols = 2 * terms.shape[2], terms.shape[0] * _BLOCK

    def tile(j, carry):
        def block(r, c, lo):
            start = r * block_rows + j * 16
            rows = pl.ds(pl.multiple_of(jnp.minimum(start, w.shape[0] - 16), 16), 16)
            words = pltpu.bitcast(
                w[rows, c * block_cols + lo:c * block_cols + lo + _BLOCK], jnp.uint32)
            if (r + 1) * block_rows > w.shape[0]:
                words = jnp.where(start < w.shape[0], words, jnp.uint32(0))
            return words

        for lo in range(0, block_cols, _BLOCK):
            words = [block(n, k, lo) if transposed else block(k, n, lo)
                     for k in range(scheme.inner) for n in range(scheme.outer)]
            even, odd = (scheme.right(rows) for rows in zip(*map(_split_words, words)))
            for i, pair in enumerate(zip(even, odd)):
                terms[lo // _BLOCK, i, pl.ds(pl.multiple_of(j * 8, 8), 8)] = (
                    pltpu.pack_elementwise(pair, packed_dtype=_BF16))
        return carry

    lax.fori_loop(0, block_rows // 16, tile, 0)


def _load_weights(sources, qkv, wo_hbm, wo, stage, wo_stage, wsem, osem,
                  later_copies):
    d_model, n_heads, dh = sources[0].shape
    n_groups = n_heads // _GROUP
    per_weight = _BLOCK // _WCHUNK
    n_jobs = len(sources) * per_weight
    full = _FROM_MODEL.inner - 1
    ragged = (d_model - full * _BLOCK) // _WCHUNK
    stage[ragged:, full] = jnp.zeros((per_weight - ragged,) + stage.shape[2:], stage.dtype)

    def for_copies(src, job, action):
        c = job % per_weight

        def copy(n):
            action(pltpu.make_async_copy(src.at[pl.ds(n * _BLOCK + c * _WCHUNK, _WCHUNK)],
                                         stage.at[c, n], wsem.at[(full + 1) * c + n]))

        for n in range(full):
            copy(n)
        pl.when(c < ragged)(functools.partial(copy, full))

    def start(job):
        for i, src in enumerate(sources):
            pl.when(job // per_weight == i)(
                functools.partial(for_copies, src, job, lambda c: c.start()))

    def wait(job):
        for i, src in enumerate(sources):
            pl.when(job // per_weight == i)(
                functools.partial(for_copies, src, job, lambda c: c.wait()))

    def split_heads(slot, n, j):
        rows = pl.ds(pl.multiple_of(j * 16, 16), 16)
        words = jnp.swapaxes(pltpu.bitcast(stage[slot, n, rows], jnp.uint32), 0, 1)
        return [half for p in range(n_heads // 2) for half in _split_words(words[p])]

    def output_group(g, carry):
        def transposed(head):
            last = jnp.concatenate(
                [wo_stage[head, full * _BLOCK:],
                 jnp.zeros(((full + 1) * _BLOCK - d_model, dh), wo_stage.dtype)], axis=0)
            return jnp.concatenate([wo_stage[head, :full * _BLOCK].T, last.T], axis=1)

        heads = [transposed(_GROUP * g + i) for i in range(_GROUP)]
        for r in range(0, dh, 16):
            blocks = [blk for h in heads
                      for blk in _column_blocks(h[r:r + 16].astype(_F32), _TO_MODEL.outer)]
            for i, t in enumerate(_TO_MODEL.right(blocks)):
                wo[g, i, r // 2:r // 2 + 8] = _pack(t)
        return carry

    wo_copy = pltpu.make_async_copy(wo_hbm, wo_stage, osem)
    lax.fori_loop(0, _INFLIGHT, lambda job, carry: start(job), None)
    wo_copy.start()

    def groups_done(job):
        return jnp.minimum(2 * jnp.maximum(job - _WO_FROM, 0), n_groups)

    def run(job, carry):
        which, c = job // per_weight, job % per_weight
        wait(job)
        start(job + _INFLIGHT)

        @pl.when(job == n_jobs - _LATER_FROM)
        def _():
            for copy in later_copies:
                copy.start()


        def main_rows(j, carry):
            rows = pl.ds(pl.multiple_of(c * (_WCHUNK // 2) + j * 8, 8), 8)
            parts = [split_heads(c, n, j) for n in range(full + 1)]
            for g in range(n_groups):
                blocks = [h for part in parts for h in part[_GROUP * g:_GROUP * (g + 1)]]
                for n, t in enumerate(_FROM_MODEL.right(blocks)):
                    qkv[which, g, n, rows] = _pack(t)
            return carry

        lax.fori_loop(0, _WCHUNK // 16, main_rows, 0)
        pl.when(job == _WO_FROM)(wo_copy.wait)
        lax.fori_loop(groups_done(job), groups_done(job + 1), output_group, 0)
        return carry

    lax.fori_loop(0, n_jobs, run, 0)


def _kernel(x_hbm, mem0_ref, wq_hbm, wk_hbm, wv_hbm, wo_hbm, w1_hbm, w3_hbm,
            w2_hbm, out_hbm,
            x_all, out_all,
            stage, wo_stage, qkv, wo,
            w1, w3, w2_t, w1_terms, w3_terms, w2_terms, res, normed, mem, acc_t, x_terms, h_terms, o_sums, wsem, osem, fsem,
            xsem, *, seg):
    n_blocks = x_hbm.shape[1] // _TOK
    _, n_heads, dh = wq_hbm.shape
    n_mem = mem0_ref.shape[0]
    steps = _TOK // seg
    ffn_copies = [pltpu.make_async_copy(s, d, fsem.at[i])
                  for i, (s, d) in enumerate(((w1_hbm, w1), (w3_hbm, w3), (w2_hbm, w2_t)))]

    x_copies = [pltpu.make_async_copy(x_hbm.at[:, cols], x_all.at[:, cols], xsem.at[i])
                for i, cols in enumerate((pl.ds(0, _TOK), pl.ds(_TOK, (n_blocks - 1) * _TOK)))]

    def tokens(block):
        return pl.ds(pl.multiple_of(block * _TOK, _TOK), _TOK)

    def out_copy(block):
        return pltpu.make_async_copy(out_all.at[:, tokens(block)], out_hbm.at[:, tokens(block)],
                                     xsem.at[2])

    def start_layer(slot, x):
        res[slot] = x
        normed[slot] = _layernorm(x)

    def prepare_swiglu(j):
        rows = pl.ds(pl.multiple_of(j * seg, seg), seg)
        for i, t in enumerate(_FROM_MODEL.left([_layernorm(res[n, rows]) for n in range(2)])):
            x_terms[i, rows] = t.astype(_BF16)

    x_copies[0].start()
    _load_weights((wq_hbm, wk_hbm, wv_hbm), qkv, wo_hbm, wo, stage, wo_stage, wsem, osem,
                  ffn_copies + x_copies[1:])
    mem[0] = mem0_ref[...].astype(_F32)
    mem[1] = mem0_ref[...].astype(_F32)
    x_copies[0].wait()
    start_layer(0, x_all[:, :_TOK].astype(_F32).T)

    def run_attention(first, n_seq):
        keep, fill = _masks(n_mem, n_mem + seg, n_seq)

        def segment(j, carry):
            rows = pl.ds(pl.multiple_of(j * seg, seg), seg)
            if n_seq == 2:
                prepare_swiglu(jnp.maximum(j - 1, 0))
            hs = [jnp.concatenate([mem[first + i], normed[first + i, rows]], axis=0)
                  for i in range(n_seq)]
            for i, out in enumerate(_attention(hs, keep, fill, qkv, wo, h_terms, o_sums,
               n_heads, dh)):
                mem[first + i] = out[:n_mem]
                res[first + i, rows] += out[n_mem:]
            return carry

        lax.fori_loop(0, steps, segment, 0)

    def block_step(b, carry):
        both = jnp.logical_and(b > 0, b < n_blocks)

        @pl.when(both)
        def _():
            run_attention(0, 2)
            prepare_swiglu(steps - 1)

            def side_work(n):
                if n == 0:
                    acc_t[...] = res[1].T
                    res[1] = res[0]
                if n == 1:
                    start_layer(0, x_all[:, tokens(jnp.minimum(b + 1, n_blocks - 1))].astype(_F32).T)

            f2, f4 = _swiglu_pair(x_terms, w1_terms, w3_terms, w2_terms, side_work)
            start_layer(1, res[1] + f2.T)
            out_all[:, tokens(b - 1)] = (acc_t[...] + f4).astype(out_all.dtype)

        @pl.when(jnp.logical_not(both))
        def _():
            slot = jnp.where(b == 0, 0, 1)
            run_attention(slot, 1)

            @pl.when(b == 0)
            def _():
                for c, w, terms in zip(ffn_copies, (w1, w3, w2_t), (w1_terms, w3_terms, w2_terms)):
                    c.wait()
                    _store_terms(w, terms, _SQUARE if w is w2_t else _FROM_MODEL, w is w2_t)

            x = res[slot]
            xn = _layernorm(x)
            terms = [t.astype(_BF16) for t in _FROM_MODEL.left([xn[:_TOK // 2], xn[_TOK // 2:]])]
            acc_t[...] = x.T

            def part(i, carry):
                tiles = [i * _EDGE_TILES + t for t in range(_EDGE_TILES)]
                acc_t[...] += _swiglu_one(terms, w1_terms, w3_terms, w2_t, tiles)
                return carry

            lax.fori_loop(0, w1_terms.shape[0] // _EDGE_TILES, part, 0)

            @pl.when(b == 0)
            def _():
                x_copies[1].wait()
                start_layer(1, acc_t[...].T)
                start_layer(0, x_all[:, tokens(jnp.minimum(b + 1, n_blocks - 1))].astype(_F32).T)

            @pl.when(b > 0)
            def _():
                out_all[:, tokens(b - 1)] = acc_t[...].astype(out_all.dtype)

        @pl.when(b > 1)
        def _():
            out_copy(b - 2).wait()

        @pl.when(b > 0)
        def _():
            out_copy(b - 1).start()

        return carry

    lax.fori_loop(0, n_blocks + 1, block_step, 0)
    out_copy(n_blocks - 1).wait()


@functools.partial(jax.jit, static_argnames=("A_seg_len",))
def pallas_interleave_layers__memory_aug_recurrent_mem_tr__glu_gated_swiglu__prompt_kernel(
    A_x: jax.Array,
    A_mem0: jax.Array,
    A_Wq: jax.Array,
    A_Wk: jax.Array,
    A_Wv: jax.Array,
    A_Wo: jax.Array,
    A_seg_len: int,
    B_x: jax.Array,
    B_w1: jax.Array,
    B_w3: jax.Array,
    B_w2: jax.Array,
):
    del B_x
    batch, seq, d_model = A_x.shape
    n_mem = A_mem0.shape[1]
    _, n_heads, dh = A_Wq.shape
    d_ff = B_w1.shape[1]
    seg = int(A_seg_len)
    assert batch == 1 and seq % _TOK == 0 and _TOK % seg == 0 and seg % 16 == 0
    assert n_mem == 8 and n_heads % _GROUP == 0 and d_ff % (4 * _BLOCK * _EDGE_TILES) == 0
    slots = _BLOCK // _WCHUNK
    assert _INFLIGHT < slots and d_model % 64 == 0
    assert (_FROM_MODEL.inner - 1) * _BLOCK < d_model < _FROM_MODEL.inner * _BLOCK
    assert dh == _BLOCK and d_ff % (4 * _PAIR_CHUNK) == 0
    ff_tiles = d_ff // (4 * _BLOCK)
    n_blocks = seq // _TOK

    hbm = pl.BlockSpec(memory_space=pl.ANY)
    out_t = pl.pallas_call(
        functools.partial(_kernel, seg=seg),
        in_specs=[hbm, pl.BlockSpec(memory_space=pltpu.VMEM)] + 7 * [hbm],
        out_specs=hbm,
        out_shape=jax.ShapeDtypeStruct((d_model, seq), A_x.dtype),
        scratch_shapes=[
            pltpu.VMEM((d_model, seq), A_x.dtype),
            pltpu.VMEM((d_model, seq), A_x.dtype),
            pltpu.VMEM((slots, _FROM_MODEL.inner, _WCHUNK, n_heads, dh), _BF16),
            pltpu.VMEM((n_heads, d_model, dh), _BF16),
            pltpu.VMEM((3, n_heads // _GROUP, _FROM_MODEL.products, _BLOCK // 2, dh), jnp.uint32),
            pltpu.VMEM((n_heads // _GROUP, _TO_MODEL.products, dh // 2, _BLOCK), jnp.uint32),
            pltpu.VMEM((d_model, d_ff), _BF16),
            pltpu.VMEM((d_model, d_ff), _BF16),
            pltpu.VMEM((d_model, d_ff), _BF16),
            *2 * [pltpu.VMEM((ff_tiles, _FROM_MODEL.products, _BLOCK // 2, _BLOCK), jnp.uint32)],
            pltpu.VMEM((ff_tiles, _SQUARE.products, d_model // 8, _BLOCK), jnp.uint32),
            pltpu.VMEM((2, _TOK, d_model), _F32),
            pltpu.VMEM((2, _TOK, d_model), _F32),
            pltpu.VMEM((2, n_mem, d_model), _F32),
            pltpu.VMEM((d_model, _TOK), _F32),
            pltpu.VMEM((_FROM_MODEL.products, _TOK, _BLOCK), _BF16),
            pltpu.VMEM((_FROM_MODEL.products, n_mem + seg, _BLOCK), _F32),
            pltpu.VMEM((_TO_MODEL.products, n_mem + seg, _BLOCK), _F32),
            pltpu.SemaphoreType.DMA((slots * _FROM_MODEL.inner,)),
            pltpu.SemaphoreType.DMA(()),
            pltpu.SemaphoreType.DMA((3,)),
            pltpu.SemaphoreType.DMA((3,)),
        ],
        compiler_params=pltpu.CompilerParams(
            vmem_limit_bytes=112 * 1024 * 1024,
        ),
    )(A_x[0].T, A_mem0[0], A_Wq, A_Wk, A_Wv, jnp.transpose(A_Wo, (0, 2, 1)),
      B_w1, B_w3, B_w2.T)
    return out_t.T[None]
```

```python
import functools

import jax
import jax.numpy as jnp
import numpy as np
from jax import lax
import jax.experimental.pallas as pl
import jax.experimental.pallas.tpu as pltpu

_BF16 = jnp.bfloat16
_F32 = jnp.float32
_NT = (((1,), (1,)), ((), ()))
_TOK = 128
_GROUP = 4
_WCHUNK = 32
_INFLIGHT = 3
_EDGE_TILES = 3
_BLOCK = 128
_WO_FROM = 5
_PAIR_CHUNK = 384
_LATER_FROM = 1
_STAGE_ORDER = (((0, 1), 0), ((2,), 0), ("mix", 1), ("scores", 0), ("output", 2))
_LOG2E = float(np.log2(np.e))
_MASKED = -1000000000.0


def _layernorm(x):
    m = jnp.mean(x, axis=-1, keepdims=True)
    c = x - m
    v = jnp.mean(c * c, axis=-1, keepdims=True)
    return c * lax.rsqrt(v + 1e-05)


def _dot(a, b):
    return lax.dot_general(a, b, (((1,), (0,)), ((), ())), preferred_element_type=_F32)


def _dot_nt(a, b):
    return lax.dot_general(a, b, _NT, preferred_element_type=_F32)


def _pack(x):
    return pltpu.bitcast(x.astype(_BF16), jnp.uint32)


def _split_words(words):
    return (pltpu.bitcast(words << 16, _F32),
            pltpu.bitcast(words & jnp.uint32(0xFFFF0000), _F32))


def _unpack(words):
    return pltpu.bitcast(words, _BF16)


_SCHEME_244 = (
    "...+.... +.......++..--.. .-......",
    "..+++..+ +.........-..... ..-.+...",
    ".+++.... ....+++......... +..-....",
    ".+.+.+.. ...+.......+...- ...-.-.+",
    "++-..... ......+......... -.+++.--",
    "+...+..+ .+-.......-...+. ..-..++.",
    "+.-..... +.....+......... +.-.....",
    "..++..+. +....-..++..-... -+..+...",
    "+....... .+.............. .++..--.",
    ".+...+.. ....++++...+...- ...+....",
    "++-..+.. ...+..-......... ...++.--",
    "..++.-.. ...++++....+.... ...+-...",
    "+..++..+ +.........-...+. ..+.....",
    ".+.+..-. .....+.......... -+...-.+",
    "..++.... +...---.++...... +...-...",
    "..+...+. +....-..+...-... +-......",
    "......+. .....+...-...... -+..+-..",
    ".....+.. ...+..+-...+.... ...+...-",
    "++-.++-. ...+............ ....-.++",
    "....+..+ .+-.......-..... ..+...-.",
    ".+.+.+.+ ...+.+.....+...- .....+.-",
    "....+.-. ...+......+..... ....+.-.",
    ".....+++ ...+.+.....+.... ....-..+",
    "+...+... ..+.......+...-. .....++.",
    ".......+ .+-+.+....-+.-+- .....-..",
    "..++..++ +..-.-....---... ....-...",
)
_SCHEME_254 = (
    "..+-.-..+. -.........+.....+... ..+.+...",
    "....+..... .-...............+.. .+...+..",
    ".++-...... ...-+-+....-...-.... +..+....",
    "....+..... ...................+ ...+....",
    "..+-...... .+-+-+-...-+-+-+-... +...+...",
    ".++....... ...-.......-...-.... .+.-.+.-",
    "+..-+..... .+-.......-...-.-... .++.....",
    "+...+..... ..-.......-...-..... +.-.+.-.",
    ".+....-... ...+-+-+............ ...+....",
    "+.-....... +.....-.........-... +.-.....",
    "....++..-. .-..............+.+. ..+..-..",
    "+--...+... ...+..-............. ...++.-+",
    ".++.....-. ...+.+.....+...+.... ++...+.-",
    "..+-....+. +-+-.-..+.+-+-+-.... ++..+...",
    "+...+...-. ..+.......+...+.+... ++..+.-.",
    "+..-.-..+. +-+................. ..+.....",
    "..+-..+... ...+-+-....+........ ...+-...",
    "..+....... -+-+....-+-+-+-+.... .+......",
    "...+....-. +..-.-..+..-+..--... ++......",
    "+--....... ......+............. +.-++.-+",
    ".....+..-. ..+.......+.......-. ..+...+.",
    "+...+-...- ................-... ....+.-.",
    "..+-...-+. ...+.+..-.-+........ ....+...",
    "........+. .+.+.+.....+.+.+.... ++..++..",
    ".....+..-+ ................+.+. .....++.",
    "......+... ...-..++...-........ ...+...+",
    ".....+.-.. ...-......+......... ....+.-.",
    "......++-. ...+.+.....+........ ....+..+",
    ".++...--.. .....-.............. .....+.-",
    ".......+.. .....-...+.......... .....+..",
    ".........+ ...................+ .......+",
    "+--..-++.. ...-................ ....+.-+",
    "....+....- ................+-+. .....+..",
)


def _sum_program(rows):
    n_in = len(rows[0])
    rows = [{i: c for i, c in enumerate(row) if c} for row in rows]
    steps, ready = [], list(range(n_in))

    def emit(a, b, sign):
        steps.append((a, b, sign))
        ready.append(max(ready[a], ready[b]))
        return len(ready) - 1

    while True:
        count = {}
        for row in rows:
            items = sorted(row.items())
            for n, (a, x) in enumerate(items):
                for b, y in items[n + 1:]:
                    count[a, b, x * y] = count.get((a, b, x * y), 0) + 1
        best = max(sorted(count), key=count.get, default=None)
        if best is None or count[best] < 2:
            break
        a, b, sign = best
        new = emit(a, b, sign)
        for row in rows:
            if a in row and b in row and row[a] * row[b] == sign:
                row[new] = row.pop(a)
                del row[b]
    outs = []
    for row in rows:
        items = sorted(row.items(), key=lambda item: (ready[item[0]], item[0]))
        at, sign = items[0]
        for b, y in items[1:]:
            if sign < 0 < y:
                at, sign = emit(b, at, -1), 1
            else:
                at = emit(at, b, sign * y)
        outs.append((at, sign))
    return n_in, steps, ready, outs


def _evaluate(program, make):
    n_in, steps, ready, outs = program
    vals = {}
    for i in range(n_in):
        vals[i] = make(i)
        for n, (a, b, sign) in enumerate(steps):
            if ready[n_in + n] == i:
                vals[n_in + n] = vals[a] + vals[b] if sign > 0 else vals[a] - vals[b]
    return [vals[i] if sign > 0 else -vals[i] for i, sign in outs]


class _Scheme:
    def __init__(self, u, v, w):
        self.products = len(u)
        self.inner, self.outer = k, n = u.shape[1] // 2, w.shape[1] // 2
        want = np.zeros((2 * k, k * n, 2 * n), np.int64)
        for i, a, j in np.ndindex(2, k, n):
            want[k * i + a, n * a + j, n * i + j] = 1
        first = (u[:k * n, :k], v[:k * n], w[:k * n, :n])
        assert np.array_equal(np.einsum("ra,rb,rc->abc", u, v, w), want)
        assert np.array_equal(np.einsum("ra,rb,rc->abc", *first), want[:k, :, :n])
        self._left = {1: _sum_program(first[0].tolist()), 2: _sum_program(u.tolist())}
        self._right = _sum_program(v.tolist())
        self._out = {1: _sum_program(first[2].T.tolist()), 2: _sum_program(w.T.tolist())}

    def left(self, rows):
        blocks = [blk for row in rows for blk in _column_blocks(row, self.inner)]
        return _evaluate(self._left[len(rows)], blocks.__getitem__)

    def right(self, blocks):
        return _evaluate(self._right, blocks.__getitem__)

    def combine(self, n_rows, product):
        c = _evaluate(self._out[n_rows], product)
        return [c[self.outer * i:self.outer * (i + 1)] for i in range(n_rows)]


def _parse(table):
    return [np.array([[{"+": 1, ".": 0, "-": -1}[c] for c in line.split()[f]]
                      for line in table]) for f in range(3)]


def _swap_inner_outer(u, v, w):
    k, n = u.shape[1] // 2, w.shape[1] // 2
    return w, v.reshape(-1, k, n).transpose(0, 2, 1).reshape(-1, k * n), u


_SQUARE = _Scheme(*_parse(_SCHEME_244))
_FROM_MODEL = _Scheme(*_parse(_SCHEME_254))
_TO_MODEL = _Scheme(*_swap_inner_outer(*_parse(_SCHEME_254)))


def _column_blocks(x, count):
    pad = count * _BLOCK - x.shape[1]
    if pad:
        x = jnp.concatenate([x, jnp.zeros((x.shape[0], pad), x.dtype)], axis=1)
    return [x[:, i * _BLOCK:(i + 1) * _BLOCK] for i in range(count)]


def _masks(n_mem, length, n_seq):
    rows = n_seq * length

    def describe(axis):
        i = lax.broadcasted_iota(jnp.int32, (rows, rows), axis)
        second = i >= length
        return jnp.where(second, 1, 0), jnp.where(second, i - length, i)

    (seq_r, idx_r), (seq_c, idx_c) = describe(0), describe(1)
    same = seq_r == seq_c
    keep = same & ((idx_r < n_mem) | (idx_r >= idx_c))
    fill = jnp.where(same, _MASKED * _LOG2E, -jnp.inf).astype(_F32)
    return keep, fill


def _attention(hs, keep, fill, qkv, wo, h_terms, o_sums,
               n_heads, dh):
    scale = dh ** -0.5
    n_groups = n_heads // _GROUP
    n_seq, length = len(hs), hs[0].shape[0]
    heads = [slice(i * dh, (i + 1) * dh) for i in range(_GROUP)]
    lhs_dtype = _BF16 if (n_seq * length) % 16 == 0 else _F32

    for i, t in enumerate(_FROM_MODEL.left(hs)):
        h_terms[i] = t

    def project(ws, g):
        c = _FROM_MODEL.combine(n_seq, lambda i: _dot(h_terms[i], jnp.concatenate(
            [_unpack(qkv[w, g, i]) for w in ws], axis=1)))
        return [jnp.concatenate(
            [jnp.concatenate([blk[:, n * dh:(n + 1) * dh] for blk in row], axis=1) for row in c],
            axis=0) for n in range(len(ws))]

    def weights(q, k):
        out = []
        for cols in heads:
            s = jnp.where(keep, _dot_nt(q[:, cols], k[:, cols]) * (scale * _LOG2E), fill)
            e = jnp.exp2(s - jnp.max(s, axis=-1, keepdims=True))
            out.append((e.astype(lhs_dtype), 1.0 / jnp.sum(e, axis=-1, keepdims=True)))
        return out

    def mix(p, v):
        return jnp.concatenate(
            [_dot(e, v[:, cols]) * inv for (e, inv), cols in zip(p, heads)], axis=1)

    def output(o, g):
        terms = _TO_MODEL.left([o[i * length:(i + 1) * length] for i in range(n_seq)])

        def product(i):
            part = _dot(terms[i], _unpack(wo[g, i]))
            return part if g == 0 else o_sums[i] + part

        if g == n_groups - 1:
            return _TO_MODEL.combine(n_seq, product)
        for i in range(len(terms)):
            o_sums[i] = product(i)

    proj, p, o, acc = {}, {}, {}, None
    for stage in range(n_groups + max(lag for _, lag in _STAGE_ORDER)):
        for task, lag in _STAGE_ORDER:
            g = stage - lag
            if not 0 <= g < n_groups:
                continue
            if task == "scores":
                p[g] = weights(proj.pop((0, g)), proj.pop((1, g)))
            elif task == "mix":
                o[g] = mix(p.pop(g), proj.pop((2, g)))
            elif task == "output":
                acc = output(o.pop(g), g)
            else:
                for w, x in zip(task, project(task, g)):
                    proj[w, g] = x.astype(lhs_dtype if w == 0 else _BF16)
    return [jnp.concatenate(row, axis=1)[:, :hs[0].shape[1]] for row in acc]


def _silu(x):
    half = 0.5 * x
    return half + half * jnp.tanh(half)


def _swiglu_one(x_terms, w1_terms, w3_terms, w2_t, tiles):
    quarter = w2_t.shape[1] // _FROM_MODEL.outer

    def project(terms, tile):
        c = _FROM_MODEL.combine(2, lambda i: _dot(x_terms[i], _unpack(terms[tile, i])))
        return jnp.concatenate([jnp.concatenate(row, axis=1) for row in c], axis=0)

    acc = hid = None
    for n in range(len(tiles) + 1):
        prev = hid
        if n < len(tiles):
            gate = _silu(project(w1_terms, tiles[n]))
            hid = (gate * project(w3_terms, tiles[n])).astype(_BF16)
        if n >= 1:
            starts = [pl.multiple_of(j * quarter + tiles[n - 1] * _BLOCK, _BLOCK)
                      for j in range(_FROM_MODEL.outer)]
            part = _dot_nt(
                jnp.concatenate([w2_t[:, pl.ds(c, _BLOCK)] for c in starts], axis=1), prev)
            acc = part if acc is None else acc + part
    return acc


def _swiglu_pair(x_terms, w1_terms, w3_terms, w2_terms, side_work):
    def project(terms, lo):
        c = _FROM_MODEL.combine(2, lambda i: _dot(x_terms[i], _unpack(terms[lo // _BLOCK, i])))
        return [jnp.concatenate(row, axis=1) for row in c]

    def hidden(lo):
        gates = [_silu(g) for g in project(w1_terms, lo)]
        hid = [g * u for g, u in zip(gates, project(w3_terms, lo))]
        return [t.astype(_BF16) for t in _SQUARE.left(hid)]

    chunks = list(range(0, w2_terms.shape[0] * _BLOCK, _PAIR_CHUNK))
    acc = hid = None
    for n in range(len(chunks) + 1):
        prev = hid
        if n < len(chunks):
            tiles = [hidden(lo) for lo in range(chunks[n], chunks[n] + _PAIR_CHUNK, _BLOCK)]
            hid = [jnp.concatenate(t, axis=1) for t in zip(*tiles)]
        if n >= 1:
            first = chunks[n - 1] // _BLOCK

            def product(i, first=first, prev=prev, acc=acc):
                left = [_unpack(w2_terms[first + c, i]) for c in range(_PAIR_CHUNK // _BLOCK)]
                part = _dot_nt(jnp.concatenate(left, axis=1), prev[i])
                return part if acc is None else acc[i] + part

            if n < len(chunks):
                acc = [product(i) for i in range(_SQUARE.products)]
            else:
                acc = _SQUARE.combine(2, product)
        side_work(n)
    return [jnp.concatenate(row, axis=0) for row in acc]


def _store_terms(w, terms, scheme, transposed):
    block_rows, block_cols = 2 * terms.shape[2], terms.shape[0] * _BLOCK

    def tile(j, carry):
        def block(r, c, lo):
            start = r * block_rows + j * 16
            rows = pl.ds(pl.multiple_of(jnp.minimum(start, w.shape[0] - 16), 16), 16)
            words = pltpu.bitcast(
                w[rows, c * block_cols + lo:c * block_cols + lo + _BLOCK], jnp.uint32)
            if (r + 1) * block_rows > w.shape[0]:
                words = jnp.where(start < w.shape[0], words, jnp.uint32(0))
            return words

        for lo in range(0, block_cols, _BLOCK):
            words = [block(n, k, lo) if transposed else block(k, n, lo)
                     for k in range(scheme.inner) for n in range(scheme.outer)]
            even, odd = (scheme.right(rows) for rows in zip(*map(_split_words, words)))
            for i, pair in enumerate(zip(even, odd)):
                terms[lo // _BLOCK, i, pl.ds(pl.multiple_of(j * 8, 8), 8)] = (
                    pltpu.pack_elementwise(pair, packed_dtype=_BF16))
        return carry

    lax.fori_loop(0, block_rows // 16, tile, 0)


def _load_weights(sources, qkv, wo_hbm, wo, stage, wo_stage, wsem, osem,
                  later_copies):
    d_model, n_heads, dh = sources[0].shape
    n_groups = n_heads // _GROUP
    per_weight = _BLOCK // _WCHUNK
    n_jobs = len(sources) * per_weight
    full = _FROM_MODEL.inner - 1
    ragged = (d_model - full * _BLOCK) // _WCHUNK
    stage[ragged:, full] = jnp.zeros((per_weight - ragged,) + stage.shape[2:], stage.dtype)

    def for_copies(src, job, action):
        c = job % per_weight

        def copy(n):
            action(pltpu.make_async_copy(src.at[pl.ds(n * _BLOCK + c * _WCHUNK, _WCHUNK)],
                                         stage.at[c, n], wsem.at[(full + 1) * c + n]))

        for n in range(full):
            copy(n)
        pl.when(c < ragged)(functools.partial(copy, full))

    def start(job):
        for i, src in enumerate(sources):
            pl.when(job // per_weight == i)(
                functools.partial(for_copies, src, job, lambda c: c.start()))

    def wait(job):
        for i, src in enumerate(sources):
            pl.when(job // per_weight == i)(
                functools.partial(for_copies, src, job, lambda c: c.wait()))

    def split_heads(slot, n, j):
        rows = pl.ds(pl.multiple_of(j * 16, 16), 16)
        words = jnp.swapaxes(pltpu.bitcast(stage[slot, n, rows], jnp.uint32), 0, 1)
        return [half for p in range(n_heads // 2) for half in _split_words(words[p])]

    def output_group(g, carry):
        def transposed(head):
            last = jnp.concatenate(
                [wo_stage[head, full * _BLOCK:],
                 jnp.zeros(((full + 1) * _BLOCK - d_model, dh), wo_stage.dtype)], axis=0)
            return jnp.concatenate([wo_stage[head, :full * _BLOCK].T, last.T], axis=1)

        heads = [transposed(_GROUP * g + i) for i in range(_GROUP)]
        for r in range(0, dh, 16):
            blocks = [blk for h in heads
                      for blk in _column_blocks(h[r:r + 16].astype(_F32), _TO_MODEL.outer)]
            for i, t in enumerate(_TO_MODEL.right(blocks)):
                wo[g, i, r // 2:r // 2 + 8] = _pack(t)
        return carry

    wo_copy = pltpu.make_async_copy(wo_hbm, wo_stage, osem)
    lax.fori_loop(0, _INFLIGHT, lambda job, carry: start(job), None)
    wo_copy.start()

    def groups_done(job):
        return jnp.minimum(2 * jnp.maximum(job - _WO_FROM, 0), n_groups)

    def run(job, carry):
        which, c = job // per_weight, job % per_weight
        wait(job)
        start(job + _INFLIGHT)

        @pl.when(job == n_jobs - _LATER_FROM)
        def _():
            for copy in later_copies:
                copy.start()


        def main_rows(j, carry):
            rows = pl.ds(pl.multiple_of(c * (_WCHUNK // 2) + j * 8, 8), 8)
            parts = [split_heads(c, n, j) for n in range(full + 1)]
            for g in range(n_groups):
                blocks = [h for part in parts for h in part[_GROUP * g:_GROUP * (g + 1)]]
                for n, t in enumerate(_FROM_MODEL.right(blocks)):
                    qkv[which, g, n, rows] = _pack(t)
            return carry

        lax.fori_loop(0, _WCHUNK // 16, main_rows, 0)
        pl.when(job == _WO_FROM)(wo_copy.wait)
        lax.fori_loop(groups_done(job), groups_done(job + 1), output_group, 0)
        return carry

    lax.fori_loop(0, n_jobs, run, 0)


def _kernel(x_hbm, mem0_ref, wq_hbm, wk_hbm, wv_hbm, wo_hbm, w1_hbm, w3_hbm,
            w2_hbm, out_hbm,
            x_all, out_all,
            stage, wo_stage, qkv, wo,
            w1, w3, w2_t, w1_terms, w3_terms, w2_terms,
            res, normed, mem, acc_t, x_terms, h_terms, o_sums,
            wsem, osem, fsem, xsem, *, seg):
    n_blocks = x_hbm.shape[1] // _TOK
    _, n_heads, dh = wq_hbm.shape
    n_mem = mem0_ref.shape[0]
    steps = _TOK // seg
    ffn_copies = [pltpu.make_async_copy(s, d, fsem.at[i])
                  for i, (s, d) in enumerate(((w1_hbm, w1), (w3_hbm, w3), (w2_hbm, w2_t)))]

    x_copies = [pltpu.make_async_copy(x_hbm.at[:, cols], x_all.at[:, cols], xsem.at[i])
                for i, cols in enumerate((pl.ds(0, _TOK), pl.ds(_TOK, (n_blocks - 1) * _TOK)))]

    def tokens(block):
        return pl.ds(pl.multiple_of(block * _TOK, _TOK), _TOK)

    def next_input(b):
        return x_all[:, tokens(jnp.minimum(b + 1, n_blocks - 1))].astype(_F32).T

    def out_copy(block):
        return pltpu.make_async_copy(out_all.at[:, tokens(block)], out_hbm.at[:, tokens(block)],
                                     xsem.at[2])

    def start_layer(slot, x):
        res[slot] = x
        normed[slot] = _layernorm(x)

    def prepare_swiglu(j):
        rows = pl.ds(pl.multiple_of(j * seg, seg), seg)
        for i, t in enumerate(_FROM_MODEL.left([_layernorm(res[n, rows]) for n in range(2)])):
            x_terms[i, rows] = t.astype(_BF16)

    x_copies[0].start()
    _load_weights((wq_hbm, wk_hbm, wv_hbm), qkv, wo_hbm, wo, stage, wo_stage, wsem, osem,
                  ffn_copies + x_copies[1:])
    mem[0] = mem0_ref[...].astype(_F32)
    mem[1] = mem0_ref[...].astype(_F32)
    x_copies[0].wait()
    start_layer(0, x_all[:, :_TOK].astype(_F32).T)

    def run_attention(first, n_seq):
        keep, fill = _masks(n_mem, n_mem + seg, n_seq)

        def segment(j, carry):
            rows = pl.ds(pl.multiple_of(j * seg, seg), seg)
            if n_seq == 2:
                prepare_swiglu(jnp.maximum(j - 1, 0))
            hs = [jnp.concatenate([mem[first + i], normed[first + i, rows]], axis=0)
                  for i in range(n_seq)]
            for i, out in enumerate(_attention(hs, keep, fill, qkv, wo, h_terms,
                                               o_sums, n_heads, dh)):
                mem[first + i] = out[:n_mem]
                res[first + i, rows] += out[n_mem:]
            return carry

        lax.fori_loop(0, steps, segment, 0)

    def block_step(b, carry):
        both = jnp.logical_and(b > 0, b < n_blocks)

        @pl.when(both)
        def _():
            run_attention(0, 2)
            prepare_swiglu(steps - 1)

            def side_work(n):
                if n == 0:
                    acc_t[...] = res[1].T
                    res[1] = res[0]
                if n == 1:
                    start_layer(0, next_input(b))

            f2, f4 = _swiglu_pair(x_terms, w1_terms, w3_terms, w2_terms, side_work)
            start_layer(1, res[1] + f2.T)
            out_all[:, tokens(b - 1)] = (acc_t[...] + f4).astype(out_all.dtype)

        @pl.when(jnp.logical_not(both))
        def _():
            slot = jnp.where(b == 0, 0, 1)
            run_attention(slot, 1)

            @pl.when(b == 0)
            def _():
                for c, w, terms in zip(ffn_copies, (w1, w3, w2_t), (w1_terms, w3_terms, w2_terms)):
                    c.wait()
                    _store_terms(w, terms, _SQUARE if w is w2_t else _FROM_MODEL, w is w2_t)

            x = res[slot]
            xn = _layernorm(x)
            terms = [t.astype(_BF16) for t in _FROM_MODEL.left([xn[:_TOK // 2], xn[_TOK // 2:]])]
            acc_t[...] = x.T

            def part(i, carry):
                tiles = [i * _EDGE_TILES + t for t in range(_EDGE_TILES)]
                acc_t[...] += _swiglu_one(terms, w1_terms, w3_terms, w2_t, tiles)
                return carry

            lax.fori_loop(0, w1_terms.shape[0] // _EDGE_TILES, part, 0)

            @pl.when(b == 0)
            def _():
                x_copies[1].wait()
                start_layer(1, acc_t[...].T)
                start_layer(0, next_input(b))

            @pl.when(b > 0)
            def _():
                out_all[:, tokens(b - 1)] = acc_t[...].astype(out_all.dtype)

        @pl.when(b > 1)
        def _():
            out_copy(b - 2).wait()

        @pl.when(b > 0)
        def _():
            out_copy(b - 1).start()

        return carry

    lax.fori_loop(0, n_blocks + 1, block_step, 0)
    out_copy(n_blocks - 1).wait()


@functools.partial(jax.jit, static_argnames=("A_seg_len",))
def pallas_interleave_layers__memory_aug_recurrent_mem_tr__glu_gated_swiglu__prompt_kernel(
    A_x: jax.Array,
    A_mem0: jax.Array,
    A_Wq: jax.Array,
    A_Wk: jax.Array,
    A_Wv: jax.Array,
    A_Wo: jax.Array,
    A_seg_len: int,
    B_x: jax.Array,
    B_w1: jax.Array,
    B_w3: jax.Array,
    B_w2: jax.Array,
):
    del B_x
    batch, seq, d_model = A_x.shape
    n_mem = A_mem0.shape[1]
    _, n_heads, dh = A_Wq.shape
    d_ff = B_w1.shape[1]
    seg = int(A_seg_len)
    assert batch == 1 and seq % _TOK == 0 and _TOK % seg == 0 and seg % 16 == 0
    assert n_mem == 8 and n_heads % _GROUP == 0 and d_ff % (4 * _BLOCK * _EDGE_TILES) == 0
    slots = _BLOCK // _WCHUNK
    assert _INFLIGHT < slots and d_model % 64 == 0
    assert (_FROM_MODEL.inner - 1) * _BLOCK < d_model < _FROM_MODEL.inner * _BLOCK
    assert dh == _BLOCK and d_ff % (4 * _PAIR_CHUNK) == 0
    ff_tiles = d_ff // (4 * _BLOCK)
    n_blocks = seq // _TOK

    hbm = pl.BlockSpec(memory_space=pl.ANY)
    out_t = pl.pallas_call(
        functools.partial(_kernel, seg=seg),
        in_specs=[hbm, pl.BlockSpec(memory_space=pltpu.VMEM)] + 7 * [hbm],
        out_specs=hbm,
        out_shape=jax.ShapeDtypeStruct((d_model, seq), A_x.dtype),
        scratch_shapes=[
            pltpu.VMEM((d_model, seq), A_x.dtype),
            pltpu.VMEM((d_model, seq), A_x.dtype),
            pltpu.VMEM((slots, _FROM_MODEL.inner, _WCHUNK, n_heads, dh), _BF16),
            pltpu.VMEM((n_heads, d_model, dh), _BF16),
            pltpu.VMEM((3, n_heads // _GROUP, _FROM_MODEL.products, _BLOCK // 2, dh), jnp.uint32),
            pltpu.VMEM((n_heads // _GROUP, _TO_MODEL.products, dh // 2, _BLOCK), jnp.uint32),
            pltpu.VMEM((d_model, d_ff), _BF16),
            pltpu.VMEM((d_model, d_ff), _BF16),
            pltpu.VMEM((d_model, d_ff), _BF16),
            *2 * [pltpu.VMEM((ff_tiles, _FROM_MODEL.products, _BLOCK // 2, _BLOCK), jnp.uint32)],
            pltpu.VMEM((ff_tiles, _SQUARE.products, d_model // 8, _BLOCK), jnp.uint32),
            pltpu.VMEM((2, _TOK, d_model), _F32),
            pltpu.VMEM((2, _TOK, d_model), _F32),
            pltpu.VMEM((2, n_mem, d_model), _F32),
            pltpu.VMEM((d_model, _TOK), _F32),
            pltpu.VMEM((_FROM_MODEL.products, _TOK, _BLOCK), _BF16),
            pltpu.VMEM((_FROM_MODEL.products, n_mem + seg, _BLOCK), _F32),
            pltpu.VMEM((_TO_MODEL.products, n_mem + seg, _BLOCK), _F32),
            pltpu.SemaphoreType.DMA((slots * _FROM_MODEL.inner,)),
            pltpu.SemaphoreType.DMA(()),
            pltpu.SemaphoreType.DMA((3,)),
            pltpu.SemaphoreType.DMA((3,)),
        ],
        compiler_params=pltpu.CompilerParams(
            vmem_limit_bytes=112 * 1024 * 1024,
        ),
    )(A_x[0].T, A_mem0[0], A_Wq, A_Wk, A_Wv, jnp.transpose(A_Wo, (0, 2, 1)),
      B_w1, B_w3, B_w2.T)
    return out_t.T[None]
```
